```python
import jax
import jax.numpy as jnp

def _softmax(x, axis=-1):
    return jax.nn.softmax(x, axis=axis)
def _gelu(x):
    return jax.nn.gelu(x, approximate=True)
def _silu(x):
    return jax.nn.silu(x)
def _sigmoid(x):
    return jax.nn.sigmoid(x)
def _layernorm(x, axis=-1, eps=1e-5):
    m = jnp.mean(x, axis=axis, keepdims=True)
    v = jnp.var(x, axis=axis, keepdims=True)
    return (x - m) / jnp.sqrt(v + eps)
def _scatter_add(tgt, idx, src, axis=0):
    return tgt.at[idx].add(src)
def _segment_sum(src, seg, n):
    return jax.ops.segment_sum(src, seg, n)
class _Rng:
    def __init__(self, key):
        self._k = key
    def _next(self):
        self._k, sub = jax.random.split(self._k)
        return sub
    def normal(self, shape):
        return jax.random.normal(self._next(), shape, dtype=jnp.bfloat16)
    def randint(self, lo, hi, shape):
        return jax.random.randint(self._next(), shape, lo, hi, dtype=jnp.int32)
    def uniform(self, shape, lo=0.0, hi=1.0):
        return jax.random.uniform(self._next(), shape, jnp.bfloat16, lo, hi)
    def permutation(self, n):
        return jax.random.permutation(self._next(), n)


kernel_name = 'gated_mix__linear_kernel_hedgehog__moe_arch_mod__prompt'

def setup_inputs():
    _rng = _Rng(jax.random.key(int.from_bytes(__import__("os").urandom(4), "little")))
    _w = (lambda a: (lambda t: t.astype(jnp.bfloat16) if jnp.issubdtype(t.dtype, jnp.floating) else t)(jnp.asarray(a)))
    def _A_setup():
        B, S, D, H = 1, 2048, 1024, 32
        Dh = D // H
        return {
            "x": _w((lambda *s: _rng.normal(s) * 0.05)(B, S, D)),
            "wqkv": _w((lambda *s: _rng.normal(s) * 0.05)(D, 3 * D)),
            "w_phi": _w((lambda *s: _rng.normal(s) * 0.05)(H, Dh, Dh) * (Dh ** -0.5)),
            "wo": _w((lambda *s: _rng.normal(s) * 0.05)(D, D)),
        }
    _A_in = _A_setup()

    def _B_setup():
        B, S, D, F, C = 1, 2048, 1024, 3584, 1
        return {
            "x": _w((lambda *s: _rng.normal(s) * 0.05)(B, S, D)),
            "w_r": _w((lambda *s: _rng.normal(s) * 0.05)(D)),
            "w_gate": _w((lambda *s: _rng.normal(s) * 0.05)(D, F)),
            "w_up": _w((lambda *s: _rng.normal(s) * 0.05)(D, F)),
            "w_down": _w((lambda *s: _rng.normal(s) * 0.05)(F, D)),
        }
    _B_in = _B_setup()

    return {
        "A_x": _A_in["x"],
        "A_wqkv": _A_in["wqkv"],
        "A_w_phi": _A_in["w_phi"],
        "A_wo": _A_in["wo"],
        "B_x": _B_in["x"],
        "B_w_r": _B_in["w_r"],
        "B_w_gate": _B_in["w_gate"],
        "B_w_up": _B_in["w_up"],
        "B_w_down": _B_in["w_down"],
        "gate_w": _w((lambda *s: _rng.normal(s) * 0.05)(1024)),
    }

def reference(A_x, A_wqkv, A_w_phi, A_wo, B_x, B_w_r, B_w_gate, B_w_up, B_w_down, gate_w):
    def _A_ref(x, wqkv, w_phi, wo):
        B, S, D = x.shape
        H = 32; Dh = D // H
        qkv = (lambda x, *d: x.transpose(*d))((x @ wqkv).reshape(B, S, 3, H, Dh), 2, 0, 3, 1, 4)
        q, k, v = qkv[0], qkv[1], qkv[2]
        pq = jnp.einsum("bhsd,hdf->bhsf", q, w_phi)
        pk = jnp.einsum("bhsd,hdf->bhsf", k, w_phi)
        phi_q = jnp.concatenate([_softmax(pq, axis=-1), _softmax(-pq, axis=-1)], axis=-1)
        phi_k = jnp.concatenate([_softmax(pk, axis=-1), _softmax(-pk, axis=-1)], axis=-1)
        kv = jnp.einsum("bhsf,bhsd->bhfd", phi_k, v)
        z  = jnp.einsum("bhsf->bhf", phi_k)
        num = jnp.einsum("bhqf,bhfd->bhqd", phi_q, kv)
        den = jnp.einsum("bhqf,bhf->bhq", phi_q, z)[..., None] + 1e-6
        o = num / den
        return (lambda x, *d: x.transpose(*d))(o, 0, 2, 1, 3).reshape(B, S, D) @ wo

    def _B_ref(x, w_r, w_gate, w_up, w_down):
        B, S, D = x.shape
        C = 1
        r = x @ w_r
        idx = jnp.argsort(-r, axis=-1)[:, :C]
        idx_e = jnp.repeat(idx.reshape(B, C, 1), D, axis=2)
        x_sel = jnp.take_along_axis(x, idx_e, axis=1)
        g = _silu(x_sel @ w_gate)
        u = x_sel @ w_up
        y = (g * u) @ w_down
        r_sel = _sigmoid(jnp.take_along_axis(r, idx, axis=1))
        y = y * r_sel.reshape(B, C, 1)
        b_off = (jnp.arange(B) * S).reshape(B, 1)
        flat_idx = (idx + b_off).reshape(B * C)
        zero = (x * 0.0).reshape(B * S, D)
        upd = _scatter_add(zero, flat_idx, y.reshape(B * C, D), axis=0)
        return x + upd.reshape(B, S, D)

    x = A_x
    g = _sigmoid((x * gate_w).sum(-1, keepdims=True))
    a = _A_ref(x, A_wqkv, A_w_phi, A_wo)
    b = _B_ref(x, B_w_r, B_w_gate, B_w_up, B_w_down)
    return g * a + (1 - g) * b
```

```python
import jax
import jax.numpy as jnp
from jax import lax
from jax.experimental import pallas as pl
from jax.experimental.pallas import tpu as pltpu

S, D, H, DH, F = 2048, 1024, 32, 32, 3584
T = 512
NT = S // T
RC = 256
NPAIR = H // 2
LOG2E = 1.4426950408889634
F32, BF16 = jnp.float32, jnp.bfloat16
NT_DIMS = (((1,), (1,)), ((), ()))
TN_DIMS = (((0,), (0,)), ((), ()))


def _tree(op, xs):
    xs = list(xs)
    while len(xs) > 1:
        xs = [op(xs[i], xs[i + 1]) if i + 1 < len(xs) else xs[i]
              for i in range(0, len(xs), 2)]
    return xs[0]


def _allreduce(op, xs):
    r = _tree(op, xs)
    r = op(r, pltpu.roll(r, 4, 0))
    return op(r, pltpu.roll(r, 2, 0))


def _features(p):
    rows = [p[8 * i:8 * i + 8, :] for i in range(8)]
    mx = _allreduce(jnp.maximum, rows)
    mn = _allreduce(jnp.minimum, rows)
    ep = [jnp.exp2(r - mx) for r in rows]
    en = [jnp.exp2(mn - r) for r in rows]
    rp = 1.0 / _allreduce(jnp.add, ep)
    rn = 1.0 / _allreduce(jnp.add, en)
    return [e * rp for e in ep] + [e * rn for e in en]


def _kernel(xa_hbm, wqkv_hbm, wphi_ref, wo_hbm, wr_ref, wg_hbm, wu_hbm,
            wd_hbm, gw_ref, out_hbm,
            xa, wqkv, wo, wg, wu, wd, wt, vt, phi, ot, kvacc, kvt, zacc,
            gate, outb, sem_xa, sem_xb, sem_w, sem_f, sem_o):
    def tile(i):
        return pl.ds(pl.multiple_of(i * T, T), T)

    def xa_cp(i):
        return pltpu.make_async_copy(xa_hbm.at[tile(i)], xa.at[tile(i)], sem_xa.at[i])

    def res_cp(i):
        return pltpu.make_async_copy(xa_hbm.at[tile(i)], xa.at[pl.ds(S, T)], sem_xb.at[0])

    def w_cp(j):
        c = pl.ds(j * D, D)
        return pltpu.make_async_copy(wqkv_hbm.at[:, c], wqkv.at[:, c], sem_w.at[j])

    wo_cp = pltpu.make_async_copy(wo_hbm, wo, sem_w.at[3])
    ffn_cp = [pltpu.make_async_copy(wg_hbm, wg, sem_f.at[0]),
              pltpu.make_async_copy(wu_hbm, wu, sem_f.at[1]),
              pltpu.make_async_copy(wd_hbm, wd, sem_f.at[2])]

    def out_cp(i, slot):
        return pltpu.make_async_copy(outb.at[tile(i)], out_hbm.at[tile(i)], sem_o.at[slot])

    w_cp(1).start()
    xa_cp(0).start()
    w_cp(2).start()

    er = lax.broadcasted_iota(jnp.int32, (128, DH), 0)
    ec = lax.broadcasted_iota(jnp.int32, (128, DH), 1)
    expand = jnp.where((er % 64) // 2 == ec, 1.0, 0.0).astype(BF16)
    pt = lax.dot_general(expand, wphi_ref[...], NT_DIMS, preferred_element_type=F32)
    pr = lax.broadcasted_iota(jnp.int32, (128, D), 0)
    pc = lax.broadcasted_iota(jnp.int32, (128, D), 1)
    pt = jnp.where((pc // DH) % 4 == 2 * (pr // 64) + pr % 2, pt, 0.0).astype(BF16)

    def fold(j):
        for g in range(D // 128):
            c = slice(g * 128, (g + 1) * 128)
            w = wqkv[:, j * D + g * 128:j * D + (g + 1) * 128]
            r = lax.dot_general(pt[:, c], w, NT_DIMS, preferred_element_type=F32)
            wt[j, c, :] = (r * LOG2E).astype(BF16)

    w_cp(1).wait()
    fold(1)
    w_cp(2).wait()
    for g in range(D // 128):
        c = slice(g * 128, (g + 1) * 128)
        wt[2, c, :] = wqkv[:, 2 * D + g * 128:2 * D + (g + 1) * 128].T

    kvacc[...] = jnp.zeros_like(kvacc)
    zacc[...] = jnp.zeros_like(zacc)
    wr = wr_ref[...].astype(F32).reshape(1, D)
    gw = gw_ref[...].astype(F32).reshape(1, D)

    def phase1(i, carry):
        best, bidx = carry

        @pl.when(i + 1 < NT)
        def _():
            xa_cp(i + 1).start()

        @pl.when(i == 0)
        def _():
            w_cp(0).start()
            ffn_cp[0].start()

        @pl.when(i == 1)
        def _():
            ffn_cp[1].start()

        @pl.when(i == 2)
        def _():
            wo_cp.start()
            ffn_cp[2].start()

        xa_cp(i).wait()
        x = xa[tile(i), :]
        for c in range(D // RC):
            rows = slice(c * RC, (c + 1) * RC)
            p = lax.dot_general(wt[1, rows, :], x, NT_DIMS, preferred_element_type=F32)
            for q in range(RC // 64):
                g = c * (RC // 64) + q
                ph = _features(p[64 * q:64 * q + 64, :])
                zs = [_tree(jnp.add, [a[:, 128 * l:128 * l + 128] for l in range(T // 128)])
                      for a in ph]
                zacc[128 * g:128 * g + 128, :] += jnp.concatenate(zs, axis=0)
                phi[128 * g:128 * g + 128, :] = jnp.concatenate(ph, axis=0).astype(BF16)
        for c in range(D // RC):
            rows = slice(c * RC, (c + 1) * RC)
            v = lax.dot_general(wt[2, rows, :], x, NT_DIMS, preferred_element_type=F32)
            vt[rows, :] = v.astype(BF16)
        for g in range(NPAIR):
            kvacc[64 * g:64 * g + 64, :] += lax.dot_general(
                vt[64 * g:64 * g + 64, :], phi[128 * g:128 * g + 128, :], NT_DIMS,
                preferred_element_type=F32)

        gate[tile(i), :] = jax.nn.sigmoid(
            jnp.sum(x.astype(F32) * gw, axis=-1, keepdims=True))
        r = jnp.sum(x.astype(F32) * wr, axis=-1, keepdims=True)
        r = r.astype(BF16).astype(F32)
        tok = i * T + lax.broadcasted_iota(jnp.int32, (T, 1), 0)
        m = jnp.max(r, axis=0, keepdims=True)
        mi = jnp.min(jnp.where(r == m, tok, S), axis=0, keepdims=True)
        better = m > best
        return jnp.where(better, m, best), jnp.where(better, mi, bidx)

    best, bidx = lax.fori_loop(
        0, NT, phase1,
        (jnp.full((1, 1), -jnp.inf, F32), jnp.zeros((1, 1), jnp.int32)))
    idx = jnp.clip(bidx[0, 0], 0, S - 1)
    last = idx // T
    res_cp(last).start()

    w_cp(0).wait()
    fold(0)
    kr = lax.broadcasted_iota(jnp.int32, (D, 128), 0)
    kc = lax.broadcasted_iota(jnp.int32, (D, 128), 1)
    kvt[...] = jnp.where((kr // DH) % 2 == kc % 2, kvacc[...], 0.0).astype(BF16)
    zacc[...] = jnp.broadcast_to(jnp.sum(zacc[...], axis=-1, keepdims=True), zacc.shape)
    wo_cp.wait()

    def phase2(i, carry):
        t = (last + 1 + i) % NT

        @pl.when(i == NT - 1)
        def _():
            for cp in ffn_cp + [res_cp(last)]:
                cp.wait()
            slab = pl.ds(pl.multiple_of(S + ((idx % T) // 16) * 16, 16), 16)
            xs = xa[slab, :]
            sel = lax.broadcasted_iota(jnp.int32, (16, D), 0) == idx % 16
            xsel = jnp.where(sel, xs, jnp.zeros_like(xs))
            a = jnp.dot(xsel, wg[...], preferred_element_type=F32)
            u = jnp.dot(xsel, wu[...], preferred_element_type=F32)
            h = (a * jax.nn.sigmoid(a) * u).astype(BF16)
            y = jnp.dot(h, wd[...], preferred_element_type=F32) * jax.nn.sigmoid(best)
            xa[slab, :] = jnp.where(sel, xs.astype(F32) + y, xs.astype(F32)).astype(BF16)

        x = xa[tile(t), :]
        for c in range(D // RC):
            rows = slice(c * RC, (c + 1) * RC)
            p = lax.dot_general(wt[0, rows, :], x, NT_DIMS, preferred_element_type=F32)
            for q in range(RC // 64):
                g = c * (RC // 64) + q
                ph = _features(p[64 * q:64 * q + 64, :])
                zb = zacc[128 * g:128 * g + 128, :]
                dn = [a * jnp.tile(zb[8 * k:8 * k + 8, :], (1, T // 128))
                      for k, a in enumerate(ph)]
                rden = 1.0 / (_allreduce(jnp.add, dn) + 1e-6)
                num = jnp.dot(kvt[64 * g:64 * g + 64, :],
                              jnp.concatenate(ph, axis=0).astype(BF16),
                              preferred_element_type=F32)
                scale = jnp.concatenate(
                    [jnp.broadcast_to(rden[0:1, :], (DH, T)),
                     jnp.broadcast_to(rden[1:2, :], (DH, T))], axis=0)
                ot[64 * g:64 * g + 64, :] = (num * scale).astype(BF16)
        a = lax.dot_general(ot[...], wo[...], TN_DIMS, preferred_element_type=F32)
        gt = gate[tile(t), :]
        outb[tile(t), :] = (gt * a + (1.0 - gt) * xa[tile(jnp.where(i == NT - 1, NT, t)), :].astype(F32)).astype(BF16)
        out_cp(t, i).start()
        return carry

    lax.fori_loop(0, NT, phase2, 0)
    for i in range(NT):
        out_cp(i, i).wait()


@jax.jit
def pallas_gated_mix__linear_kernel_hedgehog__moe_arch_mod__prompt_kernel(
    A_x, A_wqkv, A_w_phi, A_wo, B_x, B_w_r, B_w_gate, B_w_up, B_w_down, gate_w,
):
    hbm = pl.BlockSpec(memory_space=pl.ANY)
    vmem = pl.BlockSpec(memory_space=pltpu.VMEM)
    out = pl.pallas_call(
        _kernel,
        out_shape=jax.ShapeDtypeStruct((S, D), BF16),
        in_specs=[hbm, hbm, vmem, hbm, vmem, hbm, hbm, hbm, vmem],
        out_specs=hbm,
        scratch_shapes=[
            pltpu.VMEM((S + T, D), BF16),
            pltpu.VMEM((D, 3 * D), BF16),
            pltpu.VMEM((D, D), BF16),
            pltpu.VMEM((D, F), BF16),
            pltpu.VMEM((D, F), BF16),
            pltpu.VMEM((F, D), BF16),
            pltpu.VMEM((3, D, D), BF16),
            pltpu.VMEM((D, T), BF16),
            pltpu.VMEM((2 * D, T), BF16),
            pltpu.VMEM((D, T), BF16),
            pltpu.VMEM((D, 128), F32),
            pltpu.VMEM((D, 128), BF16),
            pltpu.VMEM((2 * D, 128), F32),
            pltpu.VMEM((S, 1), F32),
            pltpu.VMEM((S, D), BF16),
            pltpu.SemaphoreType.DMA((NT,)),
            pltpu.SemaphoreType.DMA((1,)),
            pltpu.SemaphoreType.DMA((4,)),
            pltpu.SemaphoreType.DMA((3,)),
            pltpu.SemaphoreType.DMA((NT,)),
        ],
        compiler_params=pltpu.CompilerParams(vmem_limit_bytes=110 * 2**20),
    )(A_x.reshape(S, D), A_wqkv, A_w_phi.reshape(H * DH, DH), A_wo,
      B_w_r, B_w_gate, B_w_up, B_w_down, gate_w)
    return out.reshape(1, S, D)
```

```python
import jax
import jax.numpy as jnp
from jax import lax
from jax.experimental import pallas as pl
from jax.experimental.pallas import tpu as pltpu

S, D, H, DH, F = 2048, 1024, 32, 32, 3584
T = 512
NT = S // T
RC = 256
NC = D // RC
UNROLL1 = False
UNROLL2 = False
SCOPES = False
LOG2E = 1.4426950408889634
F32, BF16, U32 = jnp.float32, jnp.bfloat16, jnp.uint32
NT_DIMS = (((1,), (1,)), ((), ()))
TN_DIMS = (((0,), (0,)), ((), ()))


def _tree(op, xs):
    xs = list(xs)
    while len(xs) > 1:
        xs = [op(xs[i], xs[i + 1]) if i + 1 < len(xs) else xs[i]
              for i in range(0, len(xs), 2)]
    return xs[0]


def _allreduce(op, xs):
    r = _tree(op, xs)
    r = op(r, pltpu.roll(r, 4, 0))
    return op(r, pltpu.roll(r, 2, 0))


def _features(p):
    rows = [p[8 * i:8 * i + 8, :] for i in range(8)]
    mx = _allreduce(jnp.maximum, rows)
    mn = _allreduce(jnp.minimum, rows)
    ep = [jnp.exp2(r - mx) for r in rows]
    en = [jnp.exp2(mn - r) for r in rows]
    rp = 1.0 / _allreduce(jnp.add, ep)
    rn = 1.0 / _allreduce(jnp.add, en)
    return [e * rp for e in ep] + [e * rn for e in en]


def _pack(x):
    return pltpu.bitcast(x.astype(BF16), jnp.uint32)


def _unpack(x):
    return pltpu.bitcast(x, BF16)


def _start(*cps):
    def step(i, carry):
        for n, cp in enumerate(cps):
            pl.when(i == n)(cp.start)
        return carry

    lax.fori_loop(0, len(cps), step, 0)


def _wait(name, *cps):
    if SCOPES:
        with jax.named_scope(name):
            for cp in cps:
                cp.wait()
    else:
        for cp in cps:
            cp.wait()


def _kernel(xa_hbm, wqkv_hbm, wphi_hbm, wo_hbm, wr_ref, wg_hbm, wu_hbm,
            wd_hbm, gw_ref, out_hbm,
            xa, wqkv, wphi, wo, wg, wu, wd, wq_t, wk_t, wv_t, vt, phi, ot, kvacc, kvt, zacc,
            gate, score, outb, pbuf, sem_x, sem_w, sem_m, sem_o):
    def tile(i):
        if isinstance(i, int):
            return pl.ds(i * T, T)
        return pl.ds(pl.multiple_of(i * T, T), T)

    def xa_cp(i):
        return pltpu.make_async_copy(xa_hbm.at[tile(i)], xa.at[tile(i)], sem_x.at[i])

    def res_cp(i):
        return pltpu.make_async_copy(xa_hbm.at[tile(i)], xa.at[pl.ds(S, T)], sem_x.at[NT])

    def w_cp(j, c):
        cols = pl.ds(j * D + c * RC, RC)
        return pltpu.make_async_copy(wqkv_hbm.at[:, cols], wqkv.at[:, cols], sem_w.at[j * NC + c])

    phi_cp = pltpu.make_async_copy(wphi_hbm, wphi, sem_m.at[0])
    wo_cp = pltpu.make_async_copy(wo_hbm, wo, sem_m.at[1])
    ffn_cp = [pltpu.make_async_copy(wg_hbm, wg, sem_m.at[2]),
              pltpu.make_async_copy(wu_hbm, wu, sem_m.at[3]),
              pltpu.make_async_copy(wd_hbm, wd, sem_m.at[4])]

    def out_cp(i, slot):
        return pltpu.make_async_copy(outb.at[tile(i)], out_hbm.at[tile(i)], sem_o.at[slot])

    _start(phi_cp, w_cp(1, 0), xa_cp(0), *[w_cp(1, c) for c in range(1, NC)],
           *[w_cp(2, c) for c in range(NC)], *[xa_cp(i) for i in range(1, NT)],
           *[w_cp(0, c) for c in range(NC)], wo_cp, *ffn_cp)

    er = lax.broadcasted_iota(jnp.int32, (128, DH), 0)
    ec = lax.broadcasted_iota(jnp.int32, (128, DH), 1)
    expand = jnp.where((er % 64) // 2 == ec, 1.0, 0.0).astype(BF16)
    pr = lax.broadcasted_iota(jnp.int32, (128, 128), 0)
    pc = lax.broadcasted_iota(jnp.int32, (128, 128), 1)
    diag = pc // DH == 2 * (pr // 64) + pr % 2
    kvacc[...] = jnp.zeros_like(kvacc)
    zacc[...] = jnp.zeros_like(zacc)
    xr = lax.broadcasted_iota(jnp.int32, (16, D), 0)
    wv_t[D // 2:D // 2 + 8, :] = _pack(jnp.where(
        xr == 0, gw_ref[...].astype(F32).reshape(1, D),
        jnp.where(xr == 1, wr_ref[...].astype(F32).reshape(1, D), 0.0)))
    _wait("wait_phi", phi_cp)

    def fold(j, dst, c):
        for g in range(c * RC // 128, (c + 1) * RC // 128):
            rows = slice(g * 128, (g + 1) * 128)
            pt = lax.dot_general(expand, wphi[rows, :], NT_DIMS, preferred_element_type=F32)
            pt = jnp.where(diag, pt, 0.0).astype(BF16)
            w = wqkv[:, j * D + g * 128:j * D + (g + 1) * 128]
            r = lax.dot_general(pt, w, NT_DIMS, preferred_element_type=F32)
            dst[g * 64:(g + 1) * 64, :] = _pack(r * LOG2E)

    def transpose_v(c):
        for g in range(c * RC // 128, (c + 1) * RC // 128):
            wv_t[g * 64:(g + 1) * 64, :] = _pack(wqkv[:, 2 * D + g * 128:2 * D + (g + 1) * 128].T)

    def k_logits(i, c):
        return lax.dot_general(_unpack(wk_t[c * RC // 2:(c + 1) * RC // 2, :]), xa[tile(i), :], NT_DIMS,
                               preferred_element_type=F32)

    def k_features(p, c):
        for q in range(RC // 64):
            g = c * (RC // 64) + q
            ph = _features(p[64 * q:64 * q + 64, :])
            zs = [_tree(jnp.add, [a[:, 128 * l:128 * l + 128] for l in range(T // 128)])
                  for a in ph]
            zacc[128 * g:128 * g + 128, :] += jnp.concatenate(zs, axis=0)
            phi[64 * g:64 * g + 64, :] = _pack(jnp.concatenate(ph, axis=0))

    def values(i):
        for c in range(NC):
            extra = 16 if c == NC - 1 else 0
            v = lax.dot_general(_unpack(wv_t[c * RC // 2:((c + 1) * RC + extra) // 2, :]), xa[tile(i), :], NT_DIMS,
                                preferred_element_type=F32)
            vt[c * RC // 2:(c + 1) * RC // 2, :] = _pack(v[:RC, :])
            if extra:
                gr = v[RC:RC + 8, :]
                score[:, tile(i)] = gr
                gt = jax.nn.sigmoid(gr)
                gate[tile(i), :] = jnp.broadcast_to(gt[0:1, :], (128, T)).T
            for g in range(c * RC // 64, (c + 1) * RC // 64):
                kvacc[64 * g:64 * g + 64, :] += lax.dot_general(
                    _unpack(vt[32 * g:32 * g + 32, :]), _unpack(phi[64 * g:64 * g + 64, :]), NT_DIMS,
                    preferred_element_type=F32)

    _wait("wait_wk", w_cp(1, 0))
    fold(1, wk_t, 0)
    _wait("wait_x", xa_cp(0))
    pbuf[...] = k_logits(0, 0)
    _wait("wait_wk", *[w_cp(1, c) for c in range(1, NC)])
    k_features(pbuf[...], 0)
    for c in range(1, NC):
        fold(1, wk_t, c)
    for c in range(1, NC - 2):
        k_features(k_logits(0, c), c)
    pbuf[...] = k_logits(0, NC - 2)
    _wait("wait_wv", *[w_cp(2, c) for c in range(NC)])
    k_features(pbuf[...], NC - 2)
    for c in range(NC):
        transpose_v(c)
    k_features(k_logits(0, NC - 1), NC - 1)
    values(0)

    def phase1(i):
        _wait("wait_x", xa_cp(i))
        for c in range(NC):
            k_features(k_logits(i, c), c)
        values(i)

    if UNROLL1:
        for i in range(1, NT):
            phase1(i)
    else:
        lax.fori_loop(1, NT, lambda i, c: phase1(i), None)

    r = score[1:2, :].astype(BF16).astype(F32)
    best = jnp.max(r, axis=-1, keepdims=True)
    tok = lax.broadcasted_iota(jnp.int32, (1, S), 1)
    idx = jnp.min(jnp.where(r == best, tok, S - 1))
    last = idx // T
    res_cp(last).start()
    _wait("wait_wq", *[w_cp(0, c) for c in range(NC)], wo_cp)
    for c in range(NC):
        fold(0, wq_t, c)
    kr = lax.broadcasted_iota(jnp.int32, (D, 128), 0)
    kc = lax.broadcasted_iota(jnp.int32, (D, 128), 1)
    kvt[...] = _pack(jnp.where((kr // DH) % 2 == kc % 2, kvacc[...], 0.0))
    zacc[...] = jnp.broadcast_to(jnp.sum(zacc[...], axis=-1, keepdims=True), zacc.shape)

    def ffn():
        _wait("wait_ffn", *ffn_cp, res_cp(last))
        slab = pl.ds(pl.multiple_of(S + ((idx % T) // 16) * 16, 16), 16)
        xs = xa[slab, :]
        sel = lax.broadcasted_iota(jnp.int32, (16, D), 0) == idx % 16
        xsel = jnp.where(sel, xs, jnp.zeros_like(xs))
        a = jnp.dot(xsel, wg[...], preferred_element_type=F32)
        u = jnp.dot(xsel, wu[...], preferred_element_type=F32)
        h = (a * jax.nn.sigmoid(a) * u).astype(BF16)
        y = jnp.dot(h, wd[...], preferred_element_type=F32) * jax.nn.sigmoid(best)
        xa[slab, :] = jnp.where(sel, xs.astype(F32) + y, xs.astype(F32)).astype(BF16)

    def phase2(i):
        t = (last + 1 + i) % NT
        if isinstance(i, int):
            if i == NT - 1:
                ffn()
            res = NT if i == NT - 1 else t
        else:
            pl.when(i == NT - 1)(ffn)
            res = jnp.where(i == NT - 1, NT, t)
        for c in range(NC):
            rows = slice(c * RC, (c + 1) * RC)
            p = lax.dot_general(_unpack(wq_t[c * RC // 2:(c + 1) * RC // 2, :]), xa[tile(t), :], NT_DIMS, preferred_element_type=F32)
            for q in range(RC // 64):
                g = c * (RC // 64) + q
                ph = _features(p[64 * q:64 * q + 64, :])
                zb = zacc[128 * g:128 * g + 128, :]
                dn = [a * jnp.tile(zb[8 * k:8 * k + 8, :], (1, T // 128))
                      for k, a in enumerate(ph)]
                rden = 1.0 / (_allreduce(jnp.add, dn) + 1e-6)
                num = jnp.dot(_unpack(kvt[32 * g:32 * g + 32, :]),
                              jnp.concatenate(ph, axis=0).astype(BF16),
                              preferred_element_type=F32)
                scale = jnp.concatenate(
                    [jnp.broadcast_to(rden[0:1, :], (DH, T)),
                     jnp.broadcast_to(rden[1:2, :], (DH, T))], axis=0)
                ot[32 * g:32 * g + 32, :] = _pack(num * scale)
        a = lax.dot_general(_unpack(ot[...]), wo[...], TN_DIMS, preferred_element_type=F32)
        gt = jnp.tile(gate[tile(t), :], (1, D // 128))
        outb[tile(t), :] = (gt * a + (1.0 - gt) * xa[tile(res), :].astype(F32)).astype(BF16)
        out_cp(t, i).start()

    if UNROLL2:
        for i in range(NT):
            phase2(i)
    else:
        lax.fori_loop(0, NT, lambda i, c: phase2(i), None)
    _wait("wait_out", *[out_cp(i, i) for i in range(NT)])


@jax.jit
def pallas_gated_mix__linear_kernel_hedgehog__moe_arch_mod__prompt_kernel(
    A_x, A_wqkv, A_w_phi, A_wo, B_x, B_w_r, B_w_gate, B_w_up, B_w_down, gate_w,
):
    del B_x
    hbm = pl.BlockSpec(memory_space=pl.ANY)
    vmem = pl.BlockSpec(memory_space=pltpu.VMEM)
    out = pl.pallas_call(
        _kernel,
        out_shape=jax.ShapeDtypeStruct((S, D), BF16),
        in_specs=[hbm, hbm, hbm, hbm, vmem, hbm, hbm, hbm, vmem],
        out_specs=hbm,
        scratch_shapes=[
            pltpu.VMEM((S + T, D), BF16),
            pltpu.VMEM((D, 3 * D), BF16),
            pltpu.VMEM((D, DH), BF16),
            pltpu.VMEM((D, D), BF16),
            pltpu.VMEM((D, F), BF16),
            pltpu.VMEM((D, F), BF16),
            pltpu.VMEM((F, D), BF16),
            pltpu.VMEM((D // 2, D), U32),
            pltpu.VMEM((D // 2, D), U32),
            pltpu.VMEM((D // 2 + 8, D), U32),
            pltpu.VMEM((D // 2, T), U32),
            pltpu.VMEM((D, T), U32),
            pltpu.VMEM((D // 2, T), U32),
            pltpu.VMEM((D, 128), F32),
            pltpu.VMEM((D // 2, 128), U32),
            pltpu.VMEM((2 * D, 128), F32),
            pltpu.VMEM((S, 128), F32),
            pltpu.VMEM((8, S), F32),
            pltpu.VMEM((S, D), BF16),
            pltpu.VMEM((RC, T), F32),
            pltpu.SemaphoreType.DMA((NT + 1,)),
            pltpu.SemaphoreType.DMA((3 * NC,)),
            pltpu.SemaphoreType.DMA((5,)),
            pltpu.SemaphoreType.DMA((NT,)),
        ],
        compiler_params=pltpu.CompilerParams(vmem_limit_bytes=110 * 2**20),
    )(A_x.reshape(S, D), A_wqkv, A_w_phi.reshape(H * DH, DH), A_wo,
      B_w_r, B_w_gate, B_w_up, B_w_down, gate_w)
    return out.reshape(1, S, D)
```

```python
import functools

import jax
import jax.numpy as jnp
from jax import lax
from jax.experimental import pallas as pl
from jax.experimental.pallas import tpu as pltpu

S, D, H, DH, F = 2048, 1024, 32, 32, 3584
T = 512
NT = S // T
TH, KH = T // 2, D // 2
WR = KH // 2 + 8
NB = KH // 128
FC = F // NT
SCOPES = False
LOG2E = 1.4426950408889634
F32, BF16, U32 = jnp.float32, jnp.bfloat16, jnp.uint32
NT_DIMS = (((1,), (1,)), ((), ()))
TN_DIMS = (((0,), (0,)), ((), ()))


def _tree(op, xs):
    xs = list(xs)
    while len(xs) > 1:
        xs = [op(xs[i], xs[i + 1]) if i + 1 < len(xs) else xs[i]
              for i in range(0, len(xs), 2)]
    return xs[0]


def _allreduce(op, xs):
    r = _tree(op, xs)
    r = op(r, pltpu.roll(r, 4, 0))
    return op(r, pltpu.roll(r, 2, 0))


def _features(p):
    rows = [p[8 * i:8 * i + 8, :] for i in range(8)]
    mx = _allreduce(jnp.maximum, rows)
    mn = _allreduce(jnp.minimum, rows)
    ep = [jnp.exp2(r - mx) for r in rows]
    en = [jnp.exp2(mn - r) for r in rows]
    rp = 1.0 / _allreduce(jnp.add, ep)
    rn = 1.0 / _allreduce(jnp.add, en)
    return [e * rp for e in ep] + [e * rn for e in en]


def _pack(x):
    return pltpu.bitcast(x.astype(BF16), U32)


def _unpack(x):
    return pltpu.bitcast(x, BF16)


_LHS = [lambda a: a[0][0] + a[1][1], lambda a: a[1][0] + a[1][1], lambda a: a[0][0],
        lambda a: a[1][1], lambda a: a[0][0] + a[0][1], lambda a: a[1][0] - a[0][0],
        lambda a: a[0][1] - a[1][1]]
_RHS = [lambda b: b[0][0] + b[1][1], lambda b: b[0][0], lambda b: b[0][1] - b[1][1],
        lambda b: b[1][0] - b[0][0], lambda b: b[1][1], lambda b: b[0][0] + b[0][1],
        lambda b: b[1][0] + b[1][1]]


def _strassen(prod, emit, fill=()):
    fill = list(fill)

    def step(j):
        m = prod(j)
        if fill:
            fill.pop(0)()
        return m

    m3 = step(2)
    m5 = step(4)
    emit(0, 1, m3 + m5)
    s2 = m3 + step(5)
    m2 = step(1)
    s2 = s2 - m2
    m4 = step(3)
    emit(1, 0, m2 + m4)
    s1 = m4 - m5
    s1 = s1 + step(6)
    m1 = step(0)
    emit(0, 0, s1 + m1)
    emit(1, 1, s2 + m1)


def _strassen_b(prod, emit, fill=()):
    fill = list(fill)

    def step(j):
        m = prod(j)
        if fill:
            fill.pop(0)()
        return m

    m3 = step(2)
    m5 = step(4)
    emit(0, 1, m3 + m5)
    m2 = step(1)
    m4 = step(3)
    emit(1, 0, m2 + m4)
    m1 = step(0)
    s1 = m4 - m5 + m1
    s2 = m3 - m2 + m1
    emit(0, 0, s1 + step(6))
    emit(1, 1, s2 + step(5))


def _strassen_c(prod, emit, fill=()):
    fill = list(fill)

    def step(j):
        m = prod(j)
        if fill:
            fill.pop(0)()
        return m

    m3 = step(2)
    m5 = step(4)
    emit(0, 1, m3 + m5)
    s2 = m3 + step(5)
    m2 = step(1)
    s2 = s2 - m2
    m4 = step(3)
    emit(1, 0, m2 + m4)
    s1 = m4 - m5
    m1 = step(0)
    emit(1, 1, s2 + m1)
    s1 = s1 + m1
    emit(0, 0, s1 + step(6))


def _start(*cps):
    def step(i, carry):
        for n, cp in enumerate(cps):
            pl.when(i == n)(cp.start)
        return carry

    lax.fori_loop(0, len(cps), step, 0)


def _wait(name, *cps):
    if SCOPES:
        with jax.named_scope(name):
            for cp in cps:
                cp.wait()
    else:
        for cp in cps:
            cp.wait()


def _ds(start, size, mult=None):
    if isinstance(start, int):
        return pl.ds(start, size)
    return pl.ds(pl.multiple_of(start, mult or size), size)


def _kernel(xa_hbm, wqkv_hbm, wphi_hbm, wo_hbm, wr_ref, wg_hbm, wu_hbm,
            wd_hbm, gw_ref, out_hbm,
            xa, wqkv, wphi, wo, wg, wu, wd, wq_s, wk_s, wv_s, wo_s, xs, vt, phi, kvacc, kvt, zacc,
            gate, score, outb, xcol, yacc, sem_x, sem_w, sem_m, sem_o):
    def xa_cp(i):
        return pltpu.make_async_copy(xa_hbm.at[_ds(i * T, T)], xa.at[_ds(i * T, T)], sem_x.at[i])

    def w_cp(j):
        cols = pl.ds(j * D, D)
        return pltpu.make_async_copy(wqkv_hbm.at[:, cols], wqkv.at[:, cols], sem_w.at[j])

    phi_cp = pltpu.make_async_copy(wphi_hbm, wphi, sem_m.at[0])
    wo_cp = pltpu.make_async_copy(wo_hbm, wo, sem_m.at[1])
    ffn_cp = [pltpu.make_async_copy(wg_hbm, wg, sem_m.at[2]),
              pltpu.make_async_copy(wu_hbm, wu, sem_m.at[3]),
              pltpu.make_async_copy(wd_hbm, wd, sem_m.at[4])]

    def out_cp(t, r, c, slot):
        blk = (_ds(t * T + r * TH, TH), pl.ds(c * KH, KH))
        return pltpu.make_async_copy(outb.at[blk], out_hbm.at[blk], sem_o.at[slot * 4 + r * 2 + c])

    _start(phi_cp, w_cp(1), xa_cp(0), w_cp(2), xa_cp(1), w_cp(0), wo_cp,
           *[xa_cp(i) for i in range(2, NT)], *ffn_cp)

    er = lax.broadcasted_iota(jnp.int32, (128, DH), 0)
    ec = lax.broadcasted_iota(jnp.int32, (128, DH), 1)
    expand = jnp.where((er % 64) // 2 == ec, 1.0, 0.0).astype(BF16)
    pr = lax.broadcasted_iota(jnp.int32, (128, 128), 0)
    pc = lax.broadcasted_iota(jnp.int32, (128, 128), 1)
    diag = pc // DH == 2 * (pr // 64) + pr % 2
    kvacc[...] = jnp.zeros_like(kvacc)
    zacc[...] = jnp.zeros_like(zacc)
    xr = lax.broadcasted_iota(jnp.int32, (16, D), 0)
    extra = jnp.where(
        xr == 0, gw_ref[...].astype(F32).reshape(1, D),
        jnp.where(xr == 1, wr_ref[...].astype(F32).reshape(1, D), 0.0))
    zero = jnp.zeros((16, KH), F32)
    for j in range(7):
        wv_s[j * WR + KH // 2:(j + 1) * WR, :] = _pack(
            _LHS[j]([[extra[:, :KH], extra[:, KH:]], [zero, zero]]))

    def folded(j, g):
        pt = lax.dot_general(expand, wphi[_ds(g * 128, 128), :], NT_DIMS,
                             preferred_element_type=F32)
        pt = jnp.where(diag, pt, 0.0).astype(BF16)
        w = wqkv[:, _ds(j * D + g * 128, 128)]
        return lax.dot_general(pt, w, NT_DIMS, preferred_element_type=F32) * LOG2E

    def transposed(j, g):
        return wqkv[:, _ds(j * D + g * 128, 128)].T.astype(F32)

    def prep_w(rows_of, j, dst, b):
        r1, r2 = rows_of(j, b), rows_of(j, b + NB)
        quad = [[r1[:, :KH], r1[:, KH:]], [r2[:, :KH], r2[:, KH:]]]
        for n in range(7):
            dst[_ds(n * WR + b * 64, 64, 8), :] = _pack(_LHS[n](quad))

    def prep_wo(b, h):
        r1 = wo[_ds(b * 128 + h * 64, 64), :].astype(F32)
        r2 = wo[_ds(KH + b * 128 + h * 64, 64), :].astype(F32)
        quad = [[r1[:, :KH], r1[:, KH:]], [r2[:, :KH], r2[:, KH:]]]
        for n in range(7):
            wo_s[_ds(n * (KH // 2) + b * 64 + h * 32, 32), :] = _pack(_RHS[n](quad))

    def prep_x(i, slot, h):
        n = TH // 4
        x1 = xa[_ds(i * T + h * n, n), :].astype(F32)
        x2 = xa[_ds(i * T + TH + h * n, n), :].astype(F32)
        quad = [[x1[:, :KH], x2[:, :KH]], [x1[:, KH:], x2[:, KH:]]]
        for j in range(7):
            xs[_ds((slot * 7 + j) * (TH // 2) + h * n // 2, n // 2), :] = _pack(_RHS[j](quad))

    def project(w_s, i, more=0):
        def prod(n):
            return lax.dot_general(_unpack(w_s[n * WR:n * WR + (KH + more) // 2, :]),
                                   _unpack(xs[_ds((i * 7 + n) * (TH // 2), TH // 2), :]),
                                   NT_DIMS, preferred_element_type=F32)
        return prod

    def keys(i, fill=()):
        def emit(r, n, p):
            for q in range(KH // 64):
                g = r * KH // 64 + q
                ph = _features(p[64 * q:64 * q + 64, :])
                zs = [_tree(jnp.add, [a[:, 128 * l:128 * l + 128] for l in range(TH // 128)])
                      for a in ph]
                zacc[128 * g:128 * g + 128, :] += jnp.concatenate(zs, axis=0)
                phi[64 * g:64 * g + 64, n * TH:(n + 1) * TH] = _pack(jnp.concatenate(ph, axis=0))
        _strassen_b(project(wk_s, i), emit, fill)

    def values(i, fill=()):
        def kv(r):
            for g in range(r * KH // 64, (r + 1) * KH // 64):
                kvacc[64 * g:64 * g + 64, :] += lax.dot_general(
                    _unpack(vt[32 * g:32 * g + 32, :]), _unpack(phi[64 * g:64 * g + 64, :]),
                    NT_DIMS, preferred_element_type=F32)

        def emit(r, n, v):
            vt[r * KH // 2:(r + 1) * KH // 2, n * TH:(n + 1) * TH] = _pack(v[:KH, :])
            if r == 0:
                gr = v[KH:KH + 8, :]
                score[:, _ds(i * T + n * TH, TH)] = gr
                gt = jax.nn.sigmoid(gr)
                gate[_ds(i * T + n * TH, TH), :] = jnp.broadcast_to(gt[0:1, :], (128, TH)).T
            if r == 1 and n == 1:
                kv(0)
                kv(1)
        _strassen_b(project(wv_s, i, 16), emit, fill)

    def bind(f, *a):
        return lambda: f(*a)

    _wait("wait_wk", phi_cp, w_cp(1))
    for b in range(NB):
        prep_w(folded, 1, wk_s, b)
    _wait("wait_x", xa_cp(0))
    for h in range(4):
        prep_x(0, 0, h)
    keys(0)
    _wait("wait_wv", w_cp(2), xa_cp(1))
    for b in range(NB):
        prep_w(transposed, 2, wv_s, b)
    values(0, [bind(prep_x, 1, 1, h) for h in range(4)])
    _wait("wait_wq", w_cp(0), wo_cp)

    def phase1(i, carry):
        pl.when(i + 1 < NT)(lambda: _wait("wait_x", xa_cp(i + 1)))
        keys(i, [bind(prep_w, folded, 0, wq_s, i - 1)])
        nxt = jnp.minimum(i + 1, NT - 1)
        values(i, [bind(prep_x, nxt, i + 1, h) for h in range(4)]
               + [bind(prep_wo, i - 1, h) for h in range(2)])
        return carry

    lax.fori_loop(1, NT, phase1, 0)

    r = score[1:2, :].astype(BF16).astype(F32)
    best = jnp.max(r, axis=-1, keepdims=True)
    tok = lax.broadcasted_iota(jnp.int32, (1, S), 1)
    idx = jnp.min(jnp.where(r == best, tok, S - 1))
    last = idx // T
    prep_w(folded, 0, wq_s, NB - 1)
    for h in range(2):
        prep_wo(NB - 1, h)
    kr = lax.broadcasted_iota(jnp.int32, (D, 128), 0)
    kc = lax.broadcasted_iota(jnp.int32, (D, 128), 1)
    kvt[...] = _pack(jnp.where((kr // DH) % 2 == kc % 2, kvacc[...], 0.0))
    zacc[...] = jnp.broadcast_to(jnp.sum(zacc[...], axis=-1, keepdims=True), zacc.shape)

    slab = pl.ds(pl.multiple_of((idx // 16) * 16, 16), 16)
    sel = lax.broadcasted_iota(jnp.int32, (16, D), 0) == idx % 16
    xrow = jnp.sum(jnp.where(sel, xa[slab, :].astype(F32), 0.0), axis=0, keepdims=True)
    for k in range(D // 128):
        xcol[128 * k:128 * k + 128, :] = jnp.broadcast_to(
            xrow[:, 128 * k:128 * k + 128], (128, 128)).T
    yacc[...] = jnp.zeros_like(yacc)
    _wait("wait_ffn", *ffn_cp)

    def fold8(x):
        return jnp.sum(x.reshape(x.shape[0] // 8, 8, 128), axis=0)

    def ffn_steps(i):
        st = {}

        def up(j, k, pin):
            f = _ds(i * FC + j * 128, 128)
            rows = slice(64 * k, 64 * k + 64)
            xc = xcol[rows, :]
            a = fold8(wg[rows, f].astype(F32) * xc)
            u = fold8(wu[rows, f].astype(F32) * xc)
            if k > 0:
                a, u = pin(st["a"]) + a, pin(st["u"]) + u
            st["a"], st["u"] = a, u
            if k == D // 64 - 1:
                a = jnp.sum(a, axis=0, keepdims=True)
                u = jnp.sum(u, axis=0, keepdims=True)
                st["h"] = jnp.broadcast_to(a * jax.nn.sigmoid(a) * u, (128, 128)).T

        def down(j, n, pin):
            cols = slice(128 * n, 128 * n + 128)
            w = wd[_ds(i * FC + j * 128, 128), cols].astype(F32)
            yacc[:, cols] = pin(yacc[:, cols]) + fold8(w * st["h"])

        steps = []
        for j in range(FC // 128):
            steps += [functools.partial(up, j, k) for k in range(D // 64)]
            steps += [functools.partial(down, j, n) for n in range(D // 128)]
        return steps

    def phase2(i, carry):
        t = (last + i) % NT
        never = jnp.full((8, 128), i, jnp.int32) < 0
        steps = ffn_steps(i)
        per = len(steps) // 7

        def shadowed(m):
            rows, cols = m.shape
            for s in range(per):
                p = s * (rows // 8) * (cols // 128) // per
                r, c = 8 * (p % (rows // 8)), 128 * (p // (rows // 8))
                slab_m = m[r:r + 8, c:c + 128]
                steps.pop(0)(lambda v: jnp.where(never, slab_m, v))
            return m
        o = [[None, None], [None, None]]

        def emit_q(r, n, p):
            parts = []
            for q in range(KH // 64):
                g = r * KH // 64 + q
                ph = _features(p[64 * q:64 * q + 64, :])
                zb = zacc[128 * g:128 * g + 128, :]
                dn = [a * jnp.tile(zb[8 * k:8 * k + 8, :], (1, TH // 128))
                      for k, a in enumerate(ph)]
                rden = 1.0 / (_allreduce(jnp.add, dn) + 1e-6)
                num = jnp.dot(_unpack(kvt[32 * g:32 * g + 32, :]),
                              jnp.concatenate(ph, axis=0).astype(BF16),
                              preferred_element_type=F32)
                scale = jnp.concatenate(
                    [jnp.broadcast_to(rden[0:1, :], (DH, TH)),
                     jnp.broadcast_to(rden[1:2, :], (DH, TH))], axis=0)
                parts.append(num * scale)
            o[n][r] = jnp.concatenate(parts, axis=0)
        _strassen_b(project(wq_s, t), emit_q)

        def prod_o(n):
            return lax.dot_general(_LHS[n](o).astype(BF16),
                                   _unpack(wo_s[n * (KH // 2):(n + 1) * (KH // 2), :]),
                                   TN_DIMS, preferred_element_type=F32)

        def emit_o(n, c, a):
            gt = jnp.tile(gate[_ds(t * T + n * TH, TH), :], (1, KH // 128))
            b = xa[_ds(t * T + n * TH, TH), c * KH:(c + 1) * KH].astype(F32)
            outb[_ds(t * T + n * TH, TH), c * KH:(c + 1) * KH] = (gt * a + (1.0 - gt) * b).astype(BF16)
            out_cp(t, n, c, i).start()
        _strassen_c(lambda n: shadowed(prod_o(n)), emit_o)
        return carry

    lax.fori_loop(0, NT, phase2, 0)
    _wait("wait_out", *[out_cp(0, r, c, 0) for r in range(2) for c in range(2)])
    y = jnp.sum(yacc[...], axis=0, keepdims=True) * jax.nn.sigmoid(best)
    xsl = xa[slab, :].astype(F32)
    upd = (xsl + y).astype(BF16).astype(F32) - xsl
    gt = jnp.tile(gate[slab, :], (1, D // 128))
    old = outb[slab, :].astype(F32)
    outb[slab, :] = jnp.where(sel, old + (1.0 - gt) * upd, old).astype(BF16)
    fix_cp = pltpu.make_async_copy(outb.at[slab], out_hbm.at[slab], sem_x.at[NT])
    fix_cp.start()
    _wait("wait_out", fix_cp,
          *[out_cp(i, r, c, i) for i in range(1, NT) for r in range(2) for c in range(2)])


@jax.jit
def pallas_gated_mix__linear_kernel_hedgehog__moe_arch_mod__prompt_kernel(
    A_x, A_wqkv, A_w_phi, A_wo, B_x, B_w_r, B_w_gate, B_w_up, B_w_down, gate_w,
):
    del B_x
    hbm = pl.BlockSpec(memory_space=pl.ANY)
    vmem = pl.BlockSpec(memory_space=pltpu.VMEM)
    out = pl.pallas_call(
        _kernel,
        out_shape=jax.ShapeDtypeStruct((S, D), BF16),
        in_specs=[hbm, hbm, hbm, hbm, vmem, hbm, hbm, hbm, vmem],
        out_specs=hbm,
        scratch_shapes=[
            pltpu.VMEM((S, D), BF16),
            pltpu.VMEM((D, 3 * D), BF16),
            pltpu.VMEM((D, DH), BF16),
            pltpu.VMEM((D, D), BF16),
            pltpu.VMEM((D, F), BF16),
            pltpu.VMEM((D, F), BF16),
            pltpu.VMEM((F, D), BF16),
            pltpu.VMEM((7 * WR, KH), U32),
            pltpu.VMEM((7 * WR, KH), U32),
            pltpu.VMEM((7 * WR, KH), U32),
            pltpu.VMEM((7 * KH // 2, KH), U32),
            pltpu.VMEM(((NT + 1) * 7 * TH // 2, KH), U32),
            pltpu.VMEM((D // 2, T), U32),
            pltpu.VMEM((D, T), U32),
            pltpu.VMEM((D, 128), F32),
            pltpu.VMEM((D // 2, 128), U32),
            pltpu.VMEM((2 * D, 128), F32),
            pltpu.VMEM((S, 128), F32),
            pltpu.VMEM((8, S), F32),
            pltpu.VMEM((S, D), BF16),
            pltpu.VMEM((D, 128), F32),
            pltpu.VMEM((8, D), F32),
            pltpu.SemaphoreType.DMA((NT + 1,)),
            pltpu.SemaphoreType.DMA((3,)),
            pltpu.SemaphoreType.DMA((5,)),
            pltpu.SemaphoreType.DMA((4 * NT,)),
        ],
        compiler_params=pltpu.CompilerParams(vmem_limit_bytes=110 * 2**20),
    )(A_x.reshape(S, D), A_wqkv, A_w_phi.reshape(H * DH, DH), A_wo,
      B_w_r, B_w_gate, B_w_up, B_w_down, gate_w)
    return out.reshape(1, S, D)
```

```python
import functools

import jax
import jax.numpy as jnp
from jax import lax
from jax.experimental import pallas as pl
from jax.experimental.pallas import tpu as pltpu

S, D, H, DH, F = 2048, 1024, 32, 32, 3584
T = 512
NT = S // T
TH, KH = T // 2, D // 2
WR = KH // 2 + 8
NB = KH // 128
FC = F // NT
SCOPES = False
DEFER_NUM = True
LOG2E = 1.4426950408889634
F32, BF16, U32 = jnp.float32, jnp.bfloat16, jnp.uint32
NT_DIMS = (((1,), (1,)), ((), ()))
TN_DIMS = (((0,), (0,)), ((), ()))
bind = functools.partial


def _tree(op, xs):
    xs = list(xs)
    while len(xs) > 1:
        xs = [op(xs[i], xs[i + 1]) if i + 1 < len(xs) else xs[i]
              for i in range(0, len(xs), 2)]
    return xs[0]


def _allreduce(op, xs):
    r = _tree(op, xs)
    r = op(r, pltpu.roll(r, 4, 0))
    return op(r, pltpu.roll(r, 2, 0))


def _features(p):
    rows = [p[8 * i:8 * i + 8, :] for i in range(8)]
    mx = _allreduce(jnp.maximum, rows)
    mn = _allreduce(jnp.minimum, rows)
    ep = [jnp.exp2(r - mx) for r in rows]
    en = [jnp.exp2(mn - r) for r in rows]
    rp = 1.0 / _allreduce(jnp.add, ep)
    rn = 1.0 / _allreduce(jnp.add, en)
    return [e * rp for e in ep] + [e * rn for e in en]


def _pack(x):
    return pltpu.bitcast(x.astype(BF16), U32)


def _unpack(x):
    return pltpu.bitcast(x, BF16)


_LHS = [lambda a: a[0][0] + a[1][1], lambda a: a[1][0] + a[1][1], lambda a: a[0][0],
        lambda a: a[1][1], lambda a: a[0][0] + a[0][1], lambda a: a[1][0] - a[0][0],
        lambda a: a[0][1] - a[1][1]]
_RHS = [lambda b: b[0][0] + b[1][1], lambda b: b[0][0], lambda b: b[0][1] - b[1][1],
        lambda b: b[1][0] - b[0][0], lambda b: b[1][1], lambda b: b[0][0] + b[0][1],
        lambda b: b[1][0] + b[1][1]]


def _strassen(prod, emit):
    m3 = prod(2)
    m5 = prod(4)
    emit(0, 1, m3 + m5)
    m2 = prod(1)
    m4 = prod(3)
    emit(1, 0, m2 + m4)
    m1 = prod(0)
    s1 = m4 - m5 + m1
    s2 = m3 - m2 + m1
    emit(0, 0, s1 + prod(6))
    emit(1, 1, s2 + prod(5))


def _strassen_late(prod, emit):
    m3 = prod(2)
    m5 = prod(4)
    emit(0, 1, m3 + m5)
    s2 = m3 + prod(5)
    m2 = prod(1)
    s2 = s2 - m2
    m4 = prod(3)
    emit(1, 0, m2 + m4)
    s1 = m4 - m5
    m1 = prod(0)
    emit(1, 1, s2 + m1)
    s1 = s1 + m1
    emit(0, 0, s1 + prod(6))


def _shadow(m, steps, never, lo=0.0):
    rows, cols = m.shape[0] // 8, m.shape[1] // 128
    for s, step in enumerate(steps):
        p = int(rows * cols * (lo + (1.0 - lo) * s / len(steps)))
        r, c = 8 * (p % rows), 128 * (p // rows)
        slab = m[r:r + 8, c:c + 128]

        def pin(v, slab=slab):
            reps = (v.shape[0] // 8, v.shape[1] // 128)
            other = slab if v.dtype == F32 else pltpu.bitcast(slab, v.dtype)
            return jnp.where(jnp.tile(never, reps) != 0, jnp.tile(other, reps), v)

        step(pin)
    return m


def _split(steps, shares):
    out, done, total = [], 0, 0
    for s in shares:
        total += s
        end = len(steps) * total // sum(shares)
        out.append(steps[done:end])
        done = end
    return out


def _start(*cps):
    def step(i, carry):
        for n, cp in enumerate(cps):
            pl.when(i == n)(cp.start)
        return carry

    lax.fori_loop(0, len(cps), step, 0)


def _wait(name, *cps):
    if SCOPES:
        with jax.named_scope(name):
            for cp in cps:
                cp.wait()
    else:
        for cp in cps:
            cp.wait()


def _ds(start, size, mult=None):
    if isinstance(start, int):
        return pl.ds(start, size)
    return pl.ds(pl.multiple_of(start, mult or size), size)


def _kernel(xa_hbm, wqkv_hbm, wphi_hbm, wo_hbm, wr_ref, wg_hbm, wu_hbm,
            wd_hbm, gw_ref, out_hbm,
            xa, wqkv, wphi, wo, wg, wu, wd, wq_s, wk_s, wv_s, wo_s, xs, vt, phi, kvacc, kvt, zacc,
            zb, gate, score, outb, xcol, sem_x, sem_w, sem_m, sem_o):
    def xa_cp(i):
        return pltpu.make_async_copy(xa_hbm.at[_ds(i * T, T)], xa.at[_ds(i * T, T)], sem_x.at[i])

    def w_cp(start, size, sem):
        cols = pl.ds(start, size)
        return pltpu.make_async_copy(wqkv_hbm.at[:, cols], wqkv.at[:, cols], sem_w.at[sem])

    def wo_cp(start, size, sem):
        rows = pl.ds(start, size)
        return pltpu.make_async_copy(wo_hbm.at[rows], wo.at[rows], sem_w.at[sem])

    wk_cp = [w_cp(D, KH, 0), w_cp(D + KH, KH, 1)]
    wv_cp = w_cp(2 * D, D, 2)
    early_cp = [w_cp(0, 128, 3), w_cp(KH, 128, 4), wo_cp(0, 128, 5), wo_cp(KH, 128, 6)]
    late_cp = [w_cp(128, KH - 128, 7), w_cp(KH + 128, KH - 128, 8),
               wo_cp(128, KH - 128, 9), wo_cp(KH + 128, KH - 128, 10)]
    phi_cp = pltpu.make_async_copy(wphi_hbm, wphi, sem_m.at[0])
    ffn_cp = [pltpu.make_async_copy(wg_hbm, wg, sem_m.at[1]),
              pltpu.make_async_copy(wu_hbm, wu, sem_m.at[2]),
              pltpu.make_async_copy(wd_hbm, wd, sem_m.at[3])]

    def out_cp(t, r, c, slot):
        blk = (_ds(t * T + r * TH, TH), pl.ds(c * KH, KH))
        return pltpu.make_async_copy(outb.at[blk], out_hbm.at[blk], sem_o.at[slot * 4 + r * 2 + c])

    zb[0:8, :] = jnp.zeros((8, 128), F32)
    _start(phi_cp, wk_cp[0], xa_cp(0), wk_cp[1], wv_cp, xa_cp(1), *early_cp, *late_cp,
           *[xa_cp(i) for i in range(2, NT)], *ffn_cp)

    er = lax.broadcasted_iota(jnp.int32, (128, DH), 0)
    ec = lax.broadcasted_iota(jnp.int32, (128, DH), 1)
    expand = jnp.where((er % 64) // 2 == ec, 1.0, 0.0).astype(BF16)
    pr = lax.broadcasted_iota(jnp.int32, (128, 128), 0)
    pc = lax.broadcasted_iota(jnp.int32, (128, 128), 1)
    diag = pc // DH == 2 * (pr // 64) + pr % 2
    kr = lax.broadcasted_iota(jnp.int32, (64, 128), 0)
    kc = lax.broadcasted_iota(jnp.int32, (64, 128), 1)
    same_head = kr // DH == kc % 2
    kvacc[...] = jnp.zeros_like(kvacc)
    zacc[...] = jnp.zeros_like(zacc)
    xr = lax.broadcasted_iota(jnp.int32, (16, D), 0)
    extra = jnp.where(
        xr == 0, gw_ref[...].astype(F32).reshape(1, D),
        jnp.where(xr == 1, wr_ref[...].astype(F32).reshape(1, D), 0.0))
    zero = jnp.zeros((16, KH), F32)
    for j in range(7):
        wv_s[j * WR + KH // 2:(j + 1) * WR, :] = _pack(
            _LHS[j]([[extra[:, :KH], extra[:, KH:]], [zero, zero]]))

    def folded(j, g):
        pt = lax.dot_general(expand, wphi[_ds(g * 128, 128), :], NT_DIMS,
                             preferred_element_type=F32)
        pt = jnp.where(diag, pt, 0.0).astype(BF16)
        w = wqkv[:, _ds(j * D + g * 128, 128)]
        return lax.dot_general(pt, w, NT_DIMS, preferred_element_type=F32) * LOG2E

    def transposed(j, g):
        return wqkv[:, _ds(j * D + g * 128, 128)].T

    def keep(v):
        return v

    def w_terms(r1, r2, dst, b, terms=range(7)):
        def step(h, pin):
            rows = slice(16 * h, 16 * h + 16)
            a = r1[rows, :].astype(F32)
            top = [pin(a[:, :KH]), a[:, KH:]]
            low = None
            if r2 is not None:
                a = r2[rows, :].astype(F32)
                low = [a[:, :KH], pin(a[:, KH:])]
            for n in terms:
                dst[_ds(n * WR + b * 64 + h * 8, 8), :] = _pack(_LHS[n]([top, low]))
        return [bind(step, h) for h in range(8)]

    def wo_terms(b):
        def step(h, pin):
            r1 = wo[_ds(b * 128 + h * 16, 16), :].astype(F32)
            r2 = wo[_ds(KH + b * 128 + h * 16, 16), :].astype(F32)
            quad = [[pin(r1[:, :KH]), r1[:, KH:]], [r2[:, :KH], pin(r2[:, KH:])]]
            for n in range(7):
                wo_s[_ds(n * (KH // 2) + b * 64 + h * 8, 8), :] = _pack(_RHS[n](quad))
        return [bind(step, h) for h in range(8)]

    def x_terms(i, slot, terms=range(7)):
        def step(h, pin):
            x1 = xa[_ds(i * T + h * 16, 16), :].astype(F32)
            x2 = xa[_ds(i * T + TH + h * 16, 16), :].astype(F32)
            quad = [[pin(x1[:, :KH]), x2[:, :KH]], [x1[:, KH:], pin(x2[:, KH:])]]
            for n in terms:
                xs[_ds((slot * 7 + n) * (TH // 2) + h * 8, 8), :] = _pack(_RHS[n](quad))
        return [bind(step, h) for h in range(TH // 16)]

    def z_total():
        def step(g, pin):
            rows = slice(128 * g, 128 * g + 128)
            z = jnp.sum(pin(zacc[rows, :]), axis=-1, keepdims=True)
            zb[rows, :] = jnp.broadcast_to(z, (128, 128))
        return [bind(step, g) for g in range(H // 2)]

    def project(w_s, i, n, more=0):
        return lax.dot_general(_unpack(w_s[n * WR:n * WR + (KH + more) // 2, :]),
                               _unpack(xs[_ds((i * 7 + n) * (TH // 2), TH // 2), :]),
                               NT_DIMS, preferred_element_type=F32)

    def staged(f, plan, never):
        plan = list(plan)

        def prod(n):
            steps = plan.pop(0)()
            return _shadow(f(n), steps, never)
        return prod

    def keys(i, plan, never):
        def emit(r, n, p):
            for q in range(KH // 64):
                g = r * KH // 64 + q
                ph = _features(p[64 * q:64 * q + 64, :])
                zs = [_tree(jnp.add, [a[:, 128 * l:128 * l + 128] for l in range(TH // 128)])
                      for a in ph]
                zacc[128 * g:128 * g + 128, :] += jnp.concatenate(zs, axis=0)
                phi[64 * g:64 * g + 64, n * TH:(n + 1) * TH] = _pack(jnp.concatenate(ph, axis=0))
        _strassen(staged(bind(project, wk_s, i), plan, never), emit)

    def values(i, plan, never):
        def emit(r, n, v):
            vt[r * KH // 2:(r + 1) * KH // 2, n * TH:(n + 1) * TH] = _pack(v[:KH, :])
            if r == 0:
                gr = v[KH:KH + 8, :]
                score[:, _ds(i * T + n * TH, TH)] = gr
                gt = jax.nn.sigmoid(gr)
                gate[_ds(i * T + n * TH, TH), :] = jnp.broadcast_to(gt[0:1, :], (128, TH)).T
        _strassen(staged(bind(project, wv_s, i, more=16), plan, never), emit)
        for g in range(H // 2):
            acc = kvacc[64 * g:64 * g + 64, :] + lax.dot_general(
                _unpack(vt[32 * g:32 * g + 32, :]), _unpack(phi[64 * g:64 * g + 64, :]),
                NT_DIMS, preferred_element_type=F32)
            kvacc[64 * g:64 * g + 64, :] = acc
            kvt[32 * g:32 * g + 32, :] = _pack(jnp.where(same_head, acc, 0.0))

    def q_terms(b):
        return w_terms(folded(0, b), folded(0, b + NB), wq_s, b)

    def fixed(steps):
        return lambda: steps

    never = pltpu.bitcast(zb[0:8, :], jnp.int32)
    _wait("wait_wk", phi_cp, wk_cp[0])
    top = [folded(1, b) for b in range(NB)]
    for b in range(NB):
        for step in w_terms(top[b], None, wk_s, b, (2, 4)):
            step(keep)
    _wait("wait_x", xa_cp(0))
    for step in x_terms(0, 0, (2, 4)):
        step(keep)
    x0 = _split(x_terms(0, 0, (0, 1, 3, 5, 6)), (1, 1))

    def rest_of_wk():
        _wait("wait_wk", wk_cp[1])
        for b in range(NB):
            for step in w_terms(top[b], folded(1, b + NB), wk_s, b, (0, 1, 3, 5, 6)):
                step(keep)
        return []

    wv = []

    def top_of_wv():
        _wait("wait_wv", wv_cp)
        steps = []
        for b in range(NB):
            steps += w_terms(transposed(2, b), None, wv_s, b, (2, 4))
        wv.extend(_split(steps, (1, 1)))
        steps = []
        for b in range(NB):
            steps += w_terms(transposed(2, b), transposed(2, b + NB), wv_s, b, (0, 1, 3, 5, 6))
        wv.extend(_split(steps, (1, 2, 2)))
        return wv.pop(0)

    nxt = bind(wv.pop, 0)
    keys(0, [fixed(x0[0]), fixed(x0[1]), rest_of_wk, fixed([]), top_of_wv, nxt, nxt], never)
    late = []

    def first_blocks():
        _wait("wait_wq", xa_cp(1), *early_cp)
        late.extend(_split(x_terms(1, 1) + wo_terms(0) + q_terms(0), (1, 1, 1)))
        return late.pop(0)

    values(0, [nxt, nxt, fixed([]), fixed([]), first_blocks, bind(late.pop, 0), bind(late.pop, 0)],
           never)
    _wait("wait_wq", *late_cp)

    def phase1(i, carry):
        never = jnp.where(jnp.full((8, 128), i, jnp.int32) < 0, 1, 0)
        pl.when(i + 1 < NT)(lambda: _wait("wait_x", xa_cp(i + 1)))
        w = _split(q_terms(i) + wo_terms(i), (2, 1, 1))
        keys(i, [fixed(w[0]), fixed([]), fixed(w[1]), fixed([]), fixed(w[2]), fixed([]), fixed([])],
             never)
        x = _split(x_terms(jnp.minimum(i + 1, NT - 1), i + 1), (1, 1, 1, 1))
        z = _split(z_total(), (1, 1, 1))
        values(i, [fixed(s) for s in x + z], never)
        return carry

    lax.fori_loop(1, NT, phase1, 0)

    r = score[1:2, :].astype(BF16).astype(F32)
    best = jnp.max(r, axis=-1, keepdims=True)
    tok = lax.broadcasted_iota(jnp.int32, (1, S), 1)
    idx = jnp.min(jnp.where(r == best, tok, S - 1))
    first = idx // T
    slab = pl.ds(pl.multiple_of((idx // 16) * 16, 16), 16)
    sel = lax.broadcasted_iota(jnp.int32, (16, D), 0) == idx % 16
    _wait("wait_ffn", *ffn_cp)

    def x_column():
        def step(k, pin):
            cols = slice(128 * k, 128 * k + 128)
            row = jnp.where(sel[:, cols], pin(xa[slab, cols].astype(F32)), 0.0)
            row = jnp.sum(row, axis=0, keepdims=True)
            xcol[cols, :] = jnp.broadcast_to(row, (128, 128)).T
        return [bind(step, k) for k in range(D // 128)]

    def fold8(x):
        return jnp.sum(x.reshape(x.shape[0] // 8, 8, 128), axis=0)

    def ffn_steps(i, y):
        st = {}

        def up(j, k, pin):
            f = _ds(i * FC + j * 128, 128)
            rows = slice(64 * k, 64 * k + 64)
            xc = xcol[rows, :]
            a = fold8(wg[rows, f].astype(F32) * xc)
            u = fold8(wu[rows, f].astype(F32) * xc)
            if k > 0:
                a, u = pin(st["a"]) + a, pin(st["u"]) + u
            st["a"], st["u"] = a, u
            if k == D // 64 - 1:
                a = jnp.sum(a, axis=0, keepdims=True)
                u = jnp.sum(u, axis=0, keepdims=True)
                st["h"] = jnp.broadcast_to(a * jax.nn.sigmoid(a) * u, (128, 128)).T

        def down(j, n, pin):
            w = wd[_ds(i * FC + j * 128, 128), 128 * n:128 * n + 128].astype(F32)
            y[n] = pin(y[n]) + fold8(w * st["h"])

        steps = []
        for j in range(FC // 128):
            steps += [bind(up, j, k) for k in range(D // 64)]
            steps += [bind(down, j, n) for n in range(D // 128)]
        return steps

    def phase2(i, y):
        y = list(y)
        t = (first + i) % NT
        never = jnp.where(jnp.full((8, 128), i, jnp.int32) < 0, 1, 0)
        o = [[[], []], [[], []]]
        todo = []

        def emit_q(r, n, p):
            def attend(g, ph, rden, pin):
                num = jnp.dot(_unpack(pin(kvt[32 * g:32 * g + 32, :])), ph,
                              preferred_element_type=F32)
                scale = jnp.concatenate(
                    [jnp.broadcast_to(rden[0:1, :], (DH, TH)),
                     jnp.broadcast_to(rden[1:2, :], (DH, TH))], axis=0)
                o[n][r].append(num * scale)

            for q in range(KH // 64):
                g = r * KH // 64 + q
                ph = _features(p[64 * q:64 * q + 64, :])
                z = zb[128 * g:128 * g + 128, :]
                dn = [a * jnp.tile(z[8 * k:8 * k + 8, :], (1, TH // 128))
                      for k, a in enumerate(ph)]
                rden = 1.0 / (_allreduce(jnp.add, dn) + 1e-6)
                todo.append(bind(attend, g, jnp.concatenate(ph, axis=0).astype(BF16), rden))
                if not DEFER_NUM:
                    todo.pop()(keep)

        def pending():
            steps = list(todo)
            todo.clear()
            return steps

        def prod_q(n):
            steps = pending()
            return _shadow(project(wq_s, t, n), steps, never, 0.3)

        col = _split(x_column(), (1, 1))
        _strassen(staged(prod_q, [fixed(col[0]), fixed(col[1])] + [fixed([])] * 5, never), emit_q)

        class Quad:
            def __init__(self, n):
                self.n = n

            def __getitem__(self, r):
                return jnp.concatenate(o[self.n][r], axis=0)

        def prod_o(n):
            steps = pending()
            m = lax.dot_general(_LHS[n]([Quad(0), Quad(1)]).astype(BF16),
                                _unpack(wo_s[n * (KH // 2):(n + 1) * (KH // 2), :]),
                                TN_DIMS, preferred_element_type=F32)
            return _shadow(m, steps, never, 0.3)

        def emit_o(n, c, a):
            gt = jnp.tile(gate[_ds(t * T + n * TH, TH), :], (1, KH // 128))
            b = xa[_ds(t * T + n * TH, TH), c * KH:(c + 1) * KH].astype(F32)
            outb[_ds(t * T + n * TH, TH), c * KH:(c + 1) * KH] = (
                gt * a + (1.0 - gt) * b).astype(BF16)
            out_cp(t, n, c, i).start()

        ffn = _split(ffn_steps(i, y), (0, 1, 1, 1, 1, 1, 1))
        _strassen_late(staged(prod_o, [fixed(s) for s in ffn], never), emit_o)
        return tuple(y)

    y = lax.fori_loop(0, NT, phase2, (jnp.zeros((8, 128), F32),) * (D // 128))

    _wait("wait_out", *[out_cp(0, r, c, 0) for r in range(2) for c in range(2)])
    y = jnp.sum(jnp.concatenate(y, axis=1), axis=0, keepdims=True) * jax.nn.sigmoid(best)
    xsl = xa[slab, :].astype(F32)
    upd = (xsl + y).astype(BF16).astype(F32) - xsl
    gt = jnp.tile(gate[slab, :], (1, D // 128))
    old = outb[slab, :].astype(F32)
    outb[slab, :] = jnp.where(sel, old + (1.0 - gt) * upd, old).astype(BF16)
    fix_cp = pltpu.make_async_copy(outb.at[slab], out_hbm.at[slab], sem_x.at[NT])
    fix_cp.start()
    _wait("wait_out", fix_cp,
          *[out_cp(i, r, c, i) for i in range(1, NT) for r in range(2) for c in range(2)])


@jax.jit
def pallas_gated_mix__linear_kernel_hedgehog__moe_arch_mod__prompt_kernel(
    A_x, A_wqkv, A_w_phi, A_wo, B_x, B_w_r, B_w_gate, B_w_up, B_w_down, gate_w,
):
    del B_x
    hbm = pl.BlockSpec(memory_space=pl.ANY)
    vmem = pl.BlockSpec(memory_space=pltpu.VMEM)
    out = pl.pallas_call(
        _kernel,
        out_shape=jax.ShapeDtypeStruct((S, D), BF16),
        in_specs=[hbm, hbm, hbm, hbm, vmem, hbm, hbm, hbm, vmem],
        out_specs=hbm,
        scratch_shapes=[
            pltpu.VMEM((S, D), BF16),
            pltpu.VMEM((D, 3 * D), BF16),
            pltpu.VMEM((D, DH), BF16),
            pltpu.VMEM((D, D), BF16),
            pltpu.VMEM((D, F), BF16),
            pltpu.VMEM((D, F), BF16),
            pltpu.VMEM((F, D), BF16),
            pltpu.VMEM((7 * WR, KH), U32),
            pltpu.VMEM((7 * WR, KH), U32),
            pltpu.VMEM((7 * WR, KH), U32),
            pltpu.VMEM((7 * KH // 2, KH), U32),
            pltpu.VMEM(((NT + 1) * 7 * TH // 2, KH), U32),
            pltpu.VMEM((D // 2, T), U32),
            pltpu.VMEM((D, T), U32),
            pltpu.VMEM((D, 128), F32),
            pltpu.VMEM((D // 2, 128), U32),
            pltpu.VMEM((2 * D, 128), F32),
            pltpu.VMEM((2 * D, 128), F32),
            pltpu.VMEM((S, 128), F32),
            pltpu.VMEM((8, S), F32),
            pltpu.VMEM((S, D), BF16),
            pltpu.VMEM((D, 128), F32),
            pltpu.SemaphoreType.DMA((NT + 1,)),
            pltpu.SemaphoreType.DMA((11,)),
            pltpu.SemaphoreType.DMA((4,)),
            pltpu.SemaphoreType.DMA((4 * NT,)),
        ],
        compiler_params=pltpu.CompilerParams(vmem_limit_bytes=110 * 2**20),
    )(A_x.reshape(S, D), A_wqkv, A_w_phi.reshape(H * DH, DH), A_wo,
      B_w_r, B_w_gate, B_w_up, B_w_down, gate_w)
    return out.reshape(1, S, D)
```

```python
import functools

import jax
import jax.numpy as jnp
from jax import lax
from jax.experimental import pallas as pl
from jax.experimental.pallas import tpu as pltpu

S, D, H, DH, F = 2048, 1024, 32, 32, 3584
T = 512
NT = S // T
TH, KH = T // 2, D // 2
WR = KH // 2 + 8
NB = KH // 128
FC = F // NT
SCOPES = False
BACK = True
FFN_SHARES = (3, 0, 2, 0, 2, 0, 0, 2, 3, 2, 2, 2, 1)
LOG2E = 1.4426950408889634
F32, BF16, U32 = jnp.float32, jnp.bfloat16, jnp.uint32
NT_DIMS = (((1,), (1,)), ((), ()))
TN_DIMS = (((0,), (0,)), ((), ()))
bind = functools.partial


def _tree(op, xs):
    xs = list(xs)
    while len(xs) > 1:
        xs = [op(xs[i], xs[i + 1]) if i + 1 < len(xs) else xs[i]
              for i in range(0, len(xs), 2)]
    return xs[0]


def _allreduce(op, xs):
    r = _tree(op, xs)
    r = op(r, pltpu.roll(r, 4, 0))
    return op(r, pltpu.roll(r, 2, 0))


def _features(p, pin):
    rows = [p[8 * i:8 * i + 8, :] for i in range(8)]
    rows[0] = pin(rows[0])
    mx = _allreduce(jnp.maximum, rows)
    mn = _allreduce(jnp.minimum, rows)
    ep = [jnp.exp2(r - mx) for r in rows]
    en = [jnp.exp2(mn - r) for r in rows]
    rp = 1.0 / _allreduce(jnp.add, ep)
    rn = 1.0 / _allreduce(jnp.add, en)
    return [e * rp for e in ep] + [e * rn for e in en]


def _pack(x):
    return pltpu.bitcast(x.astype(BF16), U32)


def _unpack(x):
    return pltpu.bitcast(x, BF16)


_LHS = [lambda a: a[0][0] + a[1][1], lambda a: a[1][0] + a[1][1], lambda a: a[0][0],
        lambda a: a[1][1], lambda a: a[0][0] + a[0][1], lambda a: a[1][0] - a[0][0],
        lambda a: a[0][1] - a[1][1]]
_RHS = [lambda b: b[0][0] + b[1][1], lambda b: b[0][0], lambda b: b[0][1] - b[1][1],
        lambda b: b[1][0] - b[0][0], lambda b: b[1][1], lambda b: b[0][0] + b[0][1],
        lambda b: b[1][0] + b[1][1]]


def _strassen(prod, emit):
    m3 = prod(2)
    m5 = prod(4)
    emit(0, 1, m3 + m5)
    m2 = prod(1)
    m4 = prod(3)
    emit(1, 0, m2 + m4)
    m1 = prod(0)
    s1 = m4 - m5 + m1
    s2 = m3 - m2 + m1
    emit(0, 0, s1 + prod(6))
    emit(1, 1, s2 + prod(5))


def _strassen_diag(prod, emit):
    m3 = prod(2)
    m4 = prod(3)
    m1 = prod(0)
    m5 = prod(4)
    emit(0, 1, m3 + m5)
    emit(0, 0, m1 + m4 - m5 + prod(6))
    m2 = prod(1)
    emit(1, 0, m2 + m4)
    emit(1, 1, m1 + m3 - m2 + prod(5))


def _shadow(m, steps, never, due):
    rows, cols = m.shape[0] // 8, m.shape[1] // 128
    for s, step in enumerate(steps):
        p = rows * cols * s // len(steps)
        r, c = 8 * (p % rows), 128 * (p // rows)
        slab = m[r:r + 8, c:c + 128]

        def pin(v, slab=slab):
            reps = (v.shape[0] // 8, v.shape[1] // 128)
            other = slab if v.dtype == F32 else pltpu.bitcast(slab, v.dtype)
            return jnp.where(jnp.tile(never, reps) != 0, jnp.tile(other, reps), v)

        token = step(pin)
        if token is not None:
            due.append(token)
    return m


def _after(w, due, never, axis):
    if not due:
        return w
    unit = (8, 128)[axis]
    parts = jnp.split(w, w.shape[axis] // unit, axis=axis)
    for s, token in enumerate(due):
        p = len(parts) * s // len(due)
        head = jnp.where(never != 0, pltpu.bitcast(token, U32), parts[p][:8, :128])
        if axis == 0:
            parts[p] = jnp.concatenate([head, parts[p][:, 128:]], axis=1)
        else:
            parts[p] = jnp.concatenate([head, parts[p][8:, :]], axis=0)
    due.clear()
    return jnp.concatenate(parts, axis=axis)


def _split(steps, shares):
    out, done, total = [], 0, 0
    for s in shares:
        total += s
        end = len(steps) * total // sum(shares)
        out.append(steps[done:end])
        done = end
    return out


def _start(*cps):
    def step(i, carry):
        for n, cp in enumerate(cps):
            pl.when(i == n)(cp.start)
        return carry

    lax.fori_loop(0, len(cps), step, 0)


def _wait(name, *cps):
    if SCOPES:
        with jax.named_scope(name):
            for cp in cps:
                cp.wait()
    else:
        for cp in cps:
            cp.wait()


def _ds(start, size, mult=None):
    if isinstance(start, int):
        return pl.ds(start, size)
    return pl.ds(pl.multiple_of(start, mult or size), size)


def _kernel(xa_hbm, wqkv_hbm, wphi_hbm, wo_hbm, wr_ref, wg_hbm, wu_hbm,
            wd_hbm, gw_ref, out_hbm,
            xa, wqkv, wphi, wo, wg, wu, wd, wq_s, wk_s, wv_s, wo_s, xs, pt, vt, phi, kvacc, kvt, zacc,
            zb, gate, score, outb, xcol, sem_x, sem_w, sem_m, sem_o):
    def xa_cp(i):
        return pltpu.make_async_copy(xa_hbm.at[_ds(i * T, T)], xa.at[_ds(i * T, T)], sem_x.at[i])

    def w_cp(start, size, sem):
        cols = _ds(start, size)
        return pltpu.make_async_copy(wqkv_hbm.at[:, cols], wqkv.at[:, cols], sem_w.at[sem])

    def x0_cp(h):
        rows = pl.ds(h * TH, TH)
        return pltpu.make_async_copy(xa_hbm.at[rows], xa.at[rows], sem_m.at[h])

    wk_cp = [w_cp(D, KH // 2, 0), w_cp(D + KH // 2, KH // 2, 1), w_cp(D + KH, KH, 2)]
    wv_cp = [w_cp(2 * D, KH, 3), w_cp(2 * D + KH, KH, 4)]
    wq_cp = w_cp(0, D, 5)
    phi_cp = pltpu.make_async_copy(wphi_hbm, wphi, sem_m.at[2])
    wo_cp = pltpu.make_async_copy(wo_hbm, wo, sem_m.at[3])
    ffn_cp = [pltpu.make_async_copy(wg_hbm, wg, sem_m.at[4]),
              pltpu.make_async_copy(wu_hbm, wu, sem_m.at[5]),
              pltpu.make_async_copy(wd_hbm, wd, sem_m.at[6])]

    def out_cp(t, r, c, slot):
        blk = (_ds(t * T + r * TH, TH), pl.ds(c * KH, KH))
        return pltpu.make_async_copy(outb.at[blk], out_hbm.at[blk], sem_o.at[slot * 4 + r * 2 + c])

    zb[0:8, :] = jnp.zeros((8, 128), F32)
    _start(phi_cp, x0_cp(1), wk_cp[0], wk_cp[1], x0_cp(0), wk_cp[2])

    er = lax.broadcasted_iota(jnp.int32, (128, DH), 0)
    ec = lax.broadcasted_iota(jnp.int32, (128, DH), 1)
    expand = jnp.where((er % 64) // 2 == ec, 1.0, 0.0).astype(BF16)
    pr = lax.broadcasted_iota(jnp.int32, (128, 128), 0)
    pc = lax.broadcasted_iota(jnp.int32, (128, 128), 1)
    diag = pc // DH == 2 * (pr // 64) + pr % 2
    kr = lax.broadcasted_iota(jnp.int32, (64, 128), 0)
    kc = lax.broadcasted_iota(jnp.int32, (64, 128), 1)
    same_head = kr // DH == kc % 2
    kvacc[...] = jnp.zeros_like(kvacc)
    zacc[...] = jnp.zeros_like(zacc)
    xr = lax.broadcasted_iota(jnp.int32, (16, D), 0)
    extra = jnp.where(
        xr == 0, gw_ref[...].astype(F32).reshape(1, D),
        jnp.where(xr == 1, wr_ref[...].astype(F32).reshape(1, D), 0.0))
    zero = jnp.zeros((16, KH), F32)
    for j in range(7):
        wv_s[j * WR + KH // 2:(j + 1) * WR, :] = _pack(
            _LHS[j]([[extra[:, :KH], extra[:, KH:]], [zero, zero]]))

    def folded(j, u, n):
        w = wqkv[:, _ds(j * D + (u // 2) * 128, 128)]
        return lax.dot_general(_unpack(pt[_ds(u * 32, n // 2), :]), w, NT_DIMS,
                               preferred_element_type=F32) * LOG2E

    def transposed(j, g):
        return wqkv[:, _ds(j * D + g * 128, 128)].T

    def keep(v):
        return v

    def w_terms(r1, r2, dst, u, terms=range(7)):
        dst = dst.at[_ds(u * 32, 6 * WR + r1.shape[0] // 2, 32)]

        def step(h, pin):
            rows = slice(16 * h, 16 * h + 16)
            a = r1[rows, :].astype(F32)
            top = [pin(a[:, :KH]), a[:, KH:]]
            low = None
            if r2 is not None:
                a = r2[rows, :].astype(F32)
                low = [a[:, :KH], pin(a[:, KH:])]
            for n in terms:
                dst[pl.ds(n * WR + h * 8, 8), :] = _pack(_LHS[n]([top, low]))
        return [bind(step, h) for h in range(r1.shape[0] // 16)]

    def wo_terms(u):
        src = wo.at[_ds(u * 64, KH + 64, 64)]
        dst = wo_s.at[_ds(u * 32, 6 * (KH // 2) + 32, 32)]

        def step(h, pin):
            r1 = src[pl.ds(KH + h * 16, 16), :].astype(F32)
            r2 = src[pl.ds(h * 16, 16), :].astype(F32)
            quad = [[pin(r1[:, :KH]), r1[:, KH:]], [r2[:, :KH], pin(r2[:, KH:])]]
            for n in range(7):
                dst[pl.ds(n * (KH // 2) + h * 8, 8), :] = _pack(_RHS[n](quad))
        return [bind(step, h) for h in range(4)]

    def x_terms(i, slot, terms=range(7)):
        src = xa.at[_ds(i * T, T)]
        dst = xs.at[_ds(slot * 7 * (TH // 2), 7 * (TH // 2))]

        def step(h, pin):
            x2 = src[pl.ds(TH + h * 16, 16), :].astype(F32)
            quad = [[None, x2[:, :KH]], [None, pin(x2[:, KH:])]]
            if set(terms) - {2, 4}:
                x1 = src[pl.ds(h * 16, 16), :].astype(F32)
                quad[0][0], quad[1][0] = pin(x1[:, :KH]), x1[:, KH:]
            for n in terms:
                dst[pl.ds(n * (TH // 2) + h * 8, 8), :] = _pack(_RHS[n](quad))
        return [bind(step, h) for h in range(TH // 16)]

    def z_total():
        def step(g, pin):
            rows = slice(128 * g, 128 * g + 128)
            z = jnp.sum(pin(zacc[rows, :]), axis=-1, keepdims=True)
            zb[rows, :] = jnp.broadcast_to(z, (128, 128))
        return [bind(step, g) for g in range(H // 2)]

    def project(w_s, i, n, due, never, more=0):
        w = _after(w_s[n * WR:n * WR + (KH + more) // 2, :], due, never, 0)
        return lax.dot_general(_unpack(w),
                               _unpack(xs[_ds((i * 7 + n) * (TH // 2), TH // 2), :]),
                               NT_DIMS, preferred_element_type=F32)

    def staged(f, plan, todo, never, due=None):
        plan = list(plan)
        due = [] if due is None else due

        def prod(n):
            steps = plan.pop(0)()
            follow = list(todo)
            todo.clear()
            return _shadow(_shadow(f(n, due, never), follow, never, due), steps, never, due)
        return prod

    def keys(i, plan, todo, never, ready=None):
        def step(g, n, p, pin):
            ph = _features(p, pin)
            zs = [_tree(jnp.add, [a[:, 128 * l:128 * l + 128] for l in range(TH // 128)])
                  for a in ph]
            zacc[128 * g:128 * g + 128, :] += jnp.concatenate(zs, axis=0)
            phi[64 * g:64 * g + 64, n * TH:(n + 1) * TH] = _pack(jnp.concatenate(ph, axis=0))

        def emit(r, n, p):
            todo.extend(bind(step, r * KH // 64 + q, n, p[64 * q:64 * q + 64, :])
                        for q in range(KH // 64))
        prod = staged(bind(project, wk_s, i), plan, todo, never)
        _strassen(lambda n: ready[n] if ready and n in ready else prod(n), emit)

    def values(i, plan, todo, never):
        def emit(r, n, v):
            vt[r * KH // 2:(r + 1) * KH // 2, n * TH:(n + 1) * TH] = _pack(v[:KH, :])
            if r == 0:
                gr = v[KH:KH + 8, :]
                score[:, _ds(i * T + n * TH, TH)] = gr
                gt = jax.nn.sigmoid(gr)
                gate[_ds(i * T + n * TH, TH), :] = jnp.broadcast_to(gt[0:1, :], (128, TH)).T
        _strassen(staged(bind(project, wv_s, i, more=16), plan, todo, never), emit)
        for g in range(H // 2):
            acc = kvacc[64 * g:64 * g + 64, :] + lax.dot_general(
                _unpack(vt[32 * g:32 * g + 32, :]), _unpack(phi[64 * g:64 * g + 64, :]),
                NT_DIMS, preferred_element_type=F32)
            kvacc[64 * g:64 * g + 64, :] = acc
            kvt[32 * g:32 * g + 32, :] = _pack(jnp.where(same_head, acc, 0.0))

    def q_terms(b):
        return w_terms(folded(0, 2 * b, 128), folded(0, 2 * (b + NB), 128), wq_s, 2 * b)

    def fixed(steps):
        return lambda: steps

    never = pltpu.bitcast(zb[0:8, :], jnp.int32)
    _wait("wait_phi", phi_cp)
    _start(*wv_cp, xa_cp(1), wq_cp, wo_cp, *[xa_cp(i) for i in range(2, NT)], *ffn_cp)
    for g in range(D // 128):
        p = lax.dot_general(expand, wphi[g * 128:(g + 1) * 128, :], NT_DIMS,
                            preferred_element_type=F32)
        pt[g * 64:(g + 1) * 64, :] = _pack(jnp.where(diag, p, 0.0))
    _wait("wait_x", x0_cp(1))
    for step in x_terms(0, 0, (2, 4)):
        step(keep)
    top, ready = [], {2: [], 4: []}
    for h in range(2):
        if h == 0:
            _wait("wait_wk", wk_cp[0])
            x0 = [[], []]
        else:
            _wait("wait_wk", wk_cp[1], x0_cp(0))
            x0 = _split(x_terms(0, 0, (0, 1, 3, 5, 6)), (1, 1))
        for b in (2 * h, 2 * h + 1):
            top.append(folded(1, 2 * b, 128))
            for step in w_terms(top[b], None, wk_s, 2 * b, (2, 4)):
                step(keep)
        for n, steps in zip(ready, x0):
            ready[n].append(_shadow(lax.dot_general(
                _unpack(wk_s[n * WR + h * 128:n * WR + (h + 1) * 128, :]),
                _unpack(xs[n * (TH // 2):(n + 1) * (TH // 2), :]),
                NT_DIMS, preferred_element_type=F32), steps, never, []))
    ready = {n: jnp.concatenate(m, axis=0) for n, m in ready.items()}
    todo = []

    def rest_of_wk():
        _wait("wait_wk", wk_cp[2])
        for b in range(NB):
            low = folded(1, 2 * (b + NB), 128)
            for step in w_terms(top[b], low, wk_s, 2 * b, (0, 1, 3, 5, 6)):
                step(keep)
        return []

    later = []

    def top_of_wv():
        _wait("wait_wv", wv_cp[0])
        steps = []
        for b in range(NB):
            steps += w_terms(transposed(2, b), None, wv_s, 2 * b, (2, 4))
        later.extend(_split(steps, (1, 3)))
        return later.pop(0)

    def rest_of_wv():
        _wait("wait_wv", wv_cp[1])
        steps = []
        for b in range(NB):
            steps += w_terms(transposed(2, b), transposed(2, b + NB), wv_s, 2 * b,
                             (0, 1, 3, 5, 6))
        later.extend(_split(steps, (1, 1, 3)))
        return later.pop(0)

    def second_tile():
        _wait("wait_x", xa_cp(1))
        later.extend(_split(x_terms(1, 1), (1, 1, 1, 1)))
        return later.pop(0)

    nxt = bind(later.pop, 0)
    keys(0, [rest_of_wk, fixed([]), top_of_wv, nxt, rest_of_wv], todo, never, ready)
    values(0, [nxt, nxt, fixed([]), second_tile, nxt, nxt, nxt], todo, never)
    _wait("wait_wq", wq_cp, wo_cp)

    def phase1(i, carry):
        never = jnp.where(jnp.full((8, 128), i, jnp.int32) < 0, 1, 0)
        pl.when(i + 1 < NT)(lambda: _wait("wait_x", xa_cp(i + 1)))
        todo = []

        none = fixed([])
        w = [fixed(wo_terms(jnp.minimum(3 * (i - 1) + s, KH // 64 - 1))) for s in range(3)]
        q = _split(q_terms(i - 1), (1, 1))
        keys(i, [fixed(q[0]), fixed(q[1]), none, w[0], none, none, none], todo, never)
        x = _split(x_terms(jnp.minimum(i + 1, NT - 1), i + 1), (1, 1, 1))
        z = _split(z_total(), (1, 1, 1))
        x[2] = x[2] + w[1]()
        z[0] = z[0] + w[2]()
        values(i, [none] + [fixed(s) for s in x + z], todo, never)
        return carry

    lax.fori_loop(1, NT, phase1, 0)

    for step in q_terms(NB - 1):
        step(keep)

    r = score[1:2, :].astype(BF16).astype(F32)
    best = jnp.max(r, axis=-1, keepdims=True)
    tok = lax.broadcasted_iota(jnp.int32, (1, S), 1)
    idx = jnp.min(jnp.where(r == best, tok, S - 1))
    first = idx // T
    slab = pl.ds(pl.multiple_of((idx // 16) * 16, 16), 16)
    sel = lax.broadcasted_iota(jnp.int32, (16, D), 0) == idx % 16
    _wait("wait_ffn", *ffn_cp)

    def x_column():
        def step(k, pin):
            cols = slice(128 * k, 128 * k + 128)
            row = jnp.where(sel[:, cols], pin(xa[slab, cols].astype(F32)), 0.0)
            row = jnp.sum(row, axis=0, keepdims=True)
            xcol[cols, :] = jnp.broadcast_to(row, (128, 128)).T
        return [bind(step, k) for k in range(D // 128)]

    def fold8(x):
        return jnp.sum(x.reshape(x.shape[0] // 8, 8, 128), axis=0)

    def ffn_steps(i, y):
        st = {}
        part = _ds(i * FC, FC, 128)
        wg_i, wu_i, wd_i = wg.at[:, part], wu.at[:, part], wd.at[part]

        def up(j, k, pin):
            f = pl.ds(j * 128, 128)
            rows = slice(64 * k, 64 * k + 64)
            xc = xcol[rows, :]
            a = fold8(wg_i[rows, f].astype(F32) * xc)
            u = fold8(wu_i[rows, f].astype(F32) * xc)
            if k > 0:
                a, u = pin(st["a"]) + a, pin(st["u"]) + u
            st["a"], st["u"] = a, u
            token = a + u if BACK else None
            if k == D // 64 - 1:
                a = jnp.sum(a, axis=0, keepdims=True)
                u = jnp.sum(u, axis=0, keepdims=True)
                st["h"] = jnp.broadcast_to(a * jax.nn.sigmoid(a) * u, (128, 128)).T
            return token

        def down(j, n, pin):
            w = wd_i[j * 128:j * 128 + 128, 128 * n:128 * n + 128].astype(F32)
            y[n] = pin(y[n]) + fold8(w * st["h"])
            return y[n] if BACK else None

        steps = []
        for j in range(FC // 128):
            steps += [bind(up, j, k) for k in range(D // 64)]
            steps += [bind(down, j, n) for n in range(D // 128)]
        return steps

    def phase2(i, y):
        y = list(y)
        t = (first + i) % NT
        never = jnp.where(jnp.full((8, 128), i, jnp.int32) < 0, 1, 0)
        o = [[[], []], [[], []]]
        todo = []

        def attend(g, dst, ph, rden, pin):
            num = jnp.dot(_unpack(pin(kvt[32 * g:32 * g + 32, :])), ph,
                          preferred_element_type=F32)
            scale = jnp.concatenate(
                [jnp.broadcast_to(rden[0:1, :], (DH, TH)),
                 jnp.broadcast_to(rden[1:2, :], (DH, TH))], axis=0)
            dst.append(num * scale)

        def query(g, dst, p, pin):
            ph = _features(p, pin)
            z = zb[128 * g:128 * g + 128, :]
            dn = [a * jnp.tile(z[8 * k:8 * k + 8, :], (1, TH // 128)) for k, a in enumerate(ph)]
            rden = 1.0 / (_allreduce(jnp.add, dn) + 1e-6)
            todo.append(bind(attend, g, dst, jnp.concatenate(ph, axis=0).astype(BF16), rden))

        def emit_q(r, n, p):
            todo.extend(bind(query, r * KH // 64 + q, o[n][1 - r], p[64 * q:64 * q + 64, :])
                        for q in range(KH // 64))

        ffn = _split(ffn_steps(i, y), FFN_SHARES)
        plan = [fixed(x_column())] + [fixed(s) for s in ffn]
        due = []
        _strassen(staged(bind(project, wq_s, t), plan[:7], todo, never, due), emit_q)

        class Quad:
            def __init__(self, n):
                self.n = n

            def __getitem__(self, r):
                return jnp.concatenate(o[self.n][r], axis=0)

        def prod_o(n, due, never):
            w = _after(wo_s[n * (KH // 2):(n + 1) * (KH // 2), :], due, never, 1)
            return lax.dot_general(_LHS[n]([Quad(0), Quad(1)]).astype(BF16), _unpack(w),
                                   TN_DIMS, preferred_element_type=F32)

        def emit_o(n, c, a):
            gt = jnp.tile(gate[_ds(t * T + n * TH, TH), :], (1, KH // 128))
            b = xa[_ds(t * T + n * TH, TH), c * KH:(c + 1) * KH].astype(F32)
            outb[_ds(t * T + n * TH, TH), c * KH:(c + 1) * KH] = (
                gt * a + (1.0 - gt) * b).astype(BF16)
            out_cp(t, n, c, i).start()

        _strassen_diag(staged(prod_o, plan[7:], todo, never, due), emit_o)
        return tuple(y)

    y = lax.fori_loop(0, NT, phase2, (jnp.zeros((8, 128), F32),) * (D // 128))

    _wait("wait_out", *[out_cp(0, r, c, 0) for r in range(2) for c in range(2)])
    y = jnp.sum(jnp.concatenate(y, axis=1), axis=0, keepdims=True) * jax.nn.sigmoid(best)
    xsl = xa[slab, :].astype(F32)
    upd = (xsl + y).astype(BF16).astype(F32) - xsl
    gt = jnp.tile(gate[slab, :], (1, D // 128))
    old = outb[slab, :].astype(F32)
    outb[slab, :] = jnp.where(sel, old + (1.0 - gt) * upd, old).astype(BF16)
    fix_cp = pltpu.make_async_copy(outb.at[slab], out_hbm.at[slab], sem_x.at[NT])
    fix_cp.start()
    _wait("wait_out", fix_cp,
          *[out_cp(i, r, c, i) for i in range(1, NT) for r in range(2) for c in range(2)])


@jax.jit
def pallas_gated_mix__linear_kernel_hedgehog__moe_arch_mod__prompt_kernel(
    A_x, A_wqkv, A_w_phi, A_wo, B_x, B_w_r, B_w_gate, B_w_up, B_w_down, gate_w,
):
    del B_x
    hbm = pl.BlockSpec(memory_space=pl.ANY)
    vmem = pl.BlockSpec(memory_space=pltpu.VMEM)
    out = pl.pallas_call(
        _kernel,
        out_shape=jax.ShapeDtypeStruct((S, D), BF16),
        in_specs=[hbm, hbm, hbm, hbm, vmem, hbm, hbm, hbm, vmem],
        out_specs=hbm,
        scratch_shapes=[
            pltpu.VMEM((S, D), BF16),
            pltpu.VMEM((D, 3 * D), BF16),
            pltpu.VMEM((D, DH), BF16),
            pltpu.VMEM((D, D), BF16),
            pltpu.VMEM((D, F), BF16),
            pltpu.VMEM((D, F), BF16),
            pltpu.VMEM((F, D), BF16),
            pltpu.VMEM((7 * WR, KH), U32),
            pltpu.VMEM((7 * WR, KH), U32),
            pltpu.VMEM((7 * WR, KH), U32),
            pltpu.VMEM((7 * KH // 2, KH), U32),
            pltpu.VMEM(((NT + 1) * 7 * TH // 2, KH), U32),
            pltpu.VMEM((D // 2, 128), U32),
            pltpu.VMEM((D // 2, T), U32),
            pltpu.VMEM((D, T), U32),
            pltpu.VMEM((D, 128), F32),
            pltpu.VMEM((D // 2, 128), U32),
            pltpu.VMEM((2 * D, 128), F32),
            pltpu.VMEM((2 * D, 128), F32),
            pltpu.VMEM((S, 128), F32),
            pltpu.VMEM((8, S), F32),
            pltpu.VMEM((S, D), BF16),
            pltpu.VMEM((D, 128), F32),
            pltpu.SemaphoreType.DMA((NT + 1,)),
            pltpu.SemaphoreType.DMA((6,)),
            pltpu.SemaphoreType.DMA((7,)),
            pltpu.SemaphoreType.DMA((4 * NT,)),
        ],
        compiler_params=pltpu.CompilerParams(vmem_limit_bytes=110 * 2**20),
    )(A_x.reshape(S, D), A_wqkv, A_w_phi.reshape(H * DH, DH), A_wo,
      B_w_r, B_w_gate, B_w_up, B_w_down, gate_w)
    return out.reshape(1, S, D)
```

```python
import functools

import jax
import jax.numpy as jnp
from jax import lax
from jax.experimental import pallas as pl
from jax.experimental.pallas import tpu as pltpu

S, D, H, DH, F = 2048, 1024, 32, 32, 3584
T = 512
NT = S // T
TH, KH = T // 2, D // 2
WR = KH // 2 + 8
NB = KH // 128
FC = F // NT
SCOPES = False
BACK = True
FFN_SHARES = (3, 0, 2, 0, 2, 0, 0, 2, 3, 2, 2, 2, 1)
LOG2E = 1.4426950408889634
F32, BF16, U32 = jnp.float32, jnp.bfloat16, jnp.uint32
NT_DIMS = (((1,), (1,)), ((), ()))
TN_DIMS = (((0,), (0,)), ((), ()))
bind = functools.partial


def _tree(op, xs):
    xs = list(xs)
    while len(xs) > 1:
        xs = [op(xs[i], xs[i + 1]) if i + 1 < len(xs) else xs[i]
              for i in range(0, len(xs), 2)]
    return xs[0]


def _allreduce(op, xs):
    r = _tree(op, xs)
    r = op(r, pltpu.roll(r, 4, 0))
    return op(r, pltpu.roll(r, 2, 0))


def _recip(x):
    r = pl.reciprocal(x, approx=True)
    return r * (2.0 - x * r)


def _features(p, pin):
    rows = [p[8 * i:8 * i + 8, :] for i in range(8)]
    rows[0] = pin(rows[0])
    mx = _allreduce(jnp.maximum, rows)
    mn = _allreduce(jnp.minimum, rows)
    ep = [jnp.exp2(r - mx) for r in rows]
    en = [jnp.exp2(mn - r) for r in rows]
    rp = _recip(_allreduce(jnp.add, ep))
    rn = _recip(_allreduce(jnp.add, en))
    return [e * rp for e in ep] + [e * rn for e in en]


def _pack(x):
    return pltpu.bitcast(x.astype(BF16), U32)


def _unpack(x):
    return pltpu.bitcast(x, BF16)


_LHS = [lambda a: a[0][0] + a[1][1], lambda a: a[1][0] + a[1][1], lambda a: a[0][0],
        lambda a: a[1][1], lambda a: a[0][0] + a[0][1], lambda a: a[1][0] - a[0][0],
        lambda a: a[0][1] - a[1][1]]
_RHS = [lambda b: b[0][0] + b[1][1], lambda b: b[0][0], lambda b: b[0][1] - b[1][1],
        lambda b: b[1][0] - b[0][0], lambda b: b[1][1], lambda b: b[0][0] + b[0][1],
        lambda b: b[1][0] + b[1][1]]


def _strassen(prod, emit):
    m3 = prod(2)
    m5 = prod(4)
    emit(0, 1, m3 + m5)
    m2 = prod(1)
    m4 = prod(3)
    emit(1, 0, m2 + m4)
    m1 = prod(0)
    s1 = m4 - m5 + m1
    s2 = m3 - m2 + m1
    emit(0, 0, s1 + prod(6))
    emit(1, 1, s2 + prod(5))


def _strassen_diag(prod, emit):
    m3 = prod(2)
    m4 = prod(3)
    m1 = prod(0)
    m5 = prod(4)
    emit(0, 1, m3 + m5)
    emit(0, 0, m1 + m4 - m5 + prod(6))
    m2 = prod(1)
    emit(1, 0, m2 + m4)
    emit(1, 1, m1 + m3 - m2 + prod(5))


def _shadow(m, steps, never, due):
    rows, cols = m.shape[0] // 8, m.shape[1] // 128
    for s, step in enumerate(steps):
        p = rows * cols * s // len(steps)
        r, c = 8 * (p % rows), 128 * (p // rows)
        slab = m[r:r + 8, c:c + 128]

        def pin(v, slab=slab):
            reps = (v.shape[0] // 8, v.shape[1] // 128)
            other = slab if v.dtype == F32 else pltpu.bitcast(slab, v.dtype)
            return jnp.where(jnp.tile(never, reps) != 0, jnp.tile(other, reps), v)

        token = step(pin)
        if token is not None:
            due.append(token)
    return m


def _after(w, due, never, axis):
    if not due:
        return w
    unit = (8, 128)[axis]
    parts = jnp.split(w, w.shape[axis] // unit, axis=axis)
    for s, token in enumerate(due):
        p = len(parts) * s // len(due)
        head = jnp.where(never != 0, pltpu.bitcast(token, U32), parts[p][:8, :128])
        if axis == 0:
            parts[p] = jnp.concatenate([head, parts[p][:, 128:]], axis=1)
        else:
            parts[p] = jnp.concatenate([head, parts[p][8:, :]], axis=0)
    due.clear()
    return jnp.concatenate(parts, axis=axis)


def _split(steps, shares):
    out, done, total = [], 0, 0
    for s in shares:
        total += s
        end = len(steps) * total // sum(shares)
        out.append(steps[done:end])
        done = end
    return out


def _start(*cps):
    def step(i, carry):
        for n, cp in enumerate(cps):
            pl.when(i == n)(cp.start)
        return carry

    lax.fori_loop(0, len(cps), step, 0)


def _wait(name, *cps):
    if SCOPES:
        with jax.named_scope(name):
            for cp in cps:
                cp.wait()
    else:
        for cp in cps:
            cp.wait()


def _ds(start, size, mult=None):
    if isinstance(start, int):
        return pl.ds(start, size)
    return pl.ds(pl.multiple_of(start, mult or size), size)


def _kernel(xa_hbm, wqkv_hbm, wphi_hbm, wo_hbm, wr_ref, wg_hbm, wu_hbm,
            wd_hbm, gw_ref, out_hbm,
            xa, wqkv, wphi, wo, wg, wu, wd, wq_s, wk_s, wv_s, wo_s, xs, pt, vt, phi, kvacc, kvt, zacc,
            zb, gate, score, outb, xcol, sem_x, sem_w, sem_m, sem_o):
    def xa_cp(i):
        return pltpu.make_async_copy(xa_hbm.at[_ds(i * T, T)], xa.at[_ds(i * T, T)], sem_x.at[i])

    def w_cp(start, size, sem):
        cols = _ds(start, size)
        return pltpu.make_async_copy(wqkv_hbm.at[:, cols], wqkv.at[:, cols], sem_w.at[sem])

    def x0_cp(h):
        rows = pl.ds(h * TH, TH)
        return pltpu.make_async_copy(xa_hbm.at[rows], xa.at[rows], sem_m.at[h])

    wk_cp = [w_cp(D, KH // 2, 0), w_cp(D + KH // 2, KH // 2, 1), w_cp(D + KH, KH, 2)]
    wv_cp = [w_cp(2 * D, KH, 3), w_cp(2 * D + KH, KH, 4)]
    wq_cp = w_cp(0, D, 5)
    phi_cp = pltpu.make_async_copy(wphi_hbm, wphi, sem_m.at[2])
    wo_cp = pltpu.make_async_copy(wo_hbm, wo, sem_m.at[3])
    ffn_cp = [pltpu.make_async_copy(wg_hbm, wg, sem_m.at[4]),
              pltpu.make_async_copy(wu_hbm, wu, sem_m.at[5]),
              pltpu.make_async_copy(wd_hbm, wd, sem_m.at[6])]

    def out_cp(t, r, c, slot):
        blk = (_ds(t * T + r * TH, TH), pl.ds(c * KH, KH))
        return pltpu.make_async_copy(outb.at[blk], out_hbm.at[blk], sem_o.at[slot * 4 + r * 2 + c])

    zb[0:8, :] = jnp.zeros((8, 128), F32)
    _start(phi_cp, x0_cp(1), wk_cp[0], wk_cp[1], x0_cp(0), wk_cp[2])

    er = lax.broadcasted_iota(jnp.int32, (128, DH), 0)
    ec = lax.broadcasted_iota(jnp.int32, (128, DH), 1)
    expand = jnp.where((er % 64) // 2 == ec, 1.0, 0.0).astype(BF16)
    pr = lax.broadcasted_iota(jnp.int32, (128, 128), 0)
    pc = lax.broadcasted_iota(jnp.int32, (128, 128), 1)
    diag = pc // DH == 2 * (pr // 64) + pr % 2
    kr = lax.broadcasted_iota(jnp.int32, (64, 128), 0)
    kc = lax.broadcasted_iota(jnp.int32, (64, 128), 1)
    same_head = kr // DH == kc % 2
    kvacc[...] = jnp.zeros_like(kvacc)
    zacc[...] = jnp.zeros_like(zacc)
    xr = lax.broadcasted_iota(jnp.int32, (16, D), 0)
    extra = jnp.where(
        xr == 0, gw_ref[...].astype(F32).reshape(1, D),
        jnp.where(xr == 1, wr_ref[...].astype(F32).reshape(1, D), 0.0))
    zero = jnp.zeros((16, KH), F32)
    for j in range(7):
        wv_s[j * WR + KH // 2:(j + 1) * WR, :] = _pack(
            _LHS[j]([[extra[:, :KH], extra[:, KH:]], [zero, zero]]))

    def folded(j, u, n):
        w = wqkv[:, _ds(j * D + (u // 2) * 128, 128)]
        return lax.dot_general(_unpack(pt[_ds(u * 32, n // 2), :]), w, NT_DIMS,
                               preferred_element_type=F32) * LOG2E

    def transposed(j, g):
        return wqkv[:, _ds(j * D + g * 128, 128)].T

    def keep(v):
        return v

    def w_terms(r1, r2, dst, u, terms=range(7)):
        dst = dst.at[_ds(u * 32, 6 * WR + r1.shape[0] // 2, 32)]

        def step(h, pin):
            rows = slice(16 * h, 16 * h + 16)
            a = r1[rows, :].astype(F32)
            top = [pin(a[:, :KH]), a[:, KH:]]
            low = None
            if r2 is not None:
                a = r2[rows, :].astype(F32)
                low = [a[:, :KH], pin(a[:, KH:])]
            for n in terms:
                dst[pl.ds(n * WR + h * 8, 8), :] = _pack(_LHS[n]([top, low]))
        return [bind(step, h) for h in range(r1.shape[0] // 16)]

    def wo_terms(u):
        src = wo.at[_ds(u * 64, KH + 64, 64)]
        dst = wo_s.at[_ds(u * 32, 6 * (KH // 2) + 32, 32)]

        def step(h, pin):
            r1 = src[pl.ds(KH + h * 16, 16), :].astype(F32)
            r2 = src[pl.ds(h * 16, 16), :].astype(F32)
            quad = [[pin(r1[:, :KH]), r1[:, KH:]], [r2[:, :KH], pin(r2[:, KH:])]]
            for n in range(7):
                dst[pl.ds(n * (KH // 2) + h * 8, 8), :] = _pack(_RHS[n](quad))
        return [bind(step, h) for h in range(4)]

    def x_terms(i, slot, terms=range(7)):
        src = xa.at[_ds(i * T, T)]
        dst = xs.at[_ds(slot * 7 * (TH // 2), 7 * (TH // 2))]

        def step(h, pin):
            x2 = src[pl.ds(TH + h * 16, 16), :].astype(F32)
            quad = [[None, x2[:, :KH]], [None, pin(x2[:, KH:])]]
            if set(terms) - {2, 4}:
                x1 = src[pl.ds(h * 16, 16), :].astype(F32)
                quad[0][0], quad[1][0] = pin(x1[:, :KH]), x1[:, KH:]
            for n in terms:
                dst[pl.ds(n * (TH // 2) + h * 8, 8), :] = _pack(_RHS[n](quad))
        return [bind(step, h) for h in range(TH // 16)]

    def z_total():
        def step(g, pin):
            rows = slice(128 * g, 128 * g + 128)
            z = jnp.sum(pin(zacc[rows, :]), axis=-1, keepdims=True)
            zb[rows, :] = jnp.broadcast_to(z, (128, 128))
        return [bind(step, g) for g in range(H // 2)]

    def project(w_s, i, n, due, never, more=0):
        w = _after(w_s[n * WR:n * WR + (KH + more) // 2, :], due, never, 0)
        return lax.dot_general(_unpack(w),
                               _unpack(xs[_ds((i * 7 + n) * (TH // 2), TH // 2), :]),
                               NT_DIMS, preferred_element_type=F32)

    def staged(f, plan, todo, never, due=None):
        plan = list(plan)
        due = [] if due is None else due

        def prod(n):
            steps = plan.pop(0)()
            follow = list(todo)
            todo.clear()
            return _shadow(_shadow(f(n, due, never), follow, never, due), steps, never, due)
        return prod

    def keys(i, plan, todo, never, ready=None):
        def step(g, n, p, pin):
            ph = _features(p, pin)
            zs = [_tree(jnp.add, [a[:, 128 * l:128 * l + 128] for l in range(TH // 128)])
                  for a in ph]
            zacc[128 * g:128 * g + 128, :] += jnp.concatenate(zs, axis=0)
            phi[64 * g:64 * g + 64, n * TH:(n + 1) * TH] = _pack(jnp.concatenate(ph, axis=0))
            return zs[0] + zs[8]

        def emit(r, n, p):
            todo.extend(bind(step, r * KH // 64 + q, n, p[64 * q:64 * q + 64, :])
                        for q in range(KH // 64))
        prod = staged(bind(project, wk_s, i), plan, todo, never)
        _strassen(lambda n: ready[n] if ready and n in ready else prod(n), emit)

    def values(i, plan, todo, never):
        def emit(r, n, v):
            vt[r * KH // 2:(r + 1) * KH // 2, n * TH:(n + 1) * TH] = _pack(v[:KH, :])
            if r == 0:
                gr = v[KH:KH + 8, :]
                score[:, _ds(i * T + n * TH, TH)] = gr
                gt = jax.nn.sigmoid(gr)
                gate[_ds(i * T + n * TH, TH), :] = jnp.broadcast_to(gt[0:1, :], (128, TH)).T
        _strassen(staged(bind(project, wv_s, i, more=16), plan, todo, never), emit)
        for g in range(H // 2):
            acc = kvacc[64 * g:64 * g + 64, :] + lax.dot_general(
                _unpack(vt[32 * g:32 * g + 32, :]), _unpack(phi[64 * g:64 * g + 64, :]),
                NT_DIMS, preferred_element_type=F32)
            kvacc[64 * g:64 * g + 64, :] = acc
            kvt[32 * g:32 * g + 32, :] = _pack(jnp.where(same_head, acc, 0.0))

    def q_terms(b):
        return w_terms(folded(0, 2 * b, 128), folded(0, 2 * (b + NB), 128), wq_s, 2 * b)

    def fixed(steps):
        return lambda: steps

    never = pltpu.bitcast(zb[0:8, :], jnp.int32)
    _wait("wait_phi", phi_cp)
    _start(*wv_cp, xa_cp(1), wq_cp, wo_cp, *[xa_cp(i) for i in range(2, NT)], *ffn_cp)
    for g in range(D // 128):
        p = lax.dot_general(expand, wphi[g * 128:(g + 1) * 128, :], NT_DIMS,
                            preferred_element_type=F32)
        pt[g * 64:(g + 1) * 64, :] = _pack(jnp.where(diag, p, 0.0))
    _wait("wait_x", x0_cp(1))
    for step in x_terms(0, 0, (2, 4)):
        step(keep)
    top, ready = [], {2: [], 4: []}
    for h in range(2):
        if h == 0:
            _wait("wait_wk", wk_cp[0])
            x0 = [[], []]
        else:
            _wait("wait_wk", wk_cp[1], x0_cp(0))
            x0 = _split(x_terms(0, 0, (0, 1, 3, 5, 6)), (1, 1))
        for b in (2 * h, 2 * h + 1):
            top.append(folded(1, 2 * b, 128))
            for step in w_terms(top[b], None, wk_s, 2 * b, (2, 4)):
                step(keep)
        for n, steps in zip(ready, x0):
            ready[n].append(_shadow(lax.dot_general(
                _unpack(wk_s[n * WR + h * 128:n * WR + (h + 1) * 128, :]),
                _unpack(xs[n * (TH // 2):(n + 1) * (TH // 2), :]),
                NT_DIMS, preferred_element_type=F32), steps, never, []))
    ready = {n: jnp.concatenate(m, axis=0) for n, m in ready.items()}
    todo = []

    def rest_of_wk():
        _wait("wait_wk", wk_cp[2])
        for b in range(NB):
            low = folded(1, 2 * (b + NB), 128)
            for step in w_terms(top[b], low, wk_s, 2 * b, (0, 1, 3, 5, 6)):
                step(keep)
        return []

    later = []

    def top_of_wv():
        _wait("wait_wv", wv_cp[0])
        steps = []
        for b in range(NB):
            steps += w_terms(transposed(2, b), None, wv_s, 2 * b, (2, 4))
        later.extend(_split(steps, (1, 3)))
        return later.pop(0)

    def rest_of_wv():
        _wait("wait_wv", wv_cp[1])
        steps = []
        for b in range(NB):
            steps += w_terms(transposed(2, b), transposed(2, b + NB), wv_s, 2 * b,
                             (0, 1, 3, 5, 6))
        later.extend(_split(steps, (1, 1, 3)))
        return later.pop(0)

    def second_tile():
        _wait("wait_x", xa_cp(1))
        later.extend(_split(x_terms(1, 1), (1, 1, 1, 1)))
        return later.pop(0)

    nxt = bind(later.pop, 0)
    keys(0, [rest_of_wk, fixed([]), top_of_wv, nxt, rest_of_wv], todo, never, ready)
    values(0, [nxt, nxt, fixed([]), second_tile, nxt, nxt, nxt], todo, never)
    _wait("wait_wq", wq_cp, wo_cp)

    def phase1(i, carry):
        never = jnp.where(jnp.full((8, 128), i, jnp.int32) < 0, 1, 0)
        pl.when(i + 1 < NT)(lambda: _wait("wait_x", xa_cp(i + 1)))
        todo = []

        none = fixed([])
        w = [fixed(wo_terms(jnp.minimum(3 * (i - 1) + s, KH // 64 - 1))) for s in range(3)]
        q = _split(q_terms(i - 1), (1, 1))
        keys(i, [fixed(q[0]), fixed(q[1]), none, w[0], none, none, none], todo, never)
        x = _split(x_terms(jnp.minimum(i + 1, NT - 1), i + 1), (1, 1, 1))
        z = _split(z_total(), (1, 1, 1))
        x[2] = x[2] + w[1]()
        z[0] = z[0] + w[2]()
        values(i, [none] + [fixed(s) for s in x + z], todo, never)
        return carry

    lax.fori_loop(1, NT, phase1, 0)

    for step in q_terms(NB - 1):
        step(keep)

    r = score[1:2, :].astype(BF16).astype(F32)
    best = jnp.max(r, axis=-1, keepdims=True)
    tok = lax.broadcasted_iota(jnp.int32, (1, S), 1)
    idx = jnp.min(jnp.where(r == best, tok, S - 1))
    first = idx // T
    slab = pl.ds(pl.multiple_of((idx // 16) * 16, 16), 16)
    sel = lax.broadcasted_iota(jnp.int32, (16, D), 0) == idx % 16
    _wait("wait_ffn", *ffn_cp)

    def x_column():
        def step(k, pin):
            cols = slice(128 * k, 128 * k + 128)
            row = jnp.where(sel[:, cols], pin(xa[slab, cols].astype(F32)), 0.0)
            row = jnp.sum(row, axis=0, keepdims=True)
            xcol[cols, :] = jnp.broadcast_to(row, (128, 128)).T
        return [bind(step, k) for k in range(D // 128)]

    def fold8(x):
        return jnp.sum(x.reshape(x.shape[0] // 8, 8, 128), axis=0)

    def ffn_steps(i, y):
        st = {}
        part = _ds(i * FC, FC, 128)
        wg_i, wu_i, wd_i = wg.at[:, part], wu.at[:, part], wd.at[part]

        def up(j, k, pin):
            f = pl.ds(j * 128, 128)
            rows = slice(64 * k, 64 * k + 64)
            xc = xcol[rows, :]
            a = fold8(wg_i[rows, f].astype(F32) * xc)
            u = fold8(wu_i[rows, f].astype(F32) * xc)
            if k > 0:
                a, u = pin(st["a"]) + a, pin(st["u"]) + u
            st["a"], st["u"] = a, u
            token = a + u if BACK else None
            if k == D // 64 - 1:
                a = jnp.sum(a, axis=0, keepdims=True)
                u = jnp.sum(u, axis=0, keepdims=True)
                st["h"] = jnp.broadcast_to(a * jax.nn.sigmoid(a) * u, (128, 128)).T
            return token

        def down(j, n, pin):
            w = wd_i[j * 128:j * 128 + 128, 128 * n:128 * n + 128].astype(F32)
            y[n] = pin(y[n]) + fold8(w * st["h"])
            return y[n] if BACK else None

        steps = []
        for j in range(FC // 128):
            steps += [bind(up, j, k) for k in range(D // 64)]
            steps += [bind(down, j, n) for n in range(D // 128)]
        return steps

    def phase2(i, y):
        y = list(y)
        t = (first + i) % NT
        never = jnp.where(jnp.full((8, 128), i, jnp.int32) < 0, 1, 0)
        o = [[[], []], [[], []]]
        todo = []

        def attend(g, dst, ph, rden, pin):
            num = jnp.dot(_unpack(pin(kvt[32 * g:32 * g + 32, :])), ph,
                          preferred_element_type=F32)
            scale = jnp.concatenate(
                [jnp.broadcast_to(rden[0:1, :], (DH, TH)),
                 jnp.broadcast_to(rden[1:2, :], (DH, TH))], axis=0)
            dst.append(num * scale)

        def query(g, dst, p, pin):
            ph = _features(p, pin)
            z = zb[128 * g:128 * g + 128, :]
            dn = [a * jnp.tile(z[8 * k:8 * k + 8, :], (1, TH // 128)) for k, a in enumerate(ph)]
            rden = _recip(_allreduce(jnp.add, dn) + 1e-6)
            todo.append(bind(attend, g, dst, jnp.concatenate(ph, axis=0).astype(BF16), rden))

        def emit_q(r, n, p):
            todo.extend(bind(query, r * KH // 64 + q, o[n][1 - r], p[64 * q:64 * q + 64, :])
                        for q in range(KH // 64))

        ffn = _split(ffn_steps(i, y), FFN_SHARES)
        plan = [fixed(x_column())] + [fixed(s) for s in ffn]
        due = []
        _strassen(staged(bind(project, wq_s, t), plan[:7], todo, never, due), emit_q)

        class Quad:
            def __init__(self, n):
                self.n = n

            def __getitem__(self, r):
                return jnp.concatenate(o[self.n][r], axis=0)

        def prod_o(n, due, never):
            w = _after(wo_s[n * (KH // 2):(n + 1) * (KH // 2), :], due, never, 1)
            return lax.dot_general(_LHS[n]([Quad(0), Quad(1)]).astype(BF16), _unpack(w),
                                   TN_DIMS, preferred_element_type=F32)

        def emit_o(n, c, a):
            gt = jnp.tile(gate[_ds(t * T + n * TH, TH), :], (1, KH // 128))
            b = xa[_ds(t * T + n * TH, TH), c * KH:(c + 1) * KH].astype(F32)
            outb[_ds(t * T + n * TH, TH), c * KH:(c + 1) * KH] = (
                gt * a + (1.0 - gt) * b).astype(BF16)
            out_cp(t, n, c, i).start()

        _strassen_diag(staged(prod_o, plan[7:], todo, never, due), emit_o)
        return tuple(y)

    y = lax.fori_loop(0, NT, phase2, (jnp.zeros((8, 128), F32),) * (D // 128))

    _wait("wait_out", *[out_cp(0, r, c, 0) for r in range(2) for c in range(2)])
    y = jnp.sum(jnp.concatenate(y, axis=1), axis=0, keepdims=True) * jax.nn.sigmoid(best)
    xsl = xa[slab, :].astype(F32)
    upd = (xsl + y).astype(BF16).astype(F32) - xsl
    gt = jnp.tile(gate[slab, :], (1, D // 128))
    old = outb[slab, :].astype(F32)
    outb[slab, :] = jnp.where(sel, old + (1.0 - gt) * upd, old).astype(BF16)
    fix_cp = pltpu.make_async_copy(outb.at[slab], out_hbm.at[slab], sem_x.at[NT])
    fix_cp.start()
    _wait("wait_out", fix_cp,
          *[out_cp(i, r, c, i) for i in range(1, NT) for r in range(2) for c in range(2)])


@jax.jit
def pallas_gated_mix__linear_kernel_hedgehog__moe_arch_mod__prompt_kernel(
    A_x, A_wqkv, A_w_phi, A_wo, B_x, B_w_r, B_w_gate, B_w_up, B_w_down, gate_w,
):
    del B_x
    hbm = pl.BlockSpec(memory_space=pl.ANY)
    vmem = pl.BlockSpec(memory_space=pltpu.VMEM)
    out = pl.pallas_call(
        _kernel,
        out_shape=jax.ShapeDtypeStruct((S, D), BF16),
        in_specs=[hbm, hbm, hbm, hbm, vmem, hbm, hbm, hbm, vmem],
        out_specs=hbm,
        scratch_shapes=[
            pltpu.VMEM((S, D), BF16),
            pltpu.VMEM((D, 3 * D), BF16),
            pltpu.VMEM((D, DH), BF16),
            pltpu.VMEM((D, D), BF16),
            pltpu.VMEM((D, F), BF16),
            pltpu.VMEM((D, F), BF16),
            pltpu.VMEM((F, D), BF16),
            pltpu.VMEM((7 * WR, KH), U32),
            pltpu.VMEM((7 * WR, KH), U32),
            pltpu.VMEM((7 * WR, KH), U32),
            pltpu.VMEM((7 * KH // 2, KH), U32),
            pltpu.VMEM(((NT + 1) * 7 * TH // 2, KH), U32),
            pltpu.VMEM((D // 2, 128), U32),
            pltpu.VMEM((D // 2, T), U32),
            pltpu.VMEM((D, T), U32),
            pltpu.VMEM((D, 128), F32),
            pltpu.VMEM((D // 2, 128), U32),
            pltpu.VMEM((2 * D, 128), F32),
            pltpu.VMEM((2 * D, 128), F32),
            pltpu.VMEM((S, 128), F32),
            pltpu.VMEM((8, S), F32),
            pltpu.VMEM((S, D), BF16),
            pltpu.VMEM((D, 128), F32),
            pltpu.SemaphoreType.DMA((NT + 1,)),
            pltpu.SemaphoreType.DMA((6,)),
            pltpu.SemaphoreType.DMA((7,)),
            pltpu.SemaphoreType.DMA((4 * NT,)),
        ],
        compiler_params=pltpu.CompilerParams(vmem_limit_bytes=110 * 2**20),
    )(A_x.reshape(S, D), A_wqkv, A_w_phi.reshape(H * DH, DH), A_wo,
      B_w_r, B_w_gate, B_w_up, B_w_down, gate_w)
    return out.reshape(1, S, D)
```

```python
import functools

import jax
import jax.numpy as jnp
from jax import lax
from jax.experimental import pallas as pl
from jax.experimental.pallas import tpu as pltpu

S, D, H, DH, F = 2048, 1024, 32, 32, 3584
T = 512
NT = S // T
TH, KH = T // 2, D // 2
WR = KH // 2
NB = KH // 128
FC = F // NT
SCOPES = False
BACK = True
FFN_SHARES = (3, 0, 2, 0, 2, 0, 0, 2, 3, 2, 2, 2, 1)
LOG2E = 1.4426950408889634
F32, BF16, U32 = jnp.float32, jnp.bfloat16, jnp.uint32
NT_DIMS = (((1,), (1,)), ((), ()))
TN_DIMS = (((0,), (0,)), ((), ()))
bind = functools.partial


def _tree(op, xs):
    xs = list(xs)
    while len(xs) > 1:
        xs = [op(xs[i], xs[i + 1]) if i + 1 < len(xs) else xs[i]
              for i in range(0, len(xs), 2)]
    return xs[0]


def _allreduce(op, xs):
    r = _tree(op, xs)
    r = op(r, pltpu.roll(r, 4, 0))
    return op(r, pltpu.roll(r, 2, 0))


def _recip(x):
    r = pl.reciprocal(x, approx=True)
    return r * (2.0 - x * r)


def _features(p, pin):
    rows = [p[8 * i:8 * i + 8, :] for i in range(8)]
    rows[0] = pin(rows[0])
    mx = _allreduce(jnp.maximum, rows)
    mn = _allreduce(jnp.minimum, rows)
    ep = [jnp.exp2(r - mx) for r in rows]
    en = [jnp.exp2(mn - r) for r in rows]
    rp = _recip(_allreduce(jnp.add, ep))
    rn = _recip(_allreduce(jnp.add, en))
    return [e * rp for e in ep] + [e * rn for e in en]


def _pack(x):
    return pltpu.bitcast(x.astype(BF16), U32)


def _unpack(x):
    return pltpu.bitcast(x, BF16)


_LHS = [lambda a: a[0][0] + a[1][1], lambda a: a[1][0] + a[1][1], lambda a: a[0][0],
        lambda a: a[1][1], lambda a: a[0][0] + a[0][1], lambda a: a[1][0] - a[0][0],
        lambda a: a[0][1] - a[1][1]]
_RHS = [lambda b: b[0][0] + b[1][1], lambda b: b[0][0], lambda b: b[0][1] - b[1][1],
        lambda b: b[1][0] - b[0][0], lambda b: b[1][1], lambda b: b[0][0] + b[0][1],
        lambda b: b[1][0] + b[1][1]]


def _strassen(prod, emit):
    m3 = prod(2)
    m5 = prod(4)
    emit(0, 1, m3 + m5)
    m2 = prod(1)
    m4 = prod(3)
    emit(1, 0, m2 + m4)
    m1 = prod(0)
    s1 = m4 - m5 + m1
    s2 = m3 - m2 + m1
    emit(0, 0, s1 + prod(6))
    emit(1, 1, s2 + prod(5))


def _strassen_diag(prod, emit):
    m3 = prod(2)
    m4 = prod(3)
    m1 = prod(0)
    m5 = prod(4)
    emit(0, 1, m3 + m5)
    emit(0, 0, m1 + m4 - m5 + prod(6))
    m2 = prod(1)
    emit(1, 0, m2 + m4)
    emit(1, 1, m1 + m3 - m2 + prod(5))


def _shadow(m, steps, never, due):
    rows, cols = m.shape[0] // 8, m.shape[1] // 128
    for s, step in enumerate(steps):
        p = rows * cols * s // len(steps)
        r, c = 8 * (p % rows), 128 * (p // rows)
        slab = m[r:r + 8, c:c + 128]

        def pin(v, slab=slab):
            reps = (v.shape[0] // 8, v.shape[1] // 128)
            other = slab if v.dtype == F32 else pltpu.bitcast(slab, v.dtype)
            return jnp.where(jnp.tile(never, reps) != 0, jnp.tile(other, reps), v)

        token = step(pin)
        if token is not None:
            due.append(token)
    return m


def _after(w, due, never, axis):
    if not due:
        return w
    unit = (8, 128)[axis]
    parts = jnp.split(w, w.shape[axis] // unit, axis=axis)
    for s, token in enumerate(due):
        p = len(parts) * s // len(due)
        head = jnp.where(never != 0, pltpu.bitcast(token, U32), parts[p][:8, :128])
        if axis == 0:
            parts[p] = jnp.concatenate([head, parts[p][:, 128:]], axis=1)
        else:
            parts[p] = jnp.concatenate([head, parts[p][8:, :]], axis=0)
    due.clear()
    return jnp.concatenate(parts, axis=axis)


def _split(steps, shares):
    out, done, total = [], 0, 0
    for s in shares:
        total += s
        end = len(steps) * total // sum(shares)
        out.append(steps[done:end])
        done = end
    return out


def _start(*cps):
    def step(i, carry):
        for n, cp in enumerate(cps):
            pl.when(i == n)(cp.start)
        return carry

    lax.fori_loop(0, len(cps), step, 0)


def _wait(name, *cps):
    if SCOPES:
        with jax.named_scope(name):
            for cp in cps:
                cp.wait()
    else:
        for cp in cps:
            cp.wait()


def _ds(start, size, mult=None):
    if isinstance(start, int):
        return pl.ds(start, size)
    return pl.ds(pl.multiple_of(start, mult or size), size)


def _kernel(xa_hbm, wqkv_hbm, wphi_hbm, wo_hbm, wr_ref, wg_hbm, wu_hbm,
            wd_hbm, gw_ref, out_hbm,
            xa, wqkv, wphi, wo, wg, wu, wd, wq_s, wk_s, wv_s, wo_s, xs, pt, vt, phi, kvacc, kvt, zacc,
            zb, gate, outb, xcol, sem_x, sem_w, sem_m, sem_o):
    def xa_cp(i):
        return pltpu.make_async_copy(xa_hbm.at[_ds(i * T, T)], xa.at[_ds(i * T, T)], sem_x.at[i])

    def w_cp(start, size, sem):
        cols = _ds(start, size)
        return pltpu.make_async_copy(wqkv_hbm.at[:, cols], wqkv.at[:, cols], sem_w.at[sem])

    def x0_cp(h):
        rows = pl.ds(h * TH, TH)
        return pltpu.make_async_copy(xa_hbm.at[rows], xa.at[rows], sem_m.at[h])

    wk_cp = [w_cp(D, KH // 2, 0), w_cp(D + KH // 2, KH // 2, 1), w_cp(D + KH, KH, 2)]
    wv_cp = [w_cp(2 * D, KH, 3), w_cp(2 * D + KH, KH, 4)]
    wq_cp = w_cp(0, D, 5)
    phi_cp = pltpu.make_async_copy(wphi_hbm, wphi, sem_m.at[2])
    wo_cp = pltpu.make_async_copy(wo_hbm, wo, sem_m.at[3])
    ffn_cp = [pltpu.make_async_copy(wg_hbm, wg, sem_m.at[4]),
              pltpu.make_async_copy(wu_hbm, wu, sem_m.at[5]),
              pltpu.make_async_copy(wd_hbm, wd, sem_m.at[6])]

    def out_cp(t, r, c, slot):
        blk = (_ds(t * T + r * TH, TH), pl.ds(c * KH, KH))
        return pltpu.make_async_copy(outb.at[blk], out_hbm.at[blk], sem_o.at[slot * 4 + r * 2 + c])

    zb[0:8, :] = jnp.zeros((8, 128), F32)
    _start(phi_cp, x0_cp(1), wk_cp[0], wk_cp[1], x0_cp(0), wk_cp[2])

    er = lax.broadcasted_iota(jnp.int32, (128, DH), 0)
    ec = lax.broadcasted_iota(jnp.int32, (128, DH), 1)
    expand = jnp.where((er % 64) // 2 == ec, 1.0, 0.0).astype(BF16)
    pr = lax.broadcasted_iota(jnp.int32, (128, 128), 0)
    pc = lax.broadcasted_iota(jnp.int32, (128, 128), 1)
    diag = pc // DH == 2 * (pr // 64) + pr % 2
    kr = lax.broadcasted_iota(jnp.int32, (64, 128), 0)
    kc = lax.broadcasted_iota(jnp.int32, (64, 128), 1)
    same_head = kr // DH == kc % 2
    kvacc[...] = jnp.zeros_like(kvacc)
    zacc[...] = jnp.zeros_like(zacc)
    gw = gw_ref[...].astype(F32).reshape(1, D)
    wr = wr_ref[...].astype(F32).reshape(1, D)

    def folded(j, u, n):
        w = wqkv[:, _ds(j * D + (u // 2) * 128, 128)]
        return lax.dot_general(_unpack(pt[_ds(u * 32, n // 2), :]), w, NT_DIMS,
                               preferred_element_type=F32) * LOG2E

    def transposed(j, g):
        return wqkv[:, _ds(j * D + g * 128, 128)].T

    def keep(v):
        return v

    def w_terms(r1, r2, dst, u, terms=range(7)):
        dst = dst.at[_ds(u * 32, 6 * WR + r1.shape[0] // 2, 32)]

        def step(h, pin):
            rows = slice(16 * h, 16 * h + 16)
            a = r1[rows, :].astype(F32)
            top = [pin(a[:, :KH]), a[:, KH:]]
            low = None
            if r2 is not None:
                a = r2[rows, :].astype(F32)
                low = [a[:, :KH], pin(a[:, KH:])]
            for n in terms:
                dst[pl.ds(n * WR + h * 8, 8), :] = _pack(_LHS[n]([top, low]))
        return [bind(step, h) for h in range(r1.shape[0] // 16)]

    def wo_terms(u):
        src = wo.at[_ds(u * 64, KH + 64, 64)]
        dst = wo_s.at[_ds(u * 32, 6 * (KH // 2) + 32, 32)]

        def step(h, pin):
            r1 = src[pl.ds(KH + h * 16, 16), :].astype(F32)
            r2 = src[pl.ds(h * 16, 16), :].astype(F32)
            quad = [[pin(r1[:, :KH]), r1[:, KH:]], [r2[:, :KH], pin(r2[:, KH:])]]
            for n in range(7):
                dst[pl.ds(n * (KH // 2) + h * 8, 8), :] = _pack(_RHS[n](quad))
        return [bind(step, h) for h in range(4)]

    def x_terms(i, slot, terms=range(7), route=None):
        src = xa.at[_ds(i * T, T)]
        dst = xs.at[_ds(slot * 7 * (TH // 2), 7 * (TH // 2))]
        mix = gate.at[_ds(i * T, T)]

        def step(h, pin):
            x2 = src[pl.ds(TH + h * 16, 16), :].astype(F32)
            quad = [[None, x2[:, :KH]], [None, pin(x2[:, KH:])]]
            if set(terms) - {2, 4}:
                x1 = src[pl.ds(h * 16, 16), :].astype(F32)
                quad[0][0], quad[1][0] = pin(x1[:, :KH]), x1[:, KH:]
            for n in terms:
                dst[pl.ds(n * (TH // 2) + h * 8, 8), :] = _pack(_RHS[n](quad))
            for c in range(2) if route else ():
                row = TH * c + 16 * h
                g = quad[0][c] * gw[:, :KH] + quad[1][c] * gw[:, KH:]
                mix[row:row + 16, :] = jnp.broadcast_to(
                    jax.nn.sigmoid(jnp.sum(g, axis=-1, keepdims=True)), (16, 128))
                r = quad[0][c] * wr[:, :KH] + quad[1][c] * wr[:, KH:]
                r = jnp.sum(r, axis=-1, keepdims=True).astype(BF16).astype(F32)
                tok = i * T + row + lax.broadcasted_iota(jnp.int32, (16, 1), 0)
                best, where = route
                better = (r > best) | ((r == best) & (tok < where))
                route[:] = jnp.where(better, r, best), jnp.where(better, tok, where)
        return [bind(step, h) for h in range(TH // 16)]

    def z_total():
        def step(g, pin):
            rows = slice(128 * g, 128 * g + 128)
            z = jnp.sum(pin(zacc[rows, :]), axis=-1, keepdims=True)
            zb[rows, :] = jnp.broadcast_to(z, (128, 128))
        return [bind(step, g) for g in range(H // 2)]

    def project(w_s, i, n, due, never):
        w = _after(w_s[n * WR:(n + 1) * WR, :], due, never, 0)
        return lax.dot_general(_unpack(w),
                               _unpack(xs[_ds((i * 7 + n) * (TH // 2), TH // 2), :]),
                               NT_DIMS, preferred_element_type=F32)

    def staged(f, plan, todo, never, due=None):
        plan = list(plan)
        due = [] if due is None else due

        def prod(n):
            steps = plan.pop(0)()
            follow = list(todo)
            todo.clear()
            return _shadow(_shadow(f(n, due, never), follow, never, due), steps, never, due)
        return prod

    def keys(i, plan, todo, never, ready=None):
        def step(g, n, p, pin):
            ph = _features(p, pin)
            zs = [_tree(jnp.add, [a[:, 128 * l:128 * l + 128] for l in range(TH // 128)])
                  for a in ph]
            zacc[128 * g:128 * g + 128, :] += jnp.concatenate(zs, axis=0)
            phi[64 * g:64 * g + 64, n * TH:(n + 1) * TH] = _pack(jnp.concatenate(ph, axis=0))
            return zs[0] + zs[8]

        def emit(r, n, p):
            todo.extend(bind(step, r * KH // 64 + q, n, p[64 * q:64 * q + 64, :])
                        for q in range(KH // 64))
        prod = staged(bind(project, wk_s, i), plan, todo, never)
        _strassen(lambda n: ready[n] if ready and n in ready else prod(n), emit)

    def values(i, plan, todo, never):
        def emit(r, n, v):
            vt[r * KH // 2:(r + 1) * KH // 2, n * TH:(n + 1) * TH] = _pack(v)
        _strassen(staged(bind(project, wv_s, i), plan, todo, never), emit)
        for g in range(H // 2):
            acc = kvacc[64 * g:64 * g + 64, :] + lax.dot_general(
                _unpack(vt[32 * g:32 * g + 32, :]), _unpack(phi[64 * g:64 * g + 64, :]),
                NT_DIMS, preferred_element_type=F32)
            kvacc[64 * g:64 * g + 64, :] = acc
            kvt[32 * g:32 * g + 32, :] = _pack(jnp.where(same_head, acc, 0.0))

    def q_terms(b):
        return w_terms(folded(0, 2 * b, 128), folded(0, 2 * (b + NB), 128), wq_s, 2 * b)

    def fixed(steps):
        return lambda: steps

    never = pltpu.bitcast(zb[0:8, :], jnp.int32)
    _wait("wait_phi", phi_cp)
    _start(*wv_cp, xa_cp(1), wq_cp, wo_cp, *[xa_cp(i) for i in range(2, NT)], *ffn_cp)
    for g in range(D // 128):
        p = lax.dot_general(expand, wphi[g * 128:(g + 1) * 128, :], NT_DIMS,
                            preferred_element_type=F32)
        pt[g * 64:(g + 1) * 64, :] = _pack(jnp.where(diag, p, 0.0))
    _wait("wait_x", x0_cp(1))
    for step in x_terms(0, 0, (2, 4)):
        step(keep)
    route = [jnp.full((16, 1), -jnp.inf, F32), jnp.zeros((16, 1), jnp.int32)]
    top, ready = [], {2: [], 4: []}
    for h in range(2):
        if h == 0:
            _wait("wait_wk", wk_cp[0])
            x0 = [[], []]
        else:
            _wait("wait_wk", wk_cp[1], x0_cp(0))
            x0 = _split(x_terms(0, 0, (0, 1, 3, 5, 6), route), (1, 1))
        for b in (2 * h, 2 * h + 1):
            top.append(folded(1, 2 * b, 128))
            for step in w_terms(top[b], None, wk_s, 2 * b, (2, 4)):
                step(keep)
        for n, steps in zip(ready, x0):
            ready[n].append(_shadow(lax.dot_general(
                _unpack(wk_s[n * WR + h * 128:n * WR + (h + 1) * 128, :]),
                _unpack(xs[n * (TH // 2):(n + 1) * (TH // 2), :]),
                NT_DIMS, preferred_element_type=F32), steps, never, []))
    ready = {n: jnp.concatenate(m, axis=0) for n, m in ready.items()}
    todo = []

    def rest_of_wk():
        _wait("wait_wk", wk_cp[2])
        for b in range(NB):
            low = folded(1, 2 * (b + NB), 128)
            for step in w_terms(top[b], low, wk_s, 2 * b, (0, 1, 3, 5, 6)):
                step(keep)
        return []

    later = []

    def top_of_wv():
        _wait("wait_wv", wv_cp[0])
        steps = []
        for b in range(NB):
            steps += w_terms(transposed(2, b), None, wv_s, 2 * b, (2, 4))
        later.extend(_split(steps, (1, 3)))
        return later.pop(0)

    def rest_of_wv():
        _wait("wait_wv", wv_cp[1])
        steps = []
        for b in range(NB):
            steps += w_terms(transposed(2, b), transposed(2, b + NB), wv_s, 2 * b,
                             (0, 1, 3, 5, 6))
        later.extend(_split(steps, (1, 1, 3)))
        return later.pop(0)

    def second_tile():
        _wait("wait_x", xa_cp(1))
        later.extend(_split(x_terms(1, 1, route=route), (1, 1, 1, 1)))
        return later.pop(0)

    nxt = bind(later.pop, 0)
    keys(0, [rest_of_wk, fixed([]), top_of_wv, nxt, rest_of_wv], todo, never, ready)
    values(0, [nxt, nxt, fixed([]), second_tile, nxt, nxt, nxt], todo, never)
    _wait("wait_wq", wq_cp, wo_cp)

    def phase1(i, route):
        route = list(route)
        never = jnp.where(jnp.full((8, 128), i, jnp.int32) < 0, 1, 0)
        pl.when(i + 1 < NT)(lambda: _wait("wait_x", xa_cp(i + 1)))
        todo = []

        none = fixed([])
        w = [fixed(wo_terms(jnp.minimum(3 * (i - 1) + s, KH // 64 - 1))) for s in range(3)]
        q = _split(q_terms(i - 1), (1, 1))
        keys(i, [fixed(q[0]), fixed(q[1]), none, w[0], none, none, none], todo, never)
        x = _split(x_terms(jnp.minimum(i + 1, NT - 1), i + 1, route=route), (1, 1, 1))
        z = _split(z_total(), (1, 1, 1))
        x[2] = x[2] + w[1]()
        z[0] = z[0] + w[2]()
        values(i, [none] + [fixed(s) for s in x + z], todo, never)
        return tuple(route)

    route = lax.fori_loop(1, NT, phase1, tuple(route))

    for step in q_terms(NB - 1):
        step(keep)

    best = jnp.max(route[0], axis=0, keepdims=True)
    idx = jnp.min(jnp.where(route[0] == best, route[1], S - 1))
    first = idx // T
    slab = pl.ds(pl.multiple_of((idx // 16) * 16, 16), 16)
    sel = lax.broadcasted_iota(jnp.int32, (16, D), 0) == idx % 16
    _wait("wait_ffn", *ffn_cp)

    def x_column():
        def step(k, pin):
            cols = slice(128 * k, 128 * k + 128)
            row = jnp.where(sel[:, cols], pin(xa[slab, cols].astype(F32)), 0.0)
            row = jnp.sum(row, axis=0, keepdims=True)
            xcol[cols, :] = jnp.broadcast_to(row, (128, 128)).T
        return [bind(step, k) for k in range(D // 128)]

    def fold8(x):
        return jnp.sum(x.reshape(x.shape[0] // 8, 8, 128), axis=0)

    def ffn_steps(i, y):
        st = {}
        part = _ds(i * FC, FC, 128)
        wg_i, wu_i, wd_i = wg.at[:, part], wu.at[:, part], wd.at[part]

        def up(j, k, pin):
            f = pl.ds(j * 128, 128)
            rows = slice(64 * k, 64 * k + 64)
            xc = xcol[rows, :]
            a = fold8(wg_i[rows, f].astype(F32) * xc)
            u = fold8(wu_i[rows, f].astype(F32) * xc)
            if k > 0:
                a, u = pin(st["a"]) + a, pin(st["u"]) + u
            st["a"], st["u"] = a, u
            token = a + u if BACK else None
            if k == D // 64 - 1:
                a = jnp.sum(a, axis=0, keepdims=True)
                u = jnp.sum(u, axis=0, keepdims=True)
                st["h"] = jnp.broadcast_to(a * jax.nn.sigmoid(a) * u, (128, 128)).T
            return token

        def down(j, n, pin):
            w = wd_i[j * 128:j * 128 + 128, 128 * n:128 * n + 128].astype(F32)
            y[n] = pin(y[n]) + fold8(w * st["h"])
            return y[n] if BACK else None

        steps = []
        for j in range(FC // 128):
            steps += [bind(up, j, k) for k in range(D // 64)]
            steps += [bind(down, j, n) for n in range(D // 128)]
        return steps

    def phase2(i, y):
        y = list(y)
        t = (first + i) % NT
        never = jnp.where(jnp.full((8, 128), i, jnp.int32) < 0, 1, 0)
        o = [[[], []], [[], []]]
        todo = []

        def attend(g, dst, ph, rden, pin):
            num = jnp.dot(_unpack(pin(kvt[32 * g:32 * g + 32, :])), ph,
                          preferred_element_type=F32)
            scale = jnp.concatenate(
                [jnp.broadcast_to(rden[0:1, :], (DH, TH)),
                 jnp.broadcast_to(rden[1:2, :], (DH, TH))], axis=0)
            dst.append(num * scale)

        def query(g, dst, p, pin):
            ph = _features(p, pin)
            z = zb[128 * g:128 * g + 128, :]
            dn = [a * jnp.tile(z[8 * k:8 * k + 8, :], (1, TH // 128)) for k, a in enumerate(ph)]
            rden = _recip(_allreduce(jnp.add, dn) + 1e-6)
            todo.append(bind(attend, g, dst, jnp.concatenate(ph, axis=0).astype(BF16), rden))

        def emit_q(r, n, p):
            todo.extend(bind(query, r * KH // 64 + q, o[n][1 - r], p[64 * q:64 * q + 64, :])
                        for q in range(KH // 64))

        ffn = _split(ffn_steps(i, y), FFN_SHARES)
        plan = [fixed(x_column())] + [fixed(s) for s in ffn]
        due = []
        _strassen(staged(bind(project, wq_s, t), plan[:7], todo, never, due), emit_q)

        class Quad:
            def __init__(self, n):
                self.n = n

            def __getitem__(self, r):
                return jnp.concatenate(o[self.n][r], axis=0)

        def prod_o(n, due, never):
            w = _after(wo_s[n * (KH // 2):(n + 1) * (KH // 2), :], due, never, 1)
            return lax.dot_general(_LHS[n]([Quad(0), Quad(1)]).astype(BF16), _unpack(w),
                                   TN_DIMS, preferred_element_type=F32)

        def emit_o(n, c, a):
            gt = jnp.tile(gate[_ds(t * T + n * TH, TH), :], (1, KH // 128))
            b = xa[_ds(t * T + n * TH, TH), c * KH:(c + 1) * KH].astype(F32)
            outb[_ds(t * T + n * TH, TH), c * KH:(c + 1) * KH] = (
                gt * a + (1.0 - gt) * b).astype(BF16)
            out_cp(t, n, c, i).start()

        _strassen_diag(staged(prod_o, plan[7:], todo, never, due), emit_o)
        return tuple(y)

    y = lax.fori_loop(0, NT, phase2, (jnp.zeros((8, 128), F32),) * (D // 128))

    _wait("wait_out", *[out_cp(0, r, c, 0) for r in range(2) for c in range(2)])
    y = jnp.sum(jnp.concatenate(y, axis=1), axis=0, keepdims=True) * jax.nn.sigmoid(best)
    xsl = xa[slab, :].astype(F32)
    upd = (xsl + y).astype(BF16).astype(F32) - xsl
    gt = jnp.tile(gate[slab, :], (1, D // 128))
    old = outb[slab, :].astype(F32)
    outb[slab, :] = jnp.where(sel, old + (1.0 - gt) * upd, old).astype(BF16)
    fix_cp = pltpu.make_async_copy(outb.at[slab], out_hbm.at[slab], sem_x.at[NT])
    fix_cp.start()
    _wait("wait_out", fix_cp,
          *[out_cp(i, r, c, i) for i in range(1, NT) for r in range(2) for c in range(2)])


@jax.jit
def pallas_gated_mix__linear_kernel_hedgehog__moe_arch_mod__prompt_kernel(
    A_x, A_wqkv, A_w_phi, A_wo, B_x, B_w_r, B_w_gate, B_w_up, B_w_down, gate_w,
):
    del B_x
    hbm = pl.BlockSpec(memory_space=pl.ANY)
    vmem = pl.BlockSpec(memory_space=pltpu.VMEM)
    out = pl.pallas_call(
        _kernel,
        out_shape=jax.ShapeDtypeStruct((S, D), BF16),
        in_specs=[hbm, hbm, hbm, hbm, vmem, hbm, hbm, hbm, vmem],
        out_specs=hbm,
        scratch_shapes=[
            pltpu.VMEM((S, D), BF16),
            pltpu.VMEM((D, 3 * D), BF16),
            pltpu.VMEM((D, DH), BF16),
            pltpu.VMEM((D, D), BF16),
            pltpu.VMEM((D, F), BF16),
            pltpu.VMEM((D, F), BF16),
            pltpu.VMEM((F, D), BF16),
            pltpu.VMEM((7 * WR, KH), U32),
            pltpu.VMEM((7 * WR, KH), U32),
            pltpu.VMEM((7 * WR, KH), U32),
            pltpu.VMEM((7 * KH // 2, KH), U32),
            pltpu.VMEM(((NT + 1) * 7 * TH // 2, KH), U32),
            pltpu.VMEM((D // 2, 128), U32),
            pltpu.VMEM((D // 2, T), U32),
            pltpu.VMEM((D, T), U32),
            pltpu.VMEM((D, 128), F32),
            pltpu.VMEM((D // 2, 128), U32),
            pltpu.VMEM((2 * D, 128), F32),
            pltpu.VMEM((2 * D, 128), F32),
            pltpu.VMEM((S, 128), F32),
            pltpu.VMEM((S, D), BF16),
            pltpu.VMEM((D, 128), F32),
            pltpu.SemaphoreType.DMA((NT + 1,)),
            pltpu.SemaphoreType.DMA((6,)),
            pltpu.SemaphoreType.DMA((7,)),
            pltpu.SemaphoreType.DMA((4 * NT,)),
        ],
        compiler_params=pltpu.CompilerParams(vmem_limit_bytes=110 * 2**20),
    )(A_x.reshape(S, D), A_wqkv, A_w_phi.reshape(H * DH, DH), A_wo,
      B_w_r, B_w_gate, B_w_up, B_w_down, gate_w)
    return out.reshape(1, S, D)
```

```python
import functools

import jax
import jax.numpy as jnp
from jax import lax
from jax.experimental import pallas as pl
from jax.experimental.pallas import tpu as pltpu

S, D, H, DH, F = 2048, 1024, 32, 32, 3584
T = 512
NT = S // T
TH, KH = T // 2, D // 2
WR = KH // 2
NB = KH // 128
FC = F // NT
SCOPES = False
CFG = dict(ffn=(0, 4, 0, 2, 0, 2, 0, 0, 2, 4, 1, 2, 2, 2), back=(1, 0, 1, 1, 1, 0, 1, 1, 1, 1, 1, 1, 0, 1), upk=64,
           q=(0, 1, 0, 0, 0, 1, 0), w=(11, 10, 9), x=(0, 0, 0, 0, 0, 0, 0, 0, 1, 1, 2, 0, 0, 0), z=(0, 0, 1, 0, 1, 0, 1), kback=0,
           kback0=1, x0=(1, 1), wv_top=(1, 3), wv_rest=(1, 1, 3), x1=(1, 1, 1, 1))
LOG2E = 1.4426950408889634
F32, BF16, U32 = jnp.float32, jnp.bfloat16, jnp.uint32
NT_DIMS = (((1,), (1,)), ((), ()))
TN_DIMS = (((0,), (0,)), ((), ()))
bind = functools.partial


def _tree(op, xs):
    xs = list(xs)
    while len(xs) > 1:
        xs = [op(xs[i], xs[i + 1]) if i + 1 < len(xs) else xs[i]
              for i in range(0, len(xs), 2)]
    return xs[0]


def _allreduce(op, xs):
    r = _tree(op, xs)
    r = op(r, pltpu.roll(r, 4, 0))
    return op(r, pltpu.roll(r, 2, 0))


def _recip(x):
    r = pl.reciprocal(x, approx=True)
    return r * (2.0 - x * r)


def _features(p, pin):
    rows = [p[8 * i:8 * i + 8, :] for i in range(8)]
    rows[0] = pin(rows[0])
    mx = _allreduce(jnp.maximum, rows)
    mn = _allreduce(jnp.minimum, rows)
    ep = [jnp.exp2(r - mx) for r in rows]
    en = [jnp.exp2(mn - r) for r in rows]
    rp = _recip(_allreduce(jnp.add, ep))
    rn = _recip(_allreduce(jnp.add, en))
    return [e * rp for e in ep] + [e * rn for e in en]


def _pack(x):
    return pltpu.bitcast(x.astype(BF16), U32)


def _unpack(x):
    return pltpu.bitcast(x, BF16)


_LHS = [lambda a: a[0][0] + a[1][1], lambda a: a[1][0] + a[1][1], lambda a: a[0][0],
        lambda a: a[1][1], lambda a: a[0][0] + a[0][1], lambda a: a[1][0] - a[0][0],
        lambda a: a[0][1] - a[1][1]]
_RHS = [lambda b: b[0][0] + b[1][1], lambda b: b[0][0], lambda b: b[0][1] - b[1][1],
        lambda b: b[1][0] - b[0][0], lambda b: b[1][1], lambda b: b[0][0] + b[0][1],
        lambda b: b[1][0] + b[1][1]]


def _strassen(prod, emit):
    m3 = prod(2)
    m5 = prod(4)
    emit(0, 1, m3 + m5)
    m2 = prod(1)
    m4 = prod(3)
    emit(1, 0, m2 + m4)
    m1 = prod(0)
    s1 = m4 - m5 + m1
    s2 = m3 - m2 + m1
    emit(0, 0, s1 + prod(6))
    emit(1, 1, s2 + prod(5))


def _strassen_diag(prod, emit):
    m3 = prod(2)
    m4 = prod(3)
    m1 = prod(0)
    m5 = prod(4)
    emit(0, 1, m3 + m5)
    emit(0, 0, m1 + m4 - m5 + prod(6))
    m2 = prod(1)
    emit(1, 0, m2 + m4)
    emit(1, 1, m1 + m3 - m2 + prod(5))


def _shadow(m, steps, never, due):
    rows, cols = m.shape[0] // 8, m.shape[1] // 128
    for s, step in enumerate(steps):
        p = rows * cols * s // len(steps)
        r, c = 8 * (p % rows), 128 * (p // rows)
        slab = m[r:r + 8, c:c + 128]

        def pin(v, slab=slab):
            reps = (v.shape[0] // 8, v.shape[1] // 128)
            other = slab if v.dtype == F32 else pltpu.bitcast(slab, v.dtype)
            return jnp.where(jnp.tile(never, reps) != 0, jnp.tile(other, reps), v)

        token = step(pin)
        if token is not None:
            due.append(token)
    return m


def _after(w, due, never, axis):
    if not due:
        return w
    unit = (8, 128)[axis]
    parts = jnp.split(w, w.shape[axis] // unit, axis=axis)
    for s, token in enumerate(due):
        p = len(parts) * s // len(due)
        head = jnp.where(never != 0, pltpu.bitcast(token, U32), parts[p][:8, :128])
        if axis == 0:
            parts[p] = jnp.concatenate([head, parts[p][:, 128:]], axis=1)
        else:
            parts[p] = jnp.concatenate([head, parts[p][8:, :]], axis=0)
    due.clear()
    return jnp.concatenate(parts, axis=axis)


def _split(steps, shares):
    out, done, total = [], 0, 0
    for s in shares:
        total += s
        end = len(steps) * total // sum(shares)
        out.append(steps[done:end])
        done = end
    return out


def _start(*cps):
    def step(i, carry):
        for n, cp in enumerate(cps):
            pl.when(i == n)(cp.start)
        return carry

    lax.fori_loop(0, len(cps), step, 0)


def _wait(name, *cps):
    if SCOPES:
        with jax.named_scope(name):
            for cp in cps:
                cp.wait()
    else:
        for cp in cps:
            cp.wait()


def _ds(start, size, mult=None):
    if isinstance(start, int):
        return pl.ds(start, size)
    return pl.ds(pl.multiple_of(start, mult or size), size)


def _kernel(xa_hbm, wqkv_hbm, wphi_hbm, wo_hbm, wr_hbm, wg_hbm, wu_hbm,
            wd_hbm, gw_hbm, out_hbm,
            xa, wqkv, wphi, wo, wg, wu, wd, wq_s, wk_s, wv_s, wo_s, xs, pt, vt, phi, kvacc, kvt, zacc,
            zb, gate, outb, xcol, wr_ref, gw_ref, sem_x, sem_w, sem_m, sem_o):
    def xa_cp(i):
        return pltpu.make_async_copy(xa_hbm.at[_ds(i * T, T)], xa.at[_ds(i * T, T)], sem_x.at[i])

    def w_cp(start, size, sem):
        cols = _ds(start, size)
        return pltpu.make_async_copy(wqkv_hbm.at[:, cols], wqkv.at[:, cols], sem_w.at[sem])

    def x0_cp(h):
        rows = pl.ds(h * TH, TH)
        return pltpu.make_async_copy(xa_hbm.at[rows], xa.at[rows], sem_m.at[h])

    wk_cp = [w_cp(D, KH // 2, 0), w_cp(D + KH // 2, KH // 2, 1), w_cp(D + KH, KH, 2)]
    wv_cp = [w_cp(2 * D, KH, 3), w_cp(2 * D + KH, KH, 4)]
    wq_cp = w_cp(0, D, 5)
    phi_cp = [pltpu.make_async_copy(wphi_hbm.at[pl.ds(h * KH, KH)], wphi.at[pl.ds(h * KH, KH)],
                                    sem_m.at[2 + 5 * h]) for h in range(2)]
    vec_cp = [pltpu.make_async_copy(wr_hbm, wr_ref, sem_m.at[8]),
              pltpu.make_async_copy(gw_hbm, gw_ref, sem_m.at[9])]
    wo_cp = pltpu.make_async_copy(wo_hbm, wo, sem_m.at[3])
    ffn_cp = [pltpu.make_async_copy(wg_hbm, wg, sem_m.at[4]),
              pltpu.make_async_copy(wu_hbm, wu, sem_m.at[5]),
              pltpu.make_async_copy(wd_hbm, wd, sem_m.at[6])]

    def out_cp(t, r, c, slot):
        blk = (_ds(t * T + r * TH, TH), pl.ds(c * KH, KH))
        return pltpu.make_async_copy(outb.at[blk], out_hbm.at[blk], sem_o.at[slot * 4 + r * 2 + c])

    zb[0:8, :] = jnp.zeros((8, 128), F32)
    _start(phi_cp[0], x0_cp(1), wk_cp[0], wk_cp[1], x0_cp(0))

    er = lax.broadcasted_iota(jnp.int32, (128, DH), 0)
    ec = lax.broadcasted_iota(jnp.int32, (128, DH), 1)
    expand = jnp.where((er % 64) // 2 == ec, 1.0, 0.0).astype(BF16)
    pr = lax.broadcasted_iota(jnp.int32, (128, 128), 0)
    pc = lax.broadcasted_iota(jnp.int32, (128, 128), 1)
    diag = pc // DH == 2 * (pr // 64) + pr % 2
    kr = lax.broadcasted_iota(jnp.int32, (64, 128), 0)
    kc = lax.broadcasted_iota(jnp.int32, (64, 128), 1)
    same_head = kr // DH == kc % 2
    kvacc[...] = jnp.zeros_like(kvacc)
    zacc[...] = jnp.zeros_like(zacc)
    def folded(j, u, n):
        w = wqkv[:, _ds(j * D + (u // 2) * 128, 128)]
        return lax.dot_general(_unpack(pt[_ds(u * 32, n // 2), :]), w, NT_DIMS,
                               preferred_element_type=F32) * LOG2E

    def transposed(j, g):
        return wqkv[:, _ds(j * D + g * 128, 128)].T

    def keep(v):
        return v

    def w_terms(r1, r2, dst, u, terms=range(7)):
        dst = dst.at[_ds(u * 32, 6 * WR + r1.shape[0] // 2, 32)]

        def step(h, pin):
            rows = slice(16 * h, 16 * h + 16)
            a = r1[rows, :].astype(F32)
            top = [pin(a[:, :KH]), a[:, KH:]]
            low = None
            if r2 is not None:
                a = r2[rows, :].astype(F32)
                low = [a[:, :KH], pin(a[:, KH:])]
            for n in terms:
                dst[pl.ds(n * WR + h * 8, 8), :] = _pack(_LHS[n]([top, low]))
        return [bind(step, h) for h in range(r1.shape[0] // 16)]

    def wo_terms(u):
        src = wo.at[_ds(u * 64, KH + 64, 64)]
        dst = wo_s.at[_ds(u * 32, 6 * (KH // 2) + 32, 32)]

        def step(h, pin):
            r1 = src[pl.ds(KH + h * 16, 16), :].astype(F32)
            r2 = src[pl.ds(h * 16, 16), :].astype(F32)
            quad = [[pin(r1[:, :KH]), r1[:, KH:]], [r2[:, :KH], pin(r2[:, KH:])]]
            for n in range(7):
                dst[pl.ds(n * (KH // 2) + h * 8, 8), :] = _pack(_RHS[n](quad))
        return [bind(step, h) for h in range(4)]

    def x_terms(i, slot, terms=range(7), route=None):
        src = xa.at[_ds(i * T, T)]
        dst = xs.at[_ds(slot * 7 * (TH // 2), 7 * (TH // 2))]
        mix = gate.at[_ds(i * T, T)]

        def step(h, pin):
            x2 = src[pl.ds(TH + h * 16, 16), :].astype(F32)
            quad = [[None, x2[:, :KH]], [None, pin(x2[:, KH:])]]
            if set(terms) - {2, 4}:
                x1 = src[pl.ds(h * 16, 16), :].astype(F32)
                quad[0][0], quad[1][0] = pin(x1[:, :KH]), x1[:, KH:]
            for n in terms:
                dst[pl.ds(n * (TH // 2) + h * 8, 8), :] = _pack(_RHS[n](quad))
            for c in range(2) if route else ():
                row = TH * c + 16 * h
                g = quad[0][c] * gw[:, :KH] + quad[1][c] * gw[:, KH:]
                mix[row:row + 16, :] = jnp.broadcast_to(
                    jax.nn.sigmoid(jnp.sum(g, axis=-1, keepdims=True)), (16, 128))
                r = quad[0][c] * wr[:, :KH] + quad[1][c] * wr[:, KH:]
                r = jnp.sum(r, axis=-1, keepdims=True).astype(BF16).astype(F32)
                tok = i * T + row + lax.broadcasted_iota(jnp.int32, (16, 1), 0)
                best, where = route
                better = (r > best) | ((r == best) & (tok < where))
                route[:] = jnp.where(better, r, best), jnp.where(better, tok, where)
        return [bind(step, h) for h in range(TH // 16)]

    def z_total():
        def step(g, pin):
            rows = slice(128 * g, 128 * g + 128)
            z = jnp.sum(pin(zacc[rows, :]), axis=-1, keepdims=True)
            zb[rows, :] = jnp.broadcast_to(z, (128, 128))
        return [bind(step, g) for g in range(H // 2)]

    def project(w_s, i, n, due, never):
        w = _after(w_s[n * WR:(n + 1) * WR, :], due, never, 0)
        return lax.dot_general(_unpack(w),
                               _unpack(xs[_ds((i * 7 + n) * (TH // 2), TH // 2), :]),
                               NT_DIMS, preferred_element_type=F32)

    def staged(f, plan, todo, never, due=None):
        plan = list(plan)
        due = [] if due is None else due

        def prod(n):
            steps = plan.pop(0)()
            follow = list(todo)
            todo.clear()
            return _shadow(_shadow(f(n, due, never), follow, never, due), steps, never, due)
        return prod

    def keys(i, plan, todo, never, ready=None):
        def step(g, n, p, pin):
            ph = _features(p, pin)
            zs = [_tree(jnp.add, [a[:, 128 * l:128 * l + 128] for l in range(TH // 128)])
                  for a in ph]
            zacc[128 * g:128 * g + 128, :] += jnp.concatenate(zs, axis=0)
            phi[64 * g:64 * g + 64, n * TH:(n + 1) * TH] = _pack(jnp.concatenate(ph, axis=0))
            return zs[0] + zs[8] if CFG['kback0' if isinstance(i, int) else 'kback'] else None

        def emit(r, n, p):
            todo.extend(bind(step, r * KH // 64 + q, n, p[64 * q:64 * q + 64, :])
                        for q in range(KH // 64))
        prod = staged(bind(project, wk_s, i), plan, todo, never)
        _strassen(lambda n: ready[n] if ready and n in ready else prod(n), emit)

    def values(i, plan, todo, never):
        def emit(r, n, v):
            vt[r * KH // 2:(r + 1) * KH // 2, n * TH:(n + 1) * TH] = _pack(v)
        _strassen(staged(bind(project, wv_s, i), plan, todo, never), emit)
        for g in range(H // 2):
            acc = kvacc[64 * g:64 * g + 64, :] + lax.dot_general(
                _unpack(vt[32 * g:32 * g + 32, :]), _unpack(phi[64 * g:64 * g + 64, :]),
                NT_DIMS, preferred_element_type=F32)
            kvacc[64 * g:64 * g + 64, :] = acc
            kvt[32 * g:32 * g + 32, :] = _pack(jnp.where(same_head, acc, 0.0))

    def q_terms(b):
        return w_terms(folded(0, 2 * b, 128), folded(0, 2 * (b + NB), 128), wq_s, 2 * b)

    def fixed(steps):
        return lambda: steps

    never = pltpu.bitcast(zb[0:8, :], jnp.int32)
    _wait("wait_phi", phi_cp[0])
    _start(*vec_cp, phi_cp[1], wk_cp[2], *wv_cp, xa_cp(1), wq_cp, wo_cp, *[xa_cp(i) for i in range(2, NT)], *ffn_cp)

    def feature_maps(h):
        for g in range(h * NB, (h + 1) * NB):
            p = lax.dot_general(expand, wphi[g * 128:(g + 1) * 128, :], NT_DIMS,
                                preferred_element_type=F32)
            pt[g * 64:(g + 1) * 64, :] = _pack(jnp.where(diag, p, 0.0))

    feature_maps(0)
    _wait("wait_x", x0_cp(1))
    for step in x_terms(0, 0, (2, 4)):
        step(keep)
    route = [jnp.full((16, 1), -jnp.inf, F32), jnp.zeros((16, 1), jnp.int32)]
    top, ready = [], {2: [], 4: []}
    for h in range(2):
        if h == 0:
            _wait("wait_wk", wk_cp[0])
            x0 = [[], []]
        else:
            _wait("wait_wk", wk_cp[1], x0_cp(0), *vec_cp, phi_cp[1])
            feature_maps(1)
            gw = gw_ref[...].astype(F32).reshape(1, D)
            wr = wr_ref[...].astype(F32).reshape(1, D)
            x0 = _split(x_terms(0, 0, (0, 1, 3, 5, 6), route), CFG['x0'])
        for b in (2 * h, 2 * h + 1):
            top.append(folded(1, 2 * b, 128))
            for step in w_terms(top[b], None, wk_s, 2 * b, (2, 4)):
                step(keep)
        for n, steps in zip(ready, x0):
            ready[n].append(_shadow(lax.dot_general(
                _unpack(wk_s[n * WR + h * 128:n * WR + (h + 1) * 128, :]),
                _unpack(xs[n * (TH // 2):(n + 1) * (TH // 2), :]),
                NT_DIMS, preferred_element_type=F32), steps, never, []))
    ready = {n: jnp.concatenate(m, axis=0) for n, m in ready.items()}
    todo = []

    def rest_of_wk():
        _wait("wait_wk", wk_cp[2])
        for b in range(NB):
            low = folded(1, 2 * (b + NB), 128)
            for step in w_terms(top[b], low, wk_s, 2 * b, (0, 1, 3, 5, 6)):
                step(keep)
        return []

    later = []

    def top_of_wv():
        _wait("wait_wv", wv_cp[0])
        steps = []
        for b in range(NB):
            steps += w_terms(transposed(2, b), None, wv_s, 2 * b, (2, 4))
        later.extend(_split(steps, CFG['wv_top']))
        return later.pop(0)

    def rest_of_wv():
        _wait("wait_wv", wv_cp[1])
        steps = []
        for b in range(NB):
            steps += w_terms(transposed(2, b), transposed(2, b + NB), wv_s, 2 * b,
                             (0, 1, 3, 5, 6))
        later.extend(_split(steps, CFG['wv_rest']))
        return later.pop(0)

    def second_tile():
        _wait("wait_x", xa_cp(1))
        later.extend(_split(x_terms(1, 1, route=route), CFG['x1']))
        return later.pop(0)

    nxt = bind(later.pop, 0)
    keys(0, [rest_of_wk, fixed([]), top_of_wv, nxt, rest_of_wv], todo, never, ready)
    values(0, [nxt, nxt, fixed([]), second_tile, nxt, nxt, nxt], todo, never)
    _wait("wait_wq", wq_cp, wo_cp)

    def phase1(i, route):
        route = list(route)
        never = jnp.where(jnp.full((8, 128), i, jnp.int32) < 0, 1, 0)
        pl.when(i + 1 < NT)(lambda: _wait("wait_x", xa_cp(i + 1)))
        todo = []

        plan = _split(x_terms(jnp.minimum(i + 1, NT - 1), i + 1, route=route), CFG['x'])
        for n, steps in enumerate(_split(z_total(), CFG['z'])):
            plan[7 + n] += steps
        for n, slot in enumerate(CFG['w']):
            plan[slot] += wo_terms(jnp.minimum(3 * (i - 1) + n, KH // 64 - 1))
        q = []

        def with_q(n):
            if CFG['q'][n] and not q:
                q.extend(_split(q_terms(i - 1), CFG['q']))
            return (q[n] if q else []) + plan[n]

        keys(i, [bind(with_q, n) for n in range(7)], todo, never)
        values(i, [fixed(s) for s in plan[7:]], todo, never)
        return tuple(route)

    route = lax.fori_loop(1, NT, phase1, tuple(route))

    for step in q_terms(NB - 1):
        step(keep)

    best = jnp.max(route[0], axis=0, keepdims=True)
    idx = jnp.min(jnp.where(route[0] == best, route[1], S - 1))
    first = idx // T
    slab = pl.ds(pl.multiple_of((idx // 16) * 16, 16), 16)
    sel = lax.broadcasted_iota(jnp.int32, (16, D), 0) == idx % 16
    _wait("wait_ffn", *ffn_cp)

    def x_column():
        def step(k, pin):
            cols = slice(128 * k, 128 * k + 128)
            row = jnp.where(sel[:, cols], pin(xa[slab, cols].astype(F32)), 0.0)
            row = jnp.sum(row, axis=0, keepdims=True)
            xcol[cols, :] = jnp.broadcast_to(row, (128, 128)).T
        return [bind(step, k) for k in range(D // 128)]

    def fold8(x):
        return jnp.sum(x.reshape(x.shape[0] // 8, 8, 128), axis=0)

    def ffn_steps(i, y):
        st = {}
        part = _ds(i * FC, FC, 128)
        wg_i, wu_i, wd_i = wg.at[:, part], wu.at[:, part], wd.at[part]

        def up(j, k, pin):
            f = pl.ds(j * 128, 128)
            rows = slice(CFG['upk'] * k, CFG['upk'] * (k + 1))
            xc = xcol[rows, :]
            a = fold8(wg_i[rows, f].astype(F32) * xc)
            u = fold8(wu_i[rows, f].astype(F32) * xc)
            if k > 0:
                a, u = pin(st["a"]) + a, pin(st["u"]) + u
            st["a"], st["u"] = a, u
            token = a + u
            if k == D // CFG['upk'] - 1:
                a = jnp.sum(a, axis=0, keepdims=True)
                u = jnp.sum(u, axis=0, keepdims=True)
                st["h"] = jnp.broadcast_to(a * jax.nn.sigmoid(a) * u, (128, 128)).T
            return token

        def down(j, n, pin):
            w = wd_i[j * 128:j * 128 + 128, 128 * n:128 * n + 128].astype(F32)
            y[n] = pin(y[n]) + fold8(w * st["h"])
            return y[n]

        steps = []
        for j in range(FC // 128):
            steps += [bind(up, j, k) for k in range(D // CFG['upk'])]
            steps += [bind(down, j, n) for n in range(D // 128)]
        return steps

    def phase2(i, y):
        y = list(y)
        t = (first + i) % NT
        never = jnp.where(jnp.full((8, 128), i, jnp.int32) < 0, 1, 0)
        o = [[[], []], [[], []]]
        todo = []

        def attend(g, dst, ph, rden, pin):
            num = jnp.dot(_unpack(pin(kvt[32 * g:32 * g + 32, :])), ph,
                          preferred_element_type=F32)
            scale = jnp.concatenate(
                [jnp.broadcast_to(rden[0:1, :], (DH, TH)),
                 jnp.broadcast_to(rden[1:2, :], (DH, TH))], axis=0)
            dst.append(num * scale)

        def query(g, dst, p, pin):
            ph = _features(p, pin)
            z = zb[128 * g:128 * g + 128, :]
            dn = [a * jnp.tile(z[8 * k:8 * k + 8, :], (1, TH // 128)) for k, a in enumerate(ph)]
            rden = _recip(_allreduce(jnp.add, dn) + 1e-6)
            todo.append(bind(attend, g, dst, jnp.concatenate(ph, axis=0).astype(BF16), rden))

        def emit_q(r, n, p):
            todo.extend(bind(query, r * KH // 64 + q, o[n][1 - r], p[64 * q:64 * q + 64, :])
                        for q in range(KH // 64))

        ffn = _split(ffn_steps(i, y), CFG['ffn'])
        quiet = lambda f: (lambda pin: (f(pin), None)[1])
        ffn = [p if b else [quiet(f) for f in p] for p, b in zip(ffn, CFG['back'])]
        plan = [fixed(s) for s in [x_column() + ffn[0]] + ffn[1:]]
        due = []
        _strassen(staged(bind(project, wq_s, t), plan[:7], todo, never, due), emit_q)

        class Quad:
            def __init__(self, n):
                self.n = n

            def __getitem__(self, r):
                return jnp.concatenate(o[self.n][r], axis=0)

        def prod_o(n, due, never):
            w = _after(wo_s[n * (KH // 2):(n + 1) * (KH // 2), :], due, never, 1)
            return lax.dot_general(_LHS[n]([Quad(0), Quad(1)]).astype(BF16), _unpack(w),
                                   TN_DIMS, preferred_element_type=F32)

        def emit_o(n, c, a):
            gt = jnp.tile(gate[_ds(t * T + n * TH, TH), :], (1, KH // 128))
            b = xa[_ds(t * T + n * TH, TH), c * KH:(c + 1) * KH].astype(F32)
            outb[_ds(t * T + n * TH, TH), c * KH:(c + 1) * KH] = (
                gt * a + (1.0 - gt) * b).astype(BF16)
            out_cp(t, n, c, i).start()

        _strassen_diag(staged(prod_o, plan[7:], todo, never, due), emit_o)
        return tuple(y)

    y = lax.fori_loop(0, NT, phase2, (jnp.zeros((8, 128), F32),) * (D // 128))

    _wait("wait_out", *[out_cp(0, r, c, 0) for r in range(2) for c in range(2)])
    y = jnp.sum(jnp.concatenate(y, axis=1), axis=0, keepdims=True) * jax.nn.sigmoid(best)
    xsl = xa[slab, :].astype(F32)
    upd = (xsl + y).astype(BF16).astype(F32) - xsl
    gt = jnp.tile(gate[slab, :], (1, D // 128))
    old = outb[slab, :].astype(F32)
    outb[slab, :] = jnp.where(sel, old + (1.0 - gt) * upd, old).astype(BF16)
    fix_cp = pltpu.make_async_copy(outb.at[slab], out_hbm.at[slab], sem_x.at[NT])
    fix_cp.start()
    _wait("wait_out", fix_cp,
          *[out_cp(i, r, c, i) for i in range(1, NT) for r in range(2) for c in range(2)])


@jax.jit
def pallas_gated_mix__linear_kernel_hedgehog__moe_arch_mod__prompt_kernel(
    A_x, A_wqkv, A_w_phi, A_wo, B_x, B_w_r, B_w_gate, B_w_up, B_w_down, gate_w,
):
    del B_x
    hbm = pl.BlockSpec(memory_space=pl.ANY)
    out = pl.pallas_call(
        _kernel,
        out_shape=jax.ShapeDtypeStruct((S, D), BF16),
        in_specs=[hbm] * 9,
        out_specs=hbm,
        scratch_shapes=[
            pltpu.VMEM((S, D), BF16),
            pltpu.VMEM((D, 3 * D), BF16),
            pltpu.VMEM((D, DH), BF16),
            pltpu.VMEM((D, D), BF16),
            pltpu.VMEM((D, F), BF16),
            pltpu.VMEM((D, F), BF16),
            pltpu.VMEM((F, D), BF16),
            pltpu.VMEM((7 * WR, KH), U32),
            pltpu.VMEM((7 * WR, KH), U32),
            pltpu.VMEM((7 * WR, KH), U32),
            pltpu.VMEM((7 * KH // 2, KH), U32),
            pltpu.VMEM(((NT + 1) * 7 * TH // 2, KH), U32),
            pltpu.VMEM((D // 2, 128), U32),
            pltpu.VMEM((D // 2, T), U32),
            pltpu.VMEM((D, T), U32),
            pltpu.VMEM((D, 128), F32),
            pltpu.VMEM((D // 2, 128), U32),
            pltpu.VMEM((2 * D, 128), F32),
            pltpu.VMEM((2 * D, 128), F32),
            pltpu.VMEM((S, 128), F32),
            pltpu.VMEM((S, D), BF16),
            pltpu.VMEM((D, 128), F32),
            pltpu.VMEM((D,), BF16),
            pltpu.VMEM((D,), BF16),
            pltpu.SemaphoreType.DMA((NT + 1,)),
            pltpu.SemaphoreType.DMA((6,)),
            pltpu.SemaphoreType.DMA((10,)),
            pltpu.SemaphoreType.DMA((4 * NT,)),
        ],
        compiler_params=pltpu.CompilerParams(vmem_limit_bytes=110 * 2**20),
    )(A_x.reshape(S, D), A_wqkv, A_w_phi.reshape(H * DH, DH), A_wo,
      B_w_r, B_w_gate, B_w_up, B_w_down, gate_w)
    return out.reshape(1, S, D)
```

```python
import functools

import jax
import jax.numpy as jnp
from jax import lax
from jax.experimental import pallas as pl
from jax.experimental.pallas import tpu as pltpu

S, D, H, DH, F = 2048, 1024, 32, 32, 3584
T = 512
NT = S // T
TH, KH = T // 2, D // 2
WR = KH // 2
NB = KH // 128
FC = F // NT
FFN_SHARES = (0, 4, 0, 2, 0, 2, 0, 0, 2, 4, 1, 2, 2, 2)
FFN_DEADLINE = (1, 0, 1, 1, 1, 0, 1, 1, 1, 1, 1, 1, 0, 1)
Q_SHARES = (0, 1, 0, 0, 0, 1, 0)
X_SHARES = (0, 0, 0, 0, 0, 0, 0, 0, 1, 1, 2, 0, 0, 0)
Z_SHARES = (0, 0, 0, 0, 0, 0, 0, 0, 0, 1, 0, 1, 0, 1)
WO_SLOTS = (11, 10, 9)
LOG2E = 1.4426950408889634
F32, BF16, U32 = jnp.float32, jnp.bfloat16, jnp.uint32
NT_DIMS = (((1,), (1,)), ((), ()))
TN_DIMS = (((0,), (0,)), ((), ()))
bind = functools.partial


def _tree(op, xs):
    xs = list(xs)
    while len(xs) > 1:
        xs = [op(xs[i], xs[i + 1]) if i + 1 < len(xs) else xs[i]
              for i in range(0, len(xs), 2)]
    return xs[0]


def _allreduce(op, xs):
    r = _tree(op, xs)
    r = op(r, pltpu.roll(r, 4, 0))
    return op(r, pltpu.roll(r, 2, 0))


def _recip(x):
    r = pl.reciprocal(x, approx=True)
    return r * (2.0 - x * r)


def _features(p, pin):
    rows = [p[8 * i:8 * i + 8, :] for i in range(8)]
    rows[0] = pin(rows[0])
    mx = _allreduce(jnp.maximum, rows)
    mn = _allreduce(jnp.minimum, rows)
    ep = [jnp.exp2(r - mx) for r in rows]
    en = [jnp.exp2(mn - r) for r in rows]
    rp = _recip(_allreduce(jnp.add, ep))
    rn = _recip(_allreduce(jnp.add, en))
    return [e * rp for e in ep] + [e * rn for e in en]


def _pack(x):
    return pltpu.bitcast(x.astype(BF16), U32)


def _unpack(x):
    return pltpu.bitcast(x, BF16)


_LHS = [lambda a: a[0][0] + a[1][1], lambda a: a[1][0] + a[1][1], lambda a: a[0][0],
        lambda a: a[1][1], lambda a: a[0][0] + a[0][1], lambda a: a[1][0] - a[0][0],
        lambda a: a[0][1] - a[1][1]]
_RHS = [lambda b: b[0][0] + b[1][1], lambda b: b[0][0], lambda b: b[0][1] - b[1][1],
        lambda b: b[1][0] - b[0][0], lambda b: b[1][1], lambda b: b[0][0] + b[0][1],
        lambda b: b[1][0] + b[1][1]]


def _strassen(prod, emit):
    m3 = prod(2)
    m5 = prod(4)
    emit(0, 1, m3 + m5)
    m2 = prod(1)
    m4 = prod(3)
    emit(1, 0, m2 + m4)
    m1 = prod(0)
    s1 = m4 - m5 + m1
    s2 = m3 - m2 + m1
    emit(0, 0, s1 + prod(6))
    emit(1, 1, s2 + prod(5))


def _strassen_diag(prod, emit):
    m3 = prod(2)
    m4 = prod(3)
    m1 = prod(0)
    m5 = prod(4)
    emit(0, 1, m3 + m5)
    emit(0, 0, m1 + m4 - m5 + prod(6))
    m2 = prod(1)
    emit(1, 0, m2 + m4)
    emit(1, 1, m1 + m3 - m2 + prod(5))


def _shadow(m, steps, never, due):
    rows, cols = m.shape[0] // 8, m.shape[1] // 128
    for s, step in enumerate(steps):
        p = rows * cols * s // len(steps)
        r, c = 8 * (p % rows), 128 * (p // rows)
        slab = m[r:r + 8, c:c + 128]

        def pin(v, slab=slab):
            reps = (v.shape[0] // 8, v.shape[1] // 128)
            other = slab if v.dtype == F32 else pltpu.bitcast(slab, v.dtype)
            return jnp.where(jnp.tile(never, reps) != 0, jnp.tile(other, reps), v)

        token = step(pin)
        if token is not None:
            due.append(token)
    return m


def _after(w, due, never, axis):
    if not due:
        return w
    unit = (8, 128)[axis]
    parts = jnp.split(w, w.shape[axis] // unit, axis=axis)
    for s, token in enumerate(due):
        p = len(parts) * s // len(due)
        head = jnp.where(never != 0, pltpu.bitcast(token, U32), parts[p][:8, :128])
        if axis == 0:
            parts[p] = jnp.concatenate([head, parts[p][:, 128:]], axis=1)
        else:
            parts[p] = jnp.concatenate([head, parts[p][8:, :]], axis=0)
    due.clear()
    return jnp.concatenate(parts, axis=axis)


def _split(steps, shares):
    out, done, total = [], 0, 0
    for s in shares:
        total += s
        end = len(steps) * total // sum(shares)
        out.append(steps[done:end])
        done = end
    return out


def _start(*cps):
    def step(i, carry):
        for n, cp in enumerate(cps):
            pl.when(i == n)(cp.start)
        return carry

    lax.fori_loop(0, len(cps), step, 0)


def _wait(*cps):
    for cp in cps:
        cp.wait()


def _ds(start, size, mult=None):
    if isinstance(start, int):
        return pl.ds(start, size)
    return pl.ds(pl.multiple_of(start, mult or size), size)


def _kernel(xa_hbm, wqkv_hbm, wphi_hbm, wo_hbm, wr_hbm, wg_hbm, wu_hbm,
            wd_hbm, gw_hbm, out_hbm,
            xa, wqkv, wphi, wo, wg, wu, wd, wq_s, wk_s, wv_s, wo_s, xs, pt, vt, phi,
            kvacc, kvt, zacc, zb, gate, outb, xcol, wr_ref, gw_ref,
            sem_x, sem_w, sem_m, sem_o):
    def xa_cp(i):
        return pltpu.make_async_copy(xa_hbm.at[_ds(i * T, T)], xa.at[_ds(i * T, T)], sem_x.at[i])

    def w_cp(start, size, sem):
        cols = pl.ds(start, size)
        return pltpu.make_async_copy(wqkv_hbm.at[:, cols], wqkv.at[:, cols], sem_w.at[sem])

    def x0_cp(h):
        rows = pl.ds(h * TH, TH)
        return pltpu.make_async_copy(xa_hbm.at[rows], xa.at[rows], sem_m.at[h])

    wk_cp = [w_cp(D, KH // 2, 0), w_cp(D + KH // 2, KH // 2, 1), w_cp(D + KH, KH, 2)]
    wv_cp = [w_cp(2 * D, KH, 3), w_cp(2 * D + KH, KH, 4)]
    wq_cp = w_cp(0, D, 5)
    phi_cp = [pltpu.make_async_copy(wphi_hbm.at[pl.ds(h * KH, KH)], wphi.at[pl.ds(h * KH, KH)],
                                    sem_m.at[2 + 5 * h]) for h in range(2)]
    vec_cp = [pltpu.make_async_copy(wr_hbm, wr_ref, sem_m.at[8]),
              pltpu.make_async_copy(gw_hbm, gw_ref, sem_m.at[9])]
    wo_cp = pltpu.make_async_copy(wo_hbm, wo, sem_m.at[3])
    ffn_cp = [pltpu.make_async_copy(wg_hbm, wg, sem_m.at[4]),
              pltpu.make_async_copy(wu_hbm, wu, sem_m.at[5]),
              pltpu.make_async_copy(wd_hbm, wd, sem_m.at[6])]

    def out_cp(t, r, c, slot):
        blk = (_ds(t * T + r * TH, TH), pl.ds(c * KH, KH))
        return pltpu.make_async_copy(outb.at[blk], out_hbm.at[blk], sem_o.at[slot * 4 + r * 2 + c])

    zb[0:8, :] = jnp.zeros((8, 128), F32)
    _start(phi_cp[0], x0_cp(1), wk_cp[0], wk_cp[1], x0_cp(0))

    er = lax.broadcasted_iota(jnp.int32, (128, DH), 0)
    ec = lax.broadcasted_iota(jnp.int32, (128, DH), 1)
    expand = jnp.where((er % 64) // 2 == ec, 1.0, 0.0).astype(BF16)
    pr = lax.broadcasted_iota(jnp.int32, (128, 128), 0)
    pc = lax.broadcasted_iota(jnp.int32, (128, 128), 1)
    diag = pc // DH == 2 * (pr // 64) + pr % 2
    kr = lax.broadcasted_iota(jnp.int32, (64, 128), 0)
    kc = lax.broadcasted_iota(jnp.int32, (64, 128), 1)
    same_head = kr // DH == kc % 2
    kvacc[...] = jnp.zeros_like(kvacc)
    zacc[...] = jnp.zeros_like(zacc)

    def folded(j, g):
        w = wqkv[:, _ds(j * D + g * 128, 128)]
        return lax.dot_general(_unpack(pt[_ds(g * 64, 64), :]), w, NT_DIMS,
                               preferred_element_type=F32) * LOG2E

    def transposed(j, g):
        return wqkv[:, _ds(j * D + g * 128, 128)].T

    def keep(v):
        return v

    def w_terms(r1, r2, dst, b, terms=range(7)):
        dst = dst.at[_ds(b * 64, 6 * WR + 64, 64)]

        def step(h, pin):
            rows = slice(16 * h, 16 * h + 16)
            a = r1[rows, :].astype(F32)
            top = [pin(a[:, :KH]), a[:, KH:]]
            low = None
            if r2 is not None:
                a = r2[rows, :].astype(F32)
                low = [a[:, :KH], pin(a[:, KH:])]
            for n in terms:
                dst[pl.ds(n * WR + h * 8, 8), :] = _pack(_LHS[n]([top, low]))
        return [bind(step, h) for h in range(8)]

    def wo_terms(u):
        src = wo.at[_ds(u * 64, KH + 64, 64)]
        dst = wo_s.at[_ds(u * 32, 6 * (KH // 2) + 32, 32)]

        def step(h, pin):
            r1 = src[pl.ds(KH + h * 16, 16), :].astype(F32)
            r2 = src[pl.ds(h * 16, 16), :].astype(F32)
            quad = [[pin(r1[:, :KH]), r1[:, KH:]], [r2[:, :KH], pin(r2[:, KH:])]]
            for n in range(7):
                dst[pl.ds(n * (KH // 2) + h * 8, 8), :] = _pack(_RHS[n](quad))
        return [bind(step, h) for h in range(4)]

    def x_terms(i, slot, terms=range(7), route=None):
        src = xa.at[_ds(i * T, T)]
        dst = xs.at[_ds(slot * 7 * (TH // 2), 7 * (TH // 2))]
        mix = gate.at[_ds(i * T, T)]

        def step(h, pin):
            x2 = src[pl.ds(TH + h * 16, 16), :].astype(F32)
            quad = [[None, x2[:, :KH]], [None, pin(x2[:, KH:])]]
            if set(terms) - {2, 4}:
                x1 = src[pl.ds(h * 16, 16), :].astype(F32)
                quad[0][0], quad[1][0] = pin(x1[:, :KH]), x1[:, KH:]
            for n in terms:
                dst[pl.ds(n * (TH // 2) + h * 8, 8), :] = _pack(_RHS[n](quad))
            for c in range(2) if route else ():
                row = TH * c + 16 * h
                g = quad[0][c] * gw[:, :KH] + quad[1][c] * gw[:, KH:]
                mix[row:row + 16, :] = jnp.broadcast_to(
                    jax.nn.sigmoid(jnp.sum(g, axis=-1, keepdims=True)), (16, 128))
                r = quad[0][c] * wr[:, :KH] + quad[1][c] * wr[:, KH:]
                r = jnp.sum(r, axis=-1, keepdims=True).astype(BF16).astype(F32)
                tok = i * T + row + lax.broadcasted_iota(jnp.int32, (16, 1), 0)
                best, where = route
                better = (r > best) | ((r == best) & (tok < where))
                route[:] = jnp.where(better, r, best), jnp.where(better, tok, where)
        return [bind(step, h) for h in range(TH // 16)]

    def z_total():
        def step(g, pin):
            rows = slice(128 * g, 128 * g + 128)
            z = jnp.sum(pin(zacc[rows, :]), axis=-1, keepdims=True)
            zb[rows, :] = jnp.broadcast_to(z, (128, 128))
        return [bind(step, g) for g in range(H // 2)]

    def project(w_s, i, n, due, never):
        w = _after(w_s[n * WR:(n + 1) * WR, :], due, never, 0)
        return lax.dot_general(_unpack(w),
                               _unpack(xs[_ds((i * 7 + n) * (TH // 2), TH // 2), :]),
                               NT_DIMS, preferred_element_type=F32)

    def staged(f, plan, todo, never, due=None):
        plan = list(plan)
        due = [] if due is None else due

        def prod(n):
            steps = plan.pop(0)()
            follow = list(todo)
            todo.clear()
            return _shadow(_shadow(f(n, due, never), follow, never, due), steps, never, due)
        return prod

    def keys(i, plan, todo, never, ready=None):
        def step(g, n, p, pin):
            ph = _features(p, pin)
            zs = [_tree(jnp.add, [a[:, 128 * l:128 * l + 128] for l in range(TH // 128)])
                  for a in ph]
            zacc[128 * g:128 * g + 128, :] += jnp.concatenate(zs, axis=0)
            phi[64 * g:64 * g + 64, n * TH:(n + 1) * TH] = _pack(jnp.concatenate(ph, axis=0))
            return zs[0] + zs[8] if ready else None

        def emit(r, n, p):
            todo.extend(bind(step, r * KH // 64 + q, n, p[64 * q:64 * q + 64, :])
                        for q in range(KH // 64))
        prod = staged(bind(project, wk_s, i), plan, todo, never)
        _strassen(lambda n: ready[n] if ready and n in ready else prod(n), emit)

    def values(i, plan, todo, never):
        def emit(r, n, v):
            vt[r * KH // 2:(r + 1) * KH // 2, n * TH:(n + 1) * TH] = _pack(v)
        _strassen(staged(bind(project, wv_s, i), plan, todo, never), emit)
        for g in range(H // 2):
            acc = kvacc[64 * g:64 * g + 64, :] + lax.dot_general(
                _unpack(vt[32 * g:32 * g + 32, :]), _unpack(phi[64 * g:64 * g + 64, :]),
                NT_DIMS, preferred_element_type=F32)
            kvacc[64 * g:64 * g + 64, :] = acc
            kvt[32 * g:32 * g + 32, :] = _pack(jnp.where(same_head, acc, 0.0))

    def q_terms(b):
        return w_terms(folded(0, b), folded(0, b + NB), wq_s, b)

    def fixed(steps):
        return lambda: steps

    never = pltpu.bitcast(zb[0:8, :], jnp.int32)
    _wait(phi_cp[0])
    _start(*vec_cp, phi_cp[1], wk_cp[2], *wv_cp, xa_cp(1), wq_cp, wo_cp,
           *[xa_cp(i) for i in range(2, NT)], *ffn_cp)

    def feature_maps(h):
        for g in range(h * NB, (h + 1) * NB):
            p = lax.dot_general(expand, wphi[g * 128:(g + 1) * 128, :], NT_DIMS,
                                preferred_element_type=F32)
            pt[g * 64:(g + 1) * 64, :] = _pack(jnp.where(diag, p, 0.0))

    feature_maps(0)
    _wait(x0_cp(1))
    for step in x_terms(0, 0, (2, 4)):
        step(keep)
    route = [jnp.full((16, 1), -jnp.inf, F32), jnp.zeros((16, 1), jnp.int32)]
    top, ready = [], {2: [], 4: []}
    for h in range(2):
        if h == 0:
            _wait(wk_cp[0])
            x0 = [[], []]
        else:
            _wait(wk_cp[1], x0_cp(0), *vec_cp, phi_cp[1])
            feature_maps(1)
            gw = gw_ref[...].astype(F32).reshape(1, D)
            wr = wr_ref[...].astype(F32).reshape(1, D)
            x0 = _split(x_terms(0, 0, (0, 1, 3, 5, 6), route), (1, 1))
        for b in (2 * h, 2 * h + 1):
            top.append(folded(1, b))
            for step in w_terms(top[b], None, wk_s, b, (2, 4)):
                step(keep)
        for n, steps in zip(ready, x0):
            ready[n].append(_shadow(lax.dot_general(
                _unpack(wk_s[n * WR + h * 128:n * WR + (h + 1) * 128, :]),
                _unpack(xs[n * (TH // 2):(n + 1) * (TH // 2), :]),
                NT_DIMS, preferred_element_type=F32), steps, never, []))
    ready = {n: jnp.concatenate(m, axis=0) for n, m in ready.items()}
    todo = []

    def rest_of_wk():
        _wait(wk_cp[2])
        for b in range(NB):
            for step in w_terms(top[b], folded(1, b + NB), wk_s, b, (0, 1, 3, 5, 6)):
                step(keep)
        return []

    later = []

    def top_of_wv():
        _wait(wv_cp[0])
        steps = []
        for b in range(NB):
            steps += w_terms(transposed(2, b), None, wv_s, b, (2, 4))
        later.extend(_split(steps, (1, 3)))
        return later.pop(0)

    def rest_of_wv():
        _wait(wv_cp[1])
        steps = []
        for b in range(NB):
            steps += w_terms(transposed(2, b), transposed(2, b + NB), wv_s, b, (0, 1, 3, 5, 6))
        later.extend(_split(steps, (1, 1, 3)))
        return later.pop(0)

    def second_tile():
        _wait(xa_cp(1))
        later.extend(_split(x_terms(1, 1, route=route), (1, 1, 1, 1)))
        return later.pop(0)

    nxt = bind(later.pop, 0)
    keys(0, [rest_of_wk, fixed([]), top_of_wv, nxt, rest_of_wv], todo, never, ready)
    values(0, [nxt, nxt, fixed([]), second_tile, nxt, nxt, nxt], todo, never)
    _wait(wq_cp, wo_cp)

    def phase1(i, route):
        route = list(route)
        never = jnp.where(jnp.full((8, 128), i, jnp.int32) < 0, 1, 0)
        pl.when(i + 1 < NT)(lambda: _wait(xa_cp(i + 1)))
        todo = []
        plan = _split(x_terms(jnp.minimum(i + 1, NT - 1), i + 1, route=route), X_SHARES)
        for n, steps in enumerate(_split(z_total(), Z_SHARES)):
            plan[n] += steps
        for n, slot in enumerate(WO_SLOTS):
            plan[slot] += wo_terms(jnp.minimum(3 * (i - 1) + n, KH // 64 - 1))
        q = []

        def with_q(n):
            if Q_SHARES[n] and not q:
                q.extend(_split(q_terms(i - 1), Q_SHARES))
            return (q[n] if q else []) + plan[n]

        keys(i, [bind(with_q, n) for n in range(7)], todo, never)
        values(i, [fixed(s) for s in plan[7:]], todo, never)
        return tuple(route)

    route = lax.fori_loop(1, NT, phase1, tuple(route))

    for step in q_terms(NB - 1):
        step(keep)

    best = jnp.max(route[0], axis=0, keepdims=True)
    idx = jnp.min(jnp.where(route[0] == best, route[1], S - 1))
    first = idx // T
    slab = pl.ds(pl.multiple_of((idx // 16) * 16, 16), 16)
    sel = lax.broadcasted_iota(jnp.int32, (16, D), 0) == idx % 16
    _wait(*ffn_cp)

    def x_column():
        def step(k, pin):
            cols = slice(128 * k, 128 * k + 128)
            row = jnp.where(sel[:, cols], pin(xa[slab, cols].astype(F32)), 0.0)
            row = jnp.sum(row, axis=0, keepdims=True)
            xcol[cols, :] = jnp.broadcast_to(row, (128, 128)).T
        return [bind(step, k) for k in range(D // 128)]

    def fold8(x):
        return jnp.sum(x.reshape(x.shape[0] // 8, 8, 128), axis=0)

    def ffn_steps(i, y):
        st = {}
        part = _ds(i * FC, FC, 128)
        wg_i, wu_i, wd_i = wg.at[:, part], wu.at[:, part], wd.at[part]

        def up(j, k, pin):
            f = pl.ds(j * 128, 128)
            rows = slice(64 * k, 64 * k + 64)
            xc = xcol[rows, :]
            a = fold8(wg_i[rows, f].astype(F32) * xc)
            u = fold8(wu_i[rows, f].astype(F32) * xc)
            if k > 0:
                a, u = pin(st["a"]) + a, pin(st["u"]) + u
            st["a"], st["u"] = a, u
            token = a + u
            if k == D // 64 - 1:
                a = jnp.sum(a, axis=0, keepdims=True)
                u = jnp.sum(u, axis=0, keepdims=True)
                st["h"] = jnp.broadcast_to(a * jax.nn.sigmoid(a) * u, (128, 128)).T
            return token

        def down(j, n, pin):
            w = wd_i[j * 128:j * 128 + 128, 128 * n:128 * n + 128].astype(F32)
            y[n] = pin(y[n]) + fold8(w * st["h"])
            return y[n]

        steps = []
        for j in range(FC // 128):
            steps += [bind(up, j, k) for k in range(D // 64)]
            steps += [bind(down, j, n) for n in range(D // 128)]
        return steps

    def phase2(i, y):
        y = list(y)
        t = (first + i) % NT
        never = jnp.where(jnp.full((8, 128), i, jnp.int32) < 0, 1, 0)
        o = [[[], []], [[], []]]
        todo = []

        def attend(g, dst, ph, rden, pin):
            num = jnp.dot(_unpack(pin(kvt[32 * g:32 * g + 32, :])), ph,
                          preferred_element_type=F32)
            scale = jnp.concatenate(
                [jnp.broadcast_to(rden[0:1, :], (DH, TH)),
                 jnp.broadcast_to(rden[1:2, :], (DH, TH))], axis=0)
            dst.append(num * scale)

        def query(g, dst, p, pin):
            ph = _features(p, pin)
            z = zb[128 * g:128 * g + 128, :]
            dn = [a * jnp.tile(z[8 * k:8 * k + 8, :], (1, TH // 128)) for k, a in enumerate(ph)]
            rden = _recip(_allreduce(jnp.add, dn) + 1e-6)
            todo.append(bind(attend, g, dst, jnp.concatenate(ph, axis=0).astype(BF16), rden))

        def emit_q(r, n, p):
            todo.extend(bind(query, r * KH // 64 + q, o[n][1 - r], p[64 * q:64 * q + 64, :])
                        for q in range(KH // 64))

        def relaxed(step):
            def run(pin):
                step(pin)
            return run

        ffn = [steps if deadline else [relaxed(step) for step in steps]
               for steps, deadline in zip(_split(ffn_steps(i, y), FFN_SHARES), FFN_DEADLINE)]
        plan = [fixed(s) for s in [x_column() + ffn[0]] + ffn[1:]]
        due = []
        _strassen(staged(bind(project, wq_s, t), plan[:7], todo, never, due), emit_q)

        class Quad:
            def __init__(self, n):
                self.n = n

            def __getitem__(self, r):
                return jnp.concatenate(o[self.n][r], axis=0)

        def prod_o(n, due, never):
            w = _after(wo_s[n * (KH // 2):(n + 1) * (KH // 2), :], due, never, 1)
            return lax.dot_general(_LHS[n]([Quad(0), Quad(1)]).astype(BF16), _unpack(w),
                                   TN_DIMS, preferred_element_type=F32)

        def emit_o(n, c, a):
            gt = jnp.tile(gate[_ds(t * T + n * TH, TH), :], (1, KH // 128))
            b = xa[_ds(t * T + n * TH, TH), c * KH:(c + 1) * KH].astype(F32)
            outb[_ds(t * T + n * TH, TH), c * KH:(c + 1) * KH] = (
                gt * a + (1.0 - gt) * b).astype(BF16)
            out_cp(t, n, c, i).start()

        _strassen_diag(staged(prod_o, plan[7:], todo, never, due), emit_o)
        return tuple(y)

    y = lax.fori_loop(0, NT, phase2, (jnp.zeros((8, 128), F32),) * (D // 128))

    _wait(*[out_cp(first, r, c, 0) for r in range(2) for c in range(2)])
    y = jnp.sum(jnp.concatenate(y, axis=1), axis=0, keepdims=True) * jax.nn.sigmoid(best)
    xsl = xa[slab, :].astype(F32)
    upd = (xsl + y).astype(BF16).astype(F32) - xsl
    gt = jnp.tile(gate[slab, :], (1, D // 128))
    old = outb[slab, :].astype(F32)
    outb[slab, :] = jnp.where(sel, old + (1.0 - gt) * upd, old).astype(BF16)
    fix_cp = pltpu.make_async_copy(outb.at[slab], out_hbm.at[slab], sem_x.at[NT])
    fix_cp.start()
    _wait(fix_cp, *[out_cp((first + i) % NT, r, c, i)
                    for i in range(1, NT) for r in range(2) for c in range(2)])


@jax.jit
def pallas_gated_mix__linear_kernel_hedgehog__moe_arch_mod__prompt_kernel(
    A_x, A_wqkv, A_w_phi, A_wo, B_x, B_w_r, B_w_gate, B_w_up, B_w_down, gate_w,
):
    del B_x
    hbm = pl.BlockSpec(memory_space=pl.ANY)
    out = pl.pallas_call(
        _kernel,
        out_shape=jax.ShapeDtypeStruct((S, D), BF16),
        in_specs=[hbm] * 9,
        out_specs=hbm,
        scratch_shapes=[
            pltpu.VMEM((S, D), BF16),
            pltpu.VMEM((D, 3 * D), BF16),
            pltpu.VMEM((D, DH), BF16),
            pltpu.VMEM((D, D), BF16),
            pltpu.VMEM((D, F), BF16),
            pltpu.VMEM((D, F), BF16),
            pltpu.VMEM((F, D), BF16),
            pltpu.VMEM((7 * WR, KH), U32),
            pltpu.VMEM((7 * WR, KH), U32),
            pltpu.VMEM((7 * WR, KH), U32),
            pltpu.VMEM((7 * KH // 2, KH), U32),
            pltpu.VMEM(((NT + 1) * 7 * TH // 2, KH), U32),
            pltpu.VMEM((D // 2, 128), U32),
            pltpu.VMEM((D // 2, T), U32),
            pltpu.VMEM((D, T), U32),
            pltpu.VMEM((D, 128), F32),
            pltpu.VMEM((D // 2, 128), U32),
            pltpu.VMEM((2 * D, 128), F32),
            pltpu.VMEM((2 * D, 128), F32),
            pltpu.VMEM((S, 128), F32),
            pltpu.VMEM((S, D), BF16),
            pltpu.VMEM((D, 128), F32),
            pltpu.VMEM((D,), BF16),
            pltpu.VMEM((D,), BF16),
            pltpu.SemaphoreType.DMA((NT + 1,)),
            pltpu.SemaphoreType.DMA((6,)),
            pltpu.SemaphoreType.DMA((10,)),
            pltpu.SemaphoreType.DMA((4 * NT,)),
        ],
        compiler_params=pltpu.CompilerParams(vmem_limit_bytes=110 * 2**20),
    )(A_x.reshape(S, D), A_wqkv, A_w_phi.reshape(H * DH, DH), A_wo,
      B_w_r, B_w_gate, B_w_up, B_w_down, gate_w)
    return out.reshape(1, S, D)
```

```python
import functools

import jax
import jax.numpy as jnp
from jax import lax
from jax.experimental import pallas as pl
from jax.experimental.pallas import tpu as pltpu

S, D, H, DH, F = 2048, 1024, 32, 32, 3584
T = 512
NT = S // T
TH, KH = T // 2, D // 2
WR = KH // 2
NB = KH // 128
FC = F // NT
FFN_SHARES = (0, 4, 0, 2, 0, 2, 0, 0, 2, 4, 1, 2, 2, 2)
FFN_DEADLINE = (1, 0, 1, 1, 1, 0, 1, 1, 1, 1, 1, 1, 0, 1)
Q_SHARES = (0, 1, 0, 0, 0, 1, 0)
X_SHARES = (0, 0, 0, 0, 0, 0, 0, 0, 1, 1, 2, 0, 0, 0)
Z_SHARES = (0, 0, 0, 0, 0, 0, 0, 0, 0, 1, 0, 1, 0, 1)
WO_SLOTS = (11, 10, 9)
LOG2E = 1.4426950408889634
F32, BF16, U32 = jnp.float32, jnp.bfloat16, jnp.uint32
NT_DIMS = (((1,), (1,)), ((), ()))
TN_DIMS = (((0,), (0,)), ((), ()))
bind = functools.partial


def _tree(op, xs):
    xs = list(xs)
    while len(xs) > 1:
        xs = [op(xs[i], xs[i + 1]) if i + 1 < len(xs) else xs[i]
              for i in range(0, len(xs), 2)]
    return xs[0]


def _allreduce(op, xs):
    r = _tree(op, xs)
    r = op(r, pltpu.roll(r, 4, 0))
    return op(r, pltpu.roll(r, 2, 0))


def _recip(x):
    r = pl.reciprocal(x, approx=True)
    return r * (2.0 - x * r)


def _features(p, pin):
    rows = [p[8 * i:8 * i + 8, :] for i in range(8)]
    rows[0] = pin(rows[0])
    mx = _allreduce(jnp.maximum, rows)
    mn = _allreduce(jnp.minimum, rows)
    ep = [jnp.exp2(r - mx) for r in rows]
    en = [jnp.exp2(mn - r) for r in rows]
    rp = _recip(_allreduce(jnp.add, ep))
    rn = _recip(_allreduce(jnp.add, en))
    return [e * rp for e in ep] + [e * rn for e in en]


def _pack(x):
    return pltpu.bitcast(x.astype(BF16), U32)


def _unpack(x):
    return pltpu.bitcast(x, BF16)


_LHS = [lambda a: a[0][0] + a[1][1], lambda a: a[1][0] + a[1][1], lambda a: a[0][0],
        lambda a: a[1][1], lambda a: a[0][0] + a[0][1], lambda a: a[1][0] - a[0][0],
        lambda a: a[0][1] - a[1][1]]
_RHS = [lambda b: b[0][0] + b[1][1], lambda b: b[0][0], lambda b: b[0][1] - b[1][1],
        lambda b: b[1][0] - b[0][0], lambda b: b[1][1], lambda b: b[0][0] + b[0][1],
        lambda b: b[1][0] + b[1][1]]


def _strassen(prod, emit):
    m3 = prod(2)
    m5 = prod(4)
    emit(0, 1, m3 + m5)
    m2 = prod(1)
    m4 = prod(3)
    emit(1, 0, m2 + m4)
    m1 = prod(0)
    s1 = m4 - m5 + m1
    s2 = m3 - m2 + m1
    emit(0, 0, s1 + prod(6))
    emit(1, 1, s2 + prod(5))


def _strassen_diag(prod, emit):
    m3 = prod(2)
    m4 = prod(3)
    m1 = prod(0)
    m5 = prod(4)
    emit(0, 1, m3 + m5)
    emit(0, 0, m1 + m4 - m5 + prod(6))
    m2 = prod(1)
    emit(1, 0, m2 + m4)
    emit(1, 1, m1 + m3 - m2 + prod(5))


def _shadow(m, steps, never, due):
    rows, cols = m.shape[0] // 8, m.shape[1] // 128
    for s, step in enumerate(steps):
        p = rows * cols * s // len(steps)
        r, c = 8 * (p % rows), 128 * (p // rows)
        slab = m[r:r + 8, c:c + 128]

        def pin(v, slab=slab):
            reps = (v.shape[0] // 8, v.shape[1] // 128)
            other = slab if v.dtype == F32 else pltpu.bitcast(slab, v.dtype)
            return jnp.where(jnp.tile(never, reps) != 0, jnp.tile(other, reps), v)

        token = step(pin)
        if token is not None:
            due.append(token)
    return m


def _after(w, due, never, axis):
    if not due:
        return w
    unit = (8, 128)[axis]
    parts = jnp.split(w, w.shape[axis] // unit, axis=axis)
    for s, token in enumerate(due):
        p = len(parts) * s // len(due)
        head = jnp.where(never != 0, pltpu.bitcast(token, U32), parts[p][:8, :128])
        if axis == 0:
            parts[p] = jnp.concatenate([head, parts[p][:, 128:]], axis=1)
        else:
            parts[p] = jnp.concatenate([head, parts[p][8:, :]], axis=0)
    due.clear()
    return jnp.concatenate(parts, axis=axis)


def _split(steps, shares):
    out, done, total = [], 0, 0
    for s in shares:
        total += s
        end = len(steps) * total // sum(shares)
        out.append(steps[done:end])
        done = end
    return out


def _start(*cps):
    def step(i, carry):
        for n, cp in enumerate(cps):
            pl.when(i == n)(cp.start)
        return carry

    lax.fori_loop(0, len(cps), step, 0)


def _wait(*cps):
    for cp in cps:
        cp.wait()


def _ds(start, size, mult=None):
    if isinstance(start, int):
        return pl.ds(start, size)
    return pl.ds(pl.multiple_of(start, mult or size), size)


def _kernel(xa_hbm, wqkv_hbm, wphi_hbm, wo_hbm, wr_hbm, wg_hbm, wu_hbm,
            wd_hbm, gw_hbm, out_hbm,
            xa, wqkv, wphi, wo, wg, wu, wd, wq_s, wk_s, wv_s, wo_s, xs, pt, vt, phi,
            kvacc, kvt, zacc, zb, gate, outb, xcol, wr_ref, gw_ref,
            sem_x, sem_w, sem_m, sem_o):
    def xa_cp(i):
        return pltpu.make_async_copy(xa_hbm.at[_ds(i * T, T)], xa.at[_ds(i * T, T)], sem_x.at[i])

    def w_cp(start, size, sem):
        cols = pl.ds(start, size)
        return pltpu.make_async_copy(wqkv_hbm.at[:, cols], wqkv.at[:, cols], sem_w.at[sem])

    def x0_cp(h):
        rows = pl.ds(h * TH, TH)
        return pltpu.make_async_copy(xa_hbm.at[rows], xa.at[rows], sem_m.at[h])

    wk_cp = [w_cp(D, KH // 2, 0), w_cp(D + KH // 2, KH // 2, 1), w_cp(D + KH, KH, 2)]
    wv_cp = [w_cp(2 * D, KH, 3), w_cp(2 * D + KH, KH, 4)]
    wq_cp = w_cp(0, D, 5)
    phi_cp = [pltpu.make_async_copy(wphi_hbm.at[pl.ds(h * KH, KH)], wphi.at[pl.ds(h * KH, KH)],
                                    sem_m.at[2 + 5 * h]) for h in range(2)]
    vec_cp = [pltpu.make_async_copy(wr_hbm, wr_ref, sem_m.at[8]),
              pltpu.make_async_copy(gw_hbm, gw_ref, sem_m.at[9])]
    wo_cp = pltpu.make_async_copy(wo_hbm, wo, sem_m.at[3])
    ffn_cp = [pltpu.make_async_copy(wg_hbm, wg, sem_m.at[4]),
              pltpu.make_async_copy(wu_hbm, wu, sem_m.at[5]),
              pltpu.make_async_copy(wd_hbm, wd, sem_m.at[6])]

    def out_cp(t, r, c, slot):
        blk = (_ds(t * T + r * TH, TH), pl.ds(c * KH, KH))
        return pltpu.make_async_copy(outb.at[blk], out_hbm.at[blk], sem_o.at[slot * 4 + r * 2 + c])

    zb[0:8, :] = jnp.zeros((8, 128), F32)
    _start(phi_cp[0], x0_cp(1), wk_cp[0], wk_cp[1], x0_cp(0))

    er = lax.broadcasted_iota(jnp.int32, (128, DH), 0)
    ec = lax.broadcasted_iota(jnp.int32, (128, DH), 1)
    expand = jnp.where((er % 64) // 2 == ec, 1.0, 0.0).astype(BF16)
    pr = lax.broadcasted_iota(jnp.int32, (128, 128), 0)
    pc = lax.broadcasted_iota(jnp.int32, (128, 128), 1)
    diag = pc // DH == 2 * (pr // 64) + pr % 2
    kr = lax.broadcasted_iota(jnp.int32, (64, 128), 0)
    kc = lax.broadcasted_iota(jnp.int32, (64, 128), 1)
    same_head = kr // DH == kc % 2
    kvacc[...] = jnp.zeros_like(kvacc)
    zacc[...] = jnp.zeros_like(zacc)

    def folded(j, g):
        w = wqkv[:, _ds(j * D + g * 128, 128)]
        return lax.dot_general(_unpack(pt[_ds(g * 64, 64), :]), w, NT_DIMS,
                               preferred_element_type=F32) * LOG2E

    def transposed(j, g):
        return wqkv[:, _ds(j * D + g * 128, 128)].T

    def keep(v):
        return v

    def w_terms(r1, r2, dst, b, terms=range(7)):
        dst = dst.at[_ds(b * 64, 6 * WR + 64, 64)]

        def step(h, pin):
            rows = slice(16 * h, 16 * h + 16)
            a = r1[rows, :].astype(F32)
            top = [pin(a[:, :KH]), a[:, KH:]]
            low = None
            if r2 is not None:
                a = r2[rows, :].astype(F32)
                low = [a[:, :KH], pin(a[:, KH:])]
            for n in terms:
                dst[pl.ds(n * WR + h * 8, 8), :] = _pack(_LHS[n]([top, low]))
        return [bind(step, h) for h in range(8)]

    def wo_terms(u):
        src = wo.at[_ds(u * 64, KH + 64, 64)]
        dst = wo_s.at[_ds(u * 32, 6 * (KH // 2) + 32, 32)]

        def step(h, pin):
            r1 = src[pl.ds(KH + h * 16, 16), :].astype(F32)
            r2 = src[pl.ds(h * 16, 16), :].astype(F32)
            quad = [[pin(r1[:, :KH]), r1[:, KH:]], [r2[:, :KH], pin(r2[:, KH:])]]
            for n in range(7):
                dst[pl.ds(n * (KH // 2) + h * 8, 8), :] = _pack(_RHS[n](quad))
        return [bind(step, h) for h in range(4)]

    def x_terms(i, slot, terms=range(7), route=None):
        src = xa.at[_ds(i * T, T)]
        dst = xs.at[_ds(slot * 7 * (TH // 2), 7 * (TH // 2))]
        mix = gate.at[_ds(i * T, T)]

        def step(h, pin):
            x2 = src[pl.ds(TH + h * 16, 16), :].astype(F32)
            quad = [[None, x2[:, :KH]], [None, pin(x2[:, KH:])]]
            if set(terms) - {2, 4}:
                x1 = src[pl.ds(h * 16, 16), :].astype(F32)
                quad[0][0], quad[1][0] = pin(x1[:, :KH]), x1[:, KH:]
            for n in terms:
                dst[pl.ds(n * (TH // 2) + h * 8, 8), :] = _pack(_RHS[n](quad))
            for c in range(2) if route else ():
                row = TH * c + 16 * h
                g = quad[0][c] * gw[:, :KH] + quad[1][c] * gw[:, KH:]
                mix[row:row + 16, :] = jnp.broadcast_to(
                    jax.nn.sigmoid(jnp.sum(g, axis=-1, keepdims=True)), (16, 128))
                r = quad[0][c] * wr[:, :KH] + quad[1][c] * wr[:, KH:]
                r = jnp.sum(r, axis=-1, keepdims=True).astype(BF16).astype(F32)
                tok = i * T + row + lax.broadcasted_iota(jnp.int32, (16, 1), 0)
                best, where = route
                better = (r > best) | ((r == best) & (tok < where))
                route[:] = jnp.where(better, r, best), jnp.where(better, tok, where)
        return [bind(step, h) for h in range(TH // 16)]

    def z_total():
        def step(g, pin):
            rows = slice(128 * g, 128 * g + 128)
            z = jnp.sum(pin(zacc[rows, :]), axis=-1, keepdims=True)
            zb[rows, :] = jnp.broadcast_to(z, (128, 128))
        return [bind(step, g) for g in range(H // 2)]

    def project(w_s, i, n, due, never):
        w = _after(w_s[n * WR:(n + 1) * WR, :], due, never, 0)
        return lax.dot_general(_unpack(w),
                               _unpack(xs[_ds((i * 7 + n) * (TH // 2), TH // 2), :]),
                               NT_DIMS, preferred_element_type=F32)

    def staged(f, plan, todo, never, due=None):
        plan = list(plan)
        due = [] if due is None else due

        def prod(n):
            steps = plan.pop(0)()
            follow = list(todo)
            todo.clear()
            return _shadow(_shadow(f(n, due, never), follow, never, due), steps, never, due)
        return prod

    def keys(i, plan, todo, never, ready=None):
        def step(g, n, p, pin):
            ph = _features(p, pin)
            zs = [_tree(jnp.add, [a[:, 128 * l:128 * l + 128] for l in range(TH // 128)])
                  for a in ph]
            zacc[128 * g:128 * g + 128, :] += jnp.concatenate(zs, axis=0)
            phi[64 * g:64 * g + 64, n * TH:(n + 1) * TH] = _pack(jnp.concatenate(ph, axis=0))
            return zs[0] + zs[8] if ready else None

        def emit(r, n, p):
            todo.extend(bind(step, r * KH // 64 + q, n, p[64 * q:64 * q + 64, :])
                        for q in range(KH // 64))
        prod = staged(bind(project, wk_s, i), plan, todo, never)
        _strassen(lambda n: ready[n] if ready and n in ready else prod(n), emit)

    def values(i, plan, todo, never):
        def emit(r, n, v):
            vt[r * KH // 2:(r + 1) * KH // 2, n * TH:(n + 1) * TH] = _pack(v)
        _strassen(staged(bind(project, wv_s, i), plan, todo, never), emit)
        for g in range(H // 2):
            acc = kvacc[64 * g:64 * g + 64, :] + lax.dot_general(
                _unpack(vt[32 * g:32 * g + 32, :]), _unpack(phi[64 * g:64 * g + 64, :]),
                NT_DIMS, preferred_element_type=F32)
            kvacc[64 * g:64 * g + 64, :] = acc
            kvt[32 * g:32 * g + 32, :] = _pack(jnp.where(same_head, acc, 0.0))

    def q_terms(b):
        return w_terms(folded(0, b), folded(0, b + NB), wq_s, b)

    def fixed(steps):
        return lambda: steps

    never = pltpu.bitcast(zb[0:8, :], jnp.int32)
    _wait(phi_cp[0])
    _start(*vec_cp, phi_cp[1], wk_cp[2], wv_cp[0], xa_cp(1), wv_cp[1], wq_cp, wo_cp,
           *[xa_cp(i) for i in range(2, NT)], *ffn_cp)

    def feature_maps(h):
        for g in range(h * NB, (h + 1) * NB):
            p = lax.dot_general(expand, wphi[g * 128:(g + 1) * 128, :], NT_DIMS,
                                preferred_element_type=F32)
            pt[g * 64:(g + 1) * 64, :] = _pack(jnp.where(diag, p, 0.0))

    feature_maps(0)
    _wait(x0_cp(1))
    for step in x_terms(0, 0, (2, 4)):
        step(keep)
    route = [jnp.full((16, 1), -jnp.inf, F32), jnp.zeros((16, 1), jnp.int32)]
    top, ready = [], {2: [], 4: []}
    for h in range(2):
        if h == 0:
            _wait(wk_cp[0])
            x0 = [[], []]
        else:
            _wait(wk_cp[1], x0_cp(0), *vec_cp, phi_cp[1])
            feature_maps(1)
            gw = gw_ref[...].astype(F32).reshape(1, D)
            wr = wr_ref[...].astype(F32).reshape(1, D)
            x0 = _split(x_terms(0, 0, (0, 1, 3, 5, 6), route), (1, 1))
        for b in (2 * h, 2 * h + 1):
            top.append(folded(1, b))
            for step in w_terms(top[b], None, wk_s, b, (2, 4)):
                step(keep)
        for n, steps in zip(ready, x0):
            ready[n].append(_shadow(lax.dot_general(
                _unpack(wk_s[n * WR + h * 128:n * WR + (h + 1) * 128, :]),
                _unpack(xs[n * (TH // 2):(n + 1) * (TH // 2), :]),
                NT_DIMS, preferred_element_type=F32), steps, never, []))
    ready = {n: jnp.concatenate(m, axis=0) for n, m in ready.items()}
    todo = []

    def rest_of_wk():
        _wait(wk_cp[2])
        for b in range(NB):
            for step in w_terms(top[b], folded(1, b + NB), wk_s, b, (0, 1, 3, 5, 6)):
                step(keep)
        return []

    later = []

    def top_of_wv():
        _wait(wv_cp[0])
        steps = []
        top[:] = [transposed(2, b) for b in range(NB)]
        for b in range(NB):
            steps += w_terms(top[b], None, wv_s, b, (2, 4))
        later.extend(_split(steps, (1, 3)))
        return later.pop(0)

    def rest_of_wv():
        _wait(wv_cp[1], xa_cp(1))
        steps = []
        for b in range(NB):
            steps += w_terms(top[b], transposed(2, b + NB), wv_s, b, (0, 1, 3, 5, 6))
        later.extend(_split(steps, (1, 1, 3)))
        return later.pop(0)

    def second_tile():
        later.extend(_split(x_terms(1, 1, route=route), (1, 1, 1, 1, 1)))
        return later.pop(0)

    nxt = bind(later.pop, 0)
    keys(0, [rest_of_wk, fixed([]), top_of_wv, nxt, rest_of_wv], todo, never, ready)
    values(0, [nxt, nxt, second_tile, nxt, nxt, nxt, nxt], todo, never)
    _wait(wq_cp, wo_cp)

    def phase1(i, route):
        route = list(route)
        never = jnp.where(jnp.full((8, 128), i, jnp.int32) < 0, 1, 0)
        pl.when(i + 1 < NT)(lambda: _wait(xa_cp(i + 1)))
        todo = []
        plan = _split(x_terms(jnp.minimum(i + 1, NT - 1), i + 1, route=route), X_SHARES)
        for n, steps in enumerate(_split(z_total(), Z_SHARES)):
            plan[n] += steps
        for n, slot in enumerate(WO_SLOTS):
            plan[slot] += wo_terms(jnp.minimum(3 * (i - 1) + n, KH // 64 - 1))
        q = []

        def with_q(n):
            if Q_SHARES[n] and not q:
                q.extend(_split(q_terms(i - 1), Q_SHARES))
            return (q[n] if q else []) + plan[n]

        keys(i, [bind(with_q, n) for n in range(7)], todo, never)
        values(i, [fixed(s) for s in plan[7:]], todo, never)
        return tuple(route)

    route = lax.fori_loop(1, NT, phase1, tuple(route))

    for step in q_terms(NB - 1):
        step(keep)

    best = jnp.max(route[0], axis=0, keepdims=True)
    idx = jnp.min(jnp.where(route[0] == best, route[1], S - 1))
    first = idx // T
    slab = pl.ds(pl.multiple_of((idx // 16) * 16, 16), 16)
    sel = lax.broadcasted_iota(jnp.int32, (16, D), 0) == idx % 16
    _wait(*ffn_cp)

    def x_column():
        def step(k, pin):
            cols = slice(128 * k, 128 * k + 128)
            row = jnp.where(sel[:, cols], pin(xa[slab, cols].astype(F32)), 0.0)
            row = jnp.sum(row, axis=0, keepdims=True)
            xcol[cols, :] = jnp.broadcast_to(row, (128, 128)).T
        return [bind(step, k) for k in range(D // 128)]

    def fold8(x):
        return jnp.sum(x.reshape(x.shape[0] // 8, 8, 128), axis=0)

    def ffn_steps(i, y):
        st = {}
        part = _ds(i * FC, FC, 128)
        wg_i, wu_i, wd_i = wg.at[:, part], wu.at[:, part], wd.at[part]

        def up(j, k, pin):
            f = pl.ds(j * 128, 128)
            rows = slice(64 * k, 64 * k + 64)
            xc = xcol[rows, :]
            a = fold8(wg_i[rows, f].astype(F32) * xc)
            u = fold8(wu_i[rows, f].astype(F32) * xc)
            if k > 0:
                a, u = pin(st["a"]) + a, pin(st["u"]) + u
            st["a"], st["u"] = a, u
            token = a + u
            if k == D // 64 - 1:
                a = jnp.sum(a, axis=0, keepdims=True)
                u = jnp.sum(u, axis=0, keepdims=True)
                st["h"] = jnp.broadcast_to(a * jax.nn.sigmoid(a) * u, (128, 128)).T
            return token

        def down(j, n, pin):
            w = wd_i[j * 128:j * 128 + 128, 128 * n:128 * n + 128].astype(F32)
            y[n] = pin(y[n]) + fold8(w * st["h"])
            return y[n]

        steps = []
        for j in range(FC // 128):
            steps += [bind(up, j, k) for k in range(D // 64)]
            steps += [bind(down, j, n) for n in range(D // 128)]
        return steps

    def phase2(i, y):
        y = list(y)
        t = (first + i) % NT
        never = jnp.where(jnp.full((8, 128), i, jnp.int32) < 0, 1, 0)
        o = [[[], []], [[], []]]
        todo = []

        def attend(g, dst, ph, rden, pin):
            num = jnp.dot(_unpack(pin(kvt[32 * g:32 * g + 32, :])), ph,
                          preferred_element_type=F32)
            scale = jnp.concatenate(
                [jnp.broadcast_to(rden[0:1, :], (DH, TH)),
                 jnp.broadcast_to(rden[1:2, :], (DH, TH))], axis=0)
            dst.append(num * scale)

        def query(g, dst, p, pin):
            ph = _features(p, pin)
            z = zb[128 * g:128 * g + 128, :]
            dn = [a * jnp.tile(z[8 * k:8 * k + 8, :], (1, TH // 128)) for k, a in enumerate(ph)]
            rden = _recip(_allreduce(jnp.add, dn) + 1e-6)
            todo.append(bind(attend, g, dst, jnp.concatenate(ph, axis=0).astype(BF16), rden))

        def emit_q(r, n, p):
            todo.extend(bind(query, r * KH // 64 + q, o[n][1 - r], p[64 * q:64 * q + 64, :])
                        for q in range(KH // 64))

        def relaxed(step):
            def run(pin):
                step(pin)
            return run

        ffn = [steps if deadline else [relaxed(step) for step in steps]
               for steps, deadline in zip(_split(ffn_steps(i, y), FFN_SHARES), FFN_DEADLINE)]
        plan = [fixed(s) for s in [x_column() + ffn[0]] + ffn[1:]]
        due = []
        _strassen(staged(bind(project, wq_s, t), plan[:7], todo, never, due), emit_q)

        class Quad:
            def __init__(self, n):
                self.n = n

            def __getitem__(self, r):
                return jnp.concatenate(o[self.n][r], axis=0)

        def prod_o(n, due, never):
            w = _after(wo_s[n * (KH // 2):(n + 1) * (KH // 2), :], due, never, 1)
            return lax.dot_general(_LHS[n]([Quad(0), Quad(1)]).astype(BF16), _unpack(w),
                                   TN_DIMS, preferred_element_type=F32)

        def emit_o(n, c, a):
            gt = jnp.tile(gate[_ds(t * T + n * TH, TH), :], (1, KH // 128))
            b = xa[_ds(t * T + n * TH, TH), c * KH:(c + 1) * KH].astype(F32)
            outb[_ds(t * T + n * TH, TH), c * KH:(c + 1) * KH] = (
                gt * a + (1.0 - gt) * b).astype(BF16)
            out_cp(t, n, c, i).start()

        _strassen_diag(staged(prod_o, plan[7:], todo, never, due), emit_o)
        return tuple(y)

    y = lax.fori_loop(0, NT, phase2, (jnp.zeros((8, 128), F32),) * (D // 128))

    _wait(*[out_cp(first, r, c, 0) for r in range(2) for c in range(2)])
    y = jnp.sum(jnp.concatenate(y, axis=1), axis=0, keepdims=True) * jax.nn.sigmoid(best)
    xsl = xa[slab, :].astype(F32)
    upd = (xsl + y).astype(BF16).astype(F32) - xsl
    gt = jnp.tile(gate[slab, :], (1, D // 128))
    old = outb[slab, :].astype(F32)
    outb[slab, :] = jnp.where(sel, old + (1.0 - gt) * upd, old).astype(BF16)
    fix_cp = pltpu.make_async_copy(outb.at[slab], out_hbm.at[slab], sem_x.at[NT])
    fix_cp.start()
    _wait(fix_cp, *[out_cp((first + i) % NT, r, c, i)
                    for i in range(1, NT) for r in range(2) for c in range(2)])


@jax.jit
def pallas_gated_mix__linear_kernel_hedgehog__moe_arch_mod__prompt_kernel(
    A_x, A_wqkv, A_w_phi, A_wo, B_x, B_w_r, B_w_gate, B_w_up, B_w_down, gate_w,
):
    del B_x
    hbm = pl.BlockSpec(memory_space=pl.ANY)
    out = pl.pallas_call(
        _kernel,
        out_shape=jax.ShapeDtypeStruct((S, D), BF16),
        in_specs=[hbm] * 9,
        out_specs=hbm,
        scratch_shapes=[
            pltpu.VMEM((S, D), BF16),
            pltpu.VMEM((D, 3 * D), BF16),
            pltpu.VMEM((D, DH), BF16),
            pltpu.VMEM((D, D), BF16),
            pltpu.VMEM((D, F), BF16),
            pltpu.VMEM((D, F), BF16),
            pltpu.VMEM((F, D), BF16),
            pltpu.VMEM((7 * WR, KH), U32),
            pltpu.VMEM((7 * WR, KH), U32),
            pltpu.VMEM((7 * WR, KH), U32),
            pltpu.VMEM((7 * KH // 2, KH), U32),
            pltpu.VMEM(((NT + 1) * 7 * TH // 2, KH), U32),
            pltpu.VMEM((D // 2, 128), U32),
            pltpu.VMEM((D // 2, T), U32),
            pltpu.VMEM((D, T), U32),
            pltpu.VMEM((D, 128), F32),
            pltpu.VMEM((D // 2, 128), U32),
            pltpu.VMEM((2 * D, 128), F32),
            pltpu.VMEM((2 * D, 128), F32),
            pltpu.VMEM((S, 128), F32),
            pltpu.VMEM((S, D), BF16),
            pltpu.VMEM((D, 128), F32),
            pltpu.VMEM((D,), BF16),
            pltpu.VMEM((D,), BF16),
            pltpu.SemaphoreType.DMA((NT + 1,)),
            pltpu.SemaphoreType.DMA((6,)),
            pltpu.SemaphoreType.DMA((10,)),
            pltpu.SemaphoreType.DMA((4 * NT,)),
        ],
        compiler_params=pltpu.CompilerParams(vmem_limit_bytes=110 * 2**20),
    )(A_x.reshape(S, D), A_wqkv, A_w_phi.reshape(H * DH, DH), A_wo,
      B_w_r, B_w_gate, B_w_up, B_w_down, gate_w)
    return out.reshape(1, S, D)
```
